```python
import jax
import jax.numpy as jnp

def _softmax(x, axis=-1):
    return jax.nn.softmax(x, axis=axis)

def _gelu(x):
    return jax.nn.gelu(x, approximate=True)

def _silu(x):
    return jax.nn.silu(x)

def _sigmoid(x):
    return jax.nn.sigmoid(x)

def _layernorm(x, axis=-1, eps=1e-05):
    m = jnp.mean(x, axis=axis, keepdims=True)
    v = jnp.var(x, axis=axis, keepdims=True)
    return (x - m) / jnp.sqrt(v + eps)

def _scatter_add(tgt, idx, src, axis=0):
    return tgt.at[idx].add(src)

def _segment_sum(src, seg, n):
    return jax.ops.segment_sum(src, seg, n)

class _Rng:

    def __init__(self, key):
        self._k = key

    def _next(self):
        self._k, sub = jax.random.split(self._k)
        return sub

    def normal(self, shape):
        return jax.random.normal(self._next(), shape, dtype=jnp.bfloat16)

    def randint(self, lo, hi, shape):
        return jax.random.randint(self._next(), shape, lo, hi, dtype=jnp.int32)

    def uniform(self, shape, lo=0.0, hi=1.0):
        return jax.random.uniform(self._next(), shape, jnp.bfloat16, lo, hi)

    def permutation(self, n):
        return jax.random.permutation(self._next(), n)
kernel_name = 'concat_heads__ssm_conv_h3__memory_aug_infini_attn__prompt'

def setup_inputs():
    _rng = _Rng(jax.random.key(int.from_bytes(__import__("os").urandom(4), "little")))
    _w = lambda a: (lambda t: t.astype(jnp.bfloat16) if jnp.issubdtype(t.dtype, jnp.floating) else t)(jnp.asarray(a))

    def _A_setup():
        B, S, D = (1, 2048, 640)
        ks = 4
        return {'q': _w((lambda *s: _rng.normal(s) * 0.05)(B, S, D)), 'k': _w((lambda *s: _rng.normal(s) * 0.05)(B, S, D)), 'v': _w((lambda *s: _rng.normal(s) * 0.05)(B, S, D)), 'shift_k': _w((lambda *s: _rng.normal(s) * 0.05)(D, ks) * 0.5), 'ssm_k': _w((lambda *s: _rng.normal(s) * 0.05)(D, S) * (1.0 / S ** 0.5)), 'ssm_D': _w((lambda *s: _rng.normal(s) * 0.05)(D))}
    _A_in = _A_setup()

    def _B_setup():
        B, S, D, H = (1, 2048, 640, 32)
        N = 4
        L = max(1, S // N)
        sc = D ** (-0.5)
        return {'x': _w((lambda *s: _rng.normal(s) * 0.05)(B, N * L, D)), 'wq': _w((lambda *s: _rng.normal(s) * 0.05)(D, D) * sc), 'wk': _w((lambda *s: _rng.normal(s) * 0.05)(D, D) * sc), 'wv': _w((lambda *s: _rng.normal(s) * 0.05)(D, D) * sc), 'wo': _w((lambda *s: _rng.normal(s) * 0.05)(D, D) * sc), 'beta': _w((lambda *s: _rng.normal(s) * 0.05)(H))}
    _B_in = _B_setup()
    return {'A_q': _A_in['q'], 'A_k': _A_in['k'], 'A_v': _A_in['v'], 'A_shift_k': _A_in['shift_k'], 'A_ssm_k': _A_in['ssm_k'], 'A_ssm_D': _A_in['ssm_D'], 'B_x': _B_in['x'], 'B_wq': _B_in['wq'], 'B_wk': _B_in['wk'], 'B_wv': _B_in['wv'], 'B_wo': _B_in['wo'], 'B_beta': _B_in['beta']}

def reference(A_q, A_k, A_v, A_shift_k, A_ssm_k, A_ssm_D, B_x, B_wq, B_wk, B_wv, B_wo, B_beta):

    def _A_ref(q, k, v, shift_k, ssm_k, ssm_D):
        B, S, D = q.shape
        ks = shift_k.shape[-1]
        k_pad = jnp.pad(k, ((0, 0), (ks - 1, 0), (0, 0)))
        k_shift = jnp.zeros_like(k)
        for t in range(ks):
            k_shift = k_shift + k_pad[:, t:t + S, :] * shift_k[:, ks - 1 - t][None, None, :]
        kv = k_shift * v
        L = 2 * S
        kv_pad = jnp.pad(kv, ((0, 0), (0, S), (0, 0)))
        kf_pad = jnp.pad(ssm_k, ((0, 0), (0, S)))
        kv_f = (lambda x, axes=(-2, -1): jnp.fft.rfft2(x.astype(jnp.float32), axes=axes))(kv_pad[:, None, :, :], axes=(1, 2))
        kf_f = (lambda x, axes=(-2, -1): jnp.fft.rfft2(x.astype(jnp.float32), axes=axes))(kf_pad[:, None, :], axes=(1, 2))
        kf_f = (lambda x, *d: x.transpose(*d))(kf_f, 1, 2, 0)
        y_f = kv_f * kf_f[None, :, :, :]
        y = (lambda x, s, axes=(-2, -1): jnp.fft.irfft2(x, s=s, axes=axes).astype(jnp.bfloat16))(y_f, (1, L), axes=(1, 2))[:, 0, :S, :]
        y = y + kv * ssm_D[None, None, :]
        return q * y

    def _B_ref(x, wq, wk, wv, wo, beta):
        B, S, D = x.shape
        H = 32
        Dh = D // H
        N = 4
        L = S // N
        q = (lambda x, *d: x.transpose(*d))((x @ wq).reshape(B, S, H, Dh), 0, 2, 1, 3).reshape(B, H, N, L, Dh)
        k = (lambda x, *d: x.transpose(*d))((x @ wk).reshape(B, S, H, Dh), 0, 2, 1, 3).reshape(B, H, N, L, Dh)
        v = (lambda x, *d: x.transpose(*d))((x @ wv).reshape(B, S, H, Dh), 0, 2, 1, 3).reshape(B, H, N, L, Dh)
        phi = lambda t: jnp.where(t > 0, t + 1.0, jnp.exp(t))
        scale = Dh ** (-0.5)
        ar = jnp.arange(L)
        mask = (lambda x, dt: x.astype(dt))(ar[:, None] < ar[None, :], x.dtype) * -1000000000.0
        g = _sigmoid(beta).reshape(1, H, 1, 1)
        M = jnp.einsum('bhd,bhe->bhde', q[:, :, 0, 0, :] * 0.0, q[:, :, 0, 0, :] * 0.0)
        z = q[:, :, 0, 0, :] * 0.0
        outs = []
        for s in range(N):
            qs, ks, vs = (q[:, :, s].copy(), k[:, :, s].copy(), v[:, :, s].copy())
            logits = jnp.einsum('bhqd,bhkd->bhqk', qs, ks) * scale + mask
            p = _softmax(logits, axis=-1)
            a_dot = jnp.einsum('bhqk,bhkd->bhqd', p, vs)
            pq = phi(qs)
            num = jnp.einsum('bhld,bhde->bhle', pq, M)
            den = jnp.einsum('bhld,bhd->bhl', pq, z)[..., None] + 1e-06
            a_mem = num / den
            o = g * a_mem + (1.0 - g) * a_dot
            outs.append(o)
            pk = phi(ks)
            M = M + jnp.einsum('bhld,bhle->bhde', pk, vs)
            z = z + jnp.einsum('bhld->bhd', pk)
        o = (lambda x, *d: x.transpose(*d))(jnp.stack(outs, 2).reshape(B, H, S, Dh), 0, 2, 1, 3).reshape(B, S, D)
        return o @ wo
    a = _A_ref(A_q, A_k, A_v, A_shift_k, A_ssm_k, A_ssm_D)
    b = _B_ref(B_x, B_wq, B_wk, B_wv, B_wo, B_beta)
    return jnp.concatenate([a, b], axis=-1)
```

```python
import math

import jax
import jax.numpy as jnp
import numpy as np
from jax import lax
from jax.experimental import pallas as pl
from jax.experimental.pallas import tpu as pltpu

S = 2048
D = 640
H = 32
DH = D // H
NSEG = 4
L = S // NSEG
KS = 4
T = 128
NCH = S // T
NSLAB = D // T
GH = 4
GR = GH * DH
NGRP = H // GH
OB = 512
LOG2E = math.log2(math.e)
NEG = -1e30

F32 = jnp.float32
BF16 = jnp.bfloat16


def _dft_matrices():
    k = np.arange(T, dtype=np.float64)[:, None]
    t = np.arange(T, dtype=np.float64)[None, :]
    theta = 2.0 * np.pi * (k + 0.25) * t / T
    re = np.cos(theta).reshape(T // 8, 1, 8, T)
    im = np.sin(theta).reshape(T // 8, 1, 8, T)
    fwd = np.concatenate([re, im], axis=1).reshape(2 * T, T)
    inv = fwd.T / T
    return fwd.astype(np.float32), inv.astype(np.float32)


_FWD, _INV = _dft_matrices()


def _dot(a, b):
    return jnp.dot(a, b, preferred_element_type=F32)


def _dot_nt(a, b):
    return lax.dot_general(a, b, (((1,), (1,)), ((), ())), preferred_element_type=F32)


def _phi(t):
    return jnp.where(t > 0, t + 1.0, jnp.exp(t))


def _tree_sum(xs):
    acc = xs[0]
    for x in xs[1:]:
        acc = acc + x
    return acc


def _causal_products(u, h):
    return [_tree_sum([u[j] * h[a - j] for j in range(a + 1)]) for a in range(len(u))]


def _kernel(
    q_hbm, k_hbm, v_hbm, shift_hbm, h_hbm, d_hbm, x_hbm, wq_hbm, wk_hbm, wv_hbm,
    wo_hbm, beta_hbm, fwd_hbm, inv_hbm,
    out_hbm,
    q_v, k_v, v_v, shift_v, h_v, d_v, x_v, w_v, wo_v, beta_v, fwd_v, inv_v,
    wt_s, taps_s, gate_s, kpad_s, kv_s, uf_s, hf_s, yf_s, ya_s,
    qs_s, pq_s, kt_s, pk_s, vt_s, ot_s, yb_s,
    in_sem, slab_sem, outa_sem, outb_sem,
):
    def slab_copies(c):
        col = pl.ds(pl.multiple_of(c * T, T), T)
        return (
            pltpu.make_async_copy(k_hbm.at[:, col], k_v.at[c], slab_sem.at[0, c]),
            pltpu.make_async_copy(v_hbm.at[:, col], v_v.at[c], slab_sem.at[1, c]),
            pltpu.make_async_copy(h_hbm.at[col, :], h_v.at[c], slab_sem.at[2, c]),
            pltpu.make_async_copy(q_hbm.at[:, col], q_v.at[c], slab_sem.at[3, c]),
        )

    def outa_copy(c):
        col = pl.ds(pl.multiple_of(c * T, T), T)
        return pltpu.make_async_copy(ya_s.at[c], out_hbm.at[:, col], outa_sem.at[c])

    def outb_copy(b):
        row = pl.ds(pl.multiple_of(b * OB, OB), OB)
        return pltpu.make_async_copy(
            yb_s.at[b], out_hbm.at[row, pl.ds(D, D)], outb_sem.at[b])

    whole = [
        (wq_hbm, w_v.at[0]), (wk_hbm, w_v.at[1]), (wv_hbm, w_v.at[2]),
        (x_hbm, x_v), (shift_hbm, shift_v), (d_hbm, d_v), (beta_hbm, beta_v),
        (fwd_hbm, fwd_v), (inv_hbm, inv_v), (wo_hbm, wo_v),
    ]
    cps = [pltpu.make_async_copy(a, b, in_sem.at[i]) for i, (a, b) in enumerate(whole)]
    for cp in cps[:-1]:
        cp.start()
    for cp in slab_copies(0):
        cp.start()

    for i in range(3):
        cps[i].wait()
        for c in range(NSLAB):
            for j in range(NSLAB):
                tile = w_v[i, j * T:(j + 1) * T, c * T:(c + 1) * T]
                wt_s[c, i * T:(i + 1) * T, j * T:(j + 1) * T] = tile.T
    for cp in cps[4:-1]:
        cp.wait()

    pick = (lax.broadcasted_iota(jnp.int32, (8, KS), 0)
            == lax.broadcasted_iota(jnp.int32, (8, KS), 1)).astype(BF16)
    d_row = d_v[...].astype(F32)
    sub8 = lax.broadcasted_iota(jnp.int32, (8, T), 0)
    for c in range(NSLAB):
        taps = _dot_nt(pick, shift_v[c * T:(c + 1) * T, :])
        taps_s[c] = jnp.where(sub8 == KS, d_row[:, c * T:(c + 1) * T], taps)

    g_row = jax.nn.sigmoid(beta_v[...].astype(F32))
    row = lax.broadcasted_iota(jnp.int32, (D, H), 0)
    head = lax.broadcasted_iota(jnp.int32, (D, H), 1)
    own = (row >= head * DH) & (row < (head + 1) * DH)
    g_col = jnp.sum(jnp.where(own, g_row, 0.0), axis=1, keepdims=True)
    gate_s[...] = jnp.broadcast_to(g_col, (D, T))

    kpad_s[0:8, :] = jnp.zeros((8, T), F32)
    cps[3].wait()
    cps[-1].start()

    q_scale = (DH ** -0.5) * LOG2E

    def phase1(c, carry):
        @pl.when(c + 1 < NSLAB)
        def _():
            for cp in slab_copies(c + 1):
                cp.start()

        for cp in slab_copies(c):
            cp.wait()

        taps = taps_s[c]
        kpad_s[8:, :] = k_v[c].astype(F32)
        for a in range(NCH):
            acc = None
            for j in range(KS):
                term = kpad_s[8 + a * T - j:8 + (a + 1) * T - j, :] * taps[j:j + 1, :]
                acc = term if acc is None else acc + term
            kv = acc * v_v[c, a * T:(a + 1) * T, :].astype(F32)
            kv_s[:, a * T:(a + 1) * T] = kv.astype(BF16)

        fwd = fwd_v[...]
        h_rows = jnp.concatenate(
            [h_v[c, :, a * T:(a + 1) * T] for a in range(NCH)], axis=0)
        hf_s[...] = _dot_nt(fwd, h_rows)
        uf_s[...] = _dot(fwd, kv_s[...])

        frow = pl.ds(pl.multiple_of(c * T, T), T)

        def project(b):
            tcol = slice(b * L, (b + 1) * L)
            r = _dot_nt(wt_s[c], x_v[tcol, :])
            qf, kf, vf = r[0:T], r[T:2 * T], r[2 * T:3 * T]
            qs_s[frow, tcol] = (qf * q_scale).astype(BF16)
            kb = kf.astype(BF16)
            kt_s[frow, tcol] = kb
            vt_s[frow, tcol] = vf.astype(BF16)
            if b > 0:
                pq_s[frow, (b - 1) * L:b * L] = _phi(
                    qf.astype(BF16).astype(F32)).astype(BF16)
            if b < NSEG - 1:
                pk_s[frow, tcol] = _phi(kb.astype(F32)).astype(BF16)

        def chunk_conv(f):
            re = slice(16 * f, 16 * f + 8)
            im = slice(16 * f + 8, 16 * f + 16)
            col = lambda a: slice(a * T, (a + 1) * T)
            ur = [uf_s[re, col(a)] for a in range(NCH)]
            ui = [uf_s[im, col(a)] for a in range(NCH)]
            hr = [hf_s[re, col(a)] for a in range(NCH)]
            hi = [hf_s[im, col(a)] for a in range(NCH)]
            gr = [hr[0]] + [hr[a] + hi[a - 1] for a in range(1, NCH)]
            gi = [hi[0]] + [hi[a] - hr[a - 1] for a in range(1, NCH)]
            k1 = _causal_products([x + y for x, y in zip(ur, ui)], gr)
            k2 = _causal_products(ur, [y - x for x, y in zip(gr, gi)])
            k3 = _causal_products(ui, [x + y for x, y in zip(gr, gi)])
            for a in range(NCH):
                y = jnp.concatenate([k1[a] - k3[a], k1[a] + k2[a]], axis=0)
                yf_s[16 * f:16 * f + 16, col(a)] = y.astype(BF16)

        per = (T // 8) // NSEG
        for b in range(NSEG):
            project(b)
            for f in range(b * per, (b + 1) * per):
                chunk_conv(f)

        y = _dot(inv_v[...], yf_s[...])
        for a in range(NCH):
            rows = slice(a * T, (a + 1) * T)
            kv = kv_s[:, rows].astype(F32)
            ya = y[:, rows] + kv * taps[KS:KS + 1, :]
            ya_s[c, rows, :] = (q_v[c, rows, :].astype(F32) * ya).astype(BF16)
        outa_copy(c).start()
        return carry

    lax.fori_loop(0, NSLAB, phase1, 0)

    def phase2(g, carry):
        rows = pl.ds(pl.multiple_of(g * GR, 16), GR)
        r16 = lax.broadcasted_iota(jnp.int32, (16, L), 0)
        r32 = lax.broadcasted_iota(jnp.int32, (32, T), 0)
        lane = lax.broadcasted_iota(jnp.int32, (32, T), 1)
        low4 = lax.broadcasted_iota(jnp.int32, (8, T), 0) < 4
        causal = (lax.broadcasted_iota(jnp.int32, (T, T), 0)
                  <= lax.broadcasted_iota(jnp.int32, (T, T), 1))
        gate = gate_s[rows, :]
        ones = jnp.ones((16, L), BF16)
        mem = None

        def assemble(parts):
            u = [[p[8 * n:8 * n + 8] for n in range(4)] for p in parts]
            vals = [u[0][0], u[0][1], jnp.where(low4, u[0][2], u[1][0]), u[1][1], u[1][2],
                    u[2][1], u[2][2], jnp.where(low4, u[2][3], u[3][1]), u[3][2], u[3][3]]
            return jnp.concatenate(vals, axis=0), (u[0][3], u[1][3], u[2][0], u[3][0])

        def spread(d):
            return jnp.concatenate(
                [d[0], d[0], jnp.where(low4, d[0], d[1]), d[1], d[1],
                 d[2], d[2], jnp.where(low4, d[2], d[3]), d[3], d[3]], axis=0)

        for s in range(NSEG):
            tcol = slice(s * L, (s + 1) * L)
            kt = jnp.concatenate([kt_s[rows, tcol], jnp.zeros((T - GR, L), BF16)], axis=0)
            kn = kt.T
            vt = vt_s[rows, tcol]
            b = [vt[16 * n:16 * n + 16] for n in range(5)]
            first = r16 < 8
            vaug = [
                jnp.concatenate([b[0], jnp.where(first, b[1], ones)], axis=0),
                jnp.concatenate([b[1], jnp.where(first, b[2], ones)], axis=0),
                jnp.concatenate([jnp.where(first, ones, b[2]), b[3]], axis=0),
                jnp.concatenate([jnp.where(first, ones, b[3]), b[4]], axis=0),
            ]
            qt = qs_s[rows, tcol]
            wq = []
            for h in range(GH):
                lo = h * DH - 16 * h
                keep = (r32 >= lo) & (r32 < lo + DH)
                parts = []
                for i in range(NSEG):
                    blk = jnp.where(keep, qt[16 * h:16 * h + 32, i * T:(i + 1) * T],
                                    jnp.zeros((32, T), BF16))
                    pieces = [blk, jnp.zeros((T - 32 - 16 * h, T), BF16)]
                    if h:
                        pieces = [jnp.zeros((16 * h, T), BF16)] + pieces
                    parts.append(jnp.concatenate(pieces, axis=0))
                wq.append(parts)

            if s > 0:
                pq = jnp.concatenate(
                    [pq_s[rows, (s - 1) * L:s * L], jnp.zeros((T - GR, L), BF16)], axis=0)
                ret = _dot(mem.astype(BF16), pq)

            for i in range(NSEG):
                nk = (i + 1) * T
                st = _dot(kn[:nk], jnp.concatenate([wq[h][i] for h in range(GH)], axis=1))
                pv = []
                for h in range(GH):
                    sc = st[:, h * T:(h + 1) * T]
                    diag = jnp.where(causal, sc[nk - T:], NEG)
                    sc = diag if i == 0 else jnp.concatenate([sc[:nk - T], diag], axis=0)
                    m = jnp.max(sc, axis=0, keepdims=True)
                    p = jnp.exp2(sc - m).astype(BF16)
                    pv.append(_dot(vaug[h][:, :nk], p))
                vals, dens = assemble(pv)
                o = vals * ((1.0 - gate) * spread([1.0 / d for d in dens]))
                if s > 0:
                    vals, dens = assemble(
                        [ret[32 * h:32 * h + 32, i * T:(i + 1) * T] for h in range(GH)])
                    o = o + vals * (gate * spread([1.0 / (d + 1e-6) for d in dens]))
                ot_s[rows, s * L + i * T:s * L + (i + 1) * T] = o.astype(BF16)

            if s < NSEG - 1:
                pk = jnp.concatenate(
                    [pk_s[rows, tcol], jnp.zeros((T - GR, L), BF16)], axis=0)
                upd = _dot_nt(jnp.concatenate(vaug, axis=0), pk)
                upd = jnp.concatenate([
                    jnp.where((lane >= h * DH) & (lane < (h + 1) * DH),
                              upd[32 * h:32 * h + 32], 0.0)
                    for h in range(GH)], axis=0)
                mem = upd if mem is None else mem + upd
        return carry

    lax.fori_loop(0, NGRP, phase2, 0)

    cps[-1].wait()

    def phase3(b, carry):
        tcol = pl.ds(pl.multiple_of(b * OB, OB), OB)
        o = ot_s[:, tcol].T
        yb_s[b] = _dot(o, wo_v[...]).astype(BF16)
        outb_copy(b).start()
        return carry

    lax.fori_loop(0, S // OB, phase3, 0)

    for c in range(NSLAB):
        outa_copy(c).wait()
    for b in range(S // OB):
        outb_copy(b).wait()


@jax.jit
def pallas_concat_heads__ssm_conv_h3__memory_aug_infini_attn__prompt_kernel(
    A_q: jax.Array,
    A_k: jax.Array,
    A_v: jax.Array,
    A_shift_k: jax.Array,
    A_ssm_k: jax.Array,
    A_ssm_D: jax.Array,
    B_x: jax.Array,
    B_wq: jax.Array,
    B_wk: jax.Array,
    B_wv: jax.Array,
    B_wo: jax.Array,
    B_beta: jax.Array,
):
    hbm = pl.BlockSpec(memory_space=pltpu.MemorySpace.HBM)
    vmem = pltpu.VMEM
    dma = pltpu.SemaphoreType.DMA
    out = pl.pallas_call(
        _kernel,
        out_shape=jax.ShapeDtypeStruct((S, 2 * D), BF16),
        in_specs=[hbm] * 14,
        out_specs=hbm,
        scratch_shapes=[
            vmem((NSLAB, S, T), BF16),
            vmem((NSLAB, S, T), BF16),
            vmem((NSLAB, S, T), BF16),
            vmem((D, KS), BF16),
            vmem((NSLAB, T, S), BF16),
            vmem((1, D), BF16),
            vmem((S, D), BF16),
            vmem((3, D, D), BF16),
            vmem((D, D), BF16),
            vmem((1, H), BF16),
            vmem((2 * T, T), BF16),
            vmem((T, 2 * T), BF16),
            vmem((NSLAB, 3 * T, D), BF16),
            vmem((NSLAB, 8, T), F32),
            vmem((D, T), F32),
            vmem((S + 8, T), F32),
            vmem((T, S), BF16),
            vmem((2 * T, S), F32),
            vmem((2 * T, S), F32),
            vmem((2 * T, S), BF16),
            vmem((NSLAB, S, T), BF16),
            vmem((D, S), BF16),
            vmem((D, S - L), BF16),
            vmem((D, S), BF16),
            vmem((D, S - L), BF16),
            vmem((D, S), BF16),
            vmem((D, S), BF16),
            vmem((S // OB, OB, D), BF16),
            dma((10,)),
            dma((4, NSLAB)),
            dma((NSLAB,)),
            dma((S // OB,)),
        ],
        compiler_params=pltpu.CompilerParams(vmem_limit_bytes=100 * 1024 * 1024),
        name="h3_infini_concat",
    )(
        A_q.reshape(S, D), A_k.reshape(S, D), A_v.reshape(S, D), A_shift_k, A_ssm_k,
        A_ssm_D.reshape(1, D), B_x.reshape(S, D), B_wq, B_wk, B_wv, B_wo,
        B_beta.reshape(1, H),
        jnp.asarray(_FWD, dtype=BF16), jnp.asarray(_INV, dtype=BF16),
    )
    return out.reshape(1, S, 2 * D)
```

```python
import math

import jax
import jax.numpy as jnp
import numpy as np
from jax import lax
from jax.experimental import pallas as pl
from jax.experimental.pallas import tpu as pltpu

CFG = dict(lag=4, lag2=6, nc=8, rs=8, rp=4, orders=['0123'] * 4, pn=512,
           p1seq='hvvvvkkcvvvvkcvvvvkcvvvvpiu', p1last='vvvvvcvvvvvcvvvvvvpip', peel=1, conv='reg', yspec=0, gateh=0, only='', hmajor=1,
           memat=2, updat=6, ob=512, p3tail=1)

S = 2048
D = 640
H = 32
DH = D // H
NSEG = 4
L = S // NSEG
KS = 4
T = 128
NT = S // T
ND = D // T
GH = 4
GR = GH * DH
NGRP = H // GH
OB = CFG['ob']
LOG2E = math.log2(math.e)
NEG = -1e30

F32 = jnp.float32
BF16 = jnp.bfloat16

SP_H, SP_U, SP_Y, SP_T, SP_PACE = 0, 2 * T, 4 * T, 4 * T, 4 * T + 32


def _dft_matrices():
    k = np.arange(T, dtype=np.float64)[:, None]
    t = np.arange(T, dtype=np.float64)[None, :]
    theta = 2.0 * np.pi * (k + 0.25) * t / T
    re = np.cos(theta).reshape(T // 8, 1, 8, T)
    im = np.sin(theta).reshape(T // 8, 1, 8, T)
    fwd = np.concatenate([re, im], axis=1).reshape(2 * T, T)
    inv = fwd.T / T
    return fwd.astype(np.float32), inv.astype(np.float32)


_FWD, _INV = _dft_matrices()


def _dot(a, b):
    return jnp.dot(a, b, preferred_element_type=F32)


def _dot_nt(a, b):
    return lax.dot_general(a, b, (((1,), (1,)), ((), ())), preferred_element_type=F32)


def _phi(t):
    return jnp.where(t > 0, t + 1.0, jnp.exp(t))


def _causal_products(u, h):
    out = []
    for a in range(len(u)):
        acc = u[0] * h[a]
        for j in range(1, a + 1):
            acc = acc + u[j] * h[a - j]
        out.append(acc)
    return out


def _kernel(
    zero_ref, q_hbm, k_hbm, v_hbm, shift_hbm, h_hbm, d_hbm, x_hbm, wq_hbm, wk_hbm, wv_hbm,
    wo_hbm, beta_hbm, fwd_hbm, inv_hbm,
    out_hbm,
    q_v, k_v, v_v, shift_v, h_v, d_v, x_v, w_v, wo_v, beta_v, fwd_v, inv_v,
    wt_s, taps_s, gate_s, kpad_s, kv_s, spec_s, yf_s, ya_s,
    qs_s, pq_s, kt_s, pk_s, vt_s, ot_s, yb_s, s_ref, kn0_s,
    in_sem, slab_sem, outa_sem, outb_sem, *p_refs,
):
    RS, RP = CFG['rs'], CFG['rp']

    def tile(i):
        return slice(i * T, (i + 1) * T)

    def slab_cols(c):
        return pl.ds(c * T if isinstance(c, int) else pl.multiple_of(c * T, T), T)

    def kvh_copies(c):
        col = slab_cols(c)
        return (
            pltpu.make_async_copy(k_hbm.at[:, col], k_v.at[c], slab_sem.at[0, c]),
            pltpu.make_async_copy(v_hbm.at[:, col], v_v.at[c], slab_sem.at[1, c]),
            pltpu.make_async_copy(h_hbm.at[col, :], h_v.at[c], slab_sem.at[2, c]),
        )

    def q_copy(c):
        return pltpu.make_async_copy(q_hbm.at[:, slab_cols(c)], q_v.at[c], slab_sem.at[3, c])

    def outa_copy(c):
        return pltpu.make_async_copy(ya_s.at[c], out_hbm.at[:, slab_cols(c)], outa_sem.at[c])

    def outb_copy(b):
        row = pl.ds(b * OB if isinstance(b, int) else pl.multiple_of(b * OB, OB), OB)
        return pltpu.make_async_copy(
            yb_s.at[b], out_hbm.at[row, pl.ds(D, D)], outb_sem.at[b])

    whole = [
        (wq_hbm, w_v.at[0]), (wk_hbm, w_v.at[1]), (wv_hbm, w_v.at[2]),
        (x_hbm, x_v), (shift_hbm, shift_v), (d_hbm, d_v), (beta_hbm, beta_v),
        (fwd_hbm, yf_s.at[NT]), (inv_hbm, inv_v), (wo_hbm, wo_v),
    ]
    cps = [pltpu.make_async_copy(a, b, in_sem.at[i]) for i, (a, b) in enumerate(whole)]
    for cp in cps[4:-1]:
        cp.start()
    for cp in kvh_copies(0):
        cp.start()
    for cp in cps[:3]:
        cp.start()

    kpad_s[0:8, :] = jnp.zeros((8, T), F32)
    s_ref[...] = jnp.zeros(s_ref.shape, F32)
    for p in p_refs:
        p[...] = jnp.zeros(p.shape, BF16)
    for cp in cps[4:-1]:
        cp.wait()

    taps_s[0:KS, :] = shift_v[...].astype(F32)
    taps_s[KS:KS + 1, :] = d_v[...].astype(F32)

    g_row = jax.nn.sigmoid(beta_v[...].astype(F32))
    row = lax.broadcasted_iota(jnp.int32, (D, H), 0)
    head = lax.broadcasted_iota(jnp.int32, (D, H), 1)
    own = (row >= head * DH) & (row < (head + 1) * DH)
    g_col = jnp.sum(jnp.where(own, g_row, 0.0), axis=1, keepdims=True)
    gate_s[...] = jnp.broadcast_to(g_col, (D, T))

    def tap(c, j):
        return taps_s[j:j + 1, slab_cols(c)]

    def kv_prep(c, a0=0, a1=NT):
        kpad_s[8 + a0 * T:8 + a1 * T, :] = k_v[c, a0 * T:a1 * T, :].astype(F32)
        w = [tap(c, j) for j in range(KS)]
        for a in range(a0, a1):
            acc = None
            for j in range(KS):
                term = kpad_s[8 + a * T - j:8 + (a + 1) * T - j, :] * w[j]
                acc = term if acc is None else acc + term
            kv = acc * v_v[c, tile(a), :].astype(F32)
            kv_s[tile(a), :] = kv.astype(BF16)
        return kv[T - 8:]

    def spec_base(rd, wr):
        return [pl.multiple_of(zero_ref[n], 8) for n in range(2)] + [zero_ref[2], zero_ref[3], rd * NT, wr * NT]

    def store_spec(z, off, val):
        for a in range(NT):
            spec_s[z[5] + a, pl.ds(z[0] + off, 2 * T), :] = val[:, tile(a)]

    def fwd_h(c, z):
        h_rows = jnp.concatenate([h_v[c, :, tile(a)] for a in range(NT)], axis=0)
        store_spec(z, SP_H, _dot_nt(yf_s[z[3] + NT if CFG['gateh'] & 1 else NT], h_rows))

    def fwd_u(z):
        u = jnp.concatenate([kv_s[tile(a), :] for a in range(NT)], axis=1)
        store_spec(z, SP_U, _dot(yf_s[z[3] + NT if CFG['gateh'] & 2 else NT], u))

    def chunk_conv(c, z, f):
        def ld(off):
            return [spec_s[z[4] + a, pl.ds(z[1] + off, 8), :] for a in range(NT)]

        def st(off, vals):
            for a in range(NT):
                spec_s[a, pl.ds(z[0] + off, 8), :] = vals[a]

        hr, hi = ld(SP_H + 16 * f), ld(SP_H + 16 * f + 8)
        hr[0] = hr[0] + tap(c, KS)
        gr = [hr[0]] + [hr[a] + hi[a - 1] for a in range(1, NT)]
        gi = [hi[0]] + [hi[a] - hr[a - 1] for a in range(1, NT)]
        gd = [y - x for x, y in zip(gr, gi)]
        gs = [x + y for x, y in zip(gr, gi)]
        if CFG['conv'] == 'store':
            st(SP_T, gd)
            st(SP_T + 8, gs)
        ur, ui = ld(SP_U + 16 * f), ld(SP_U + 16 * f + 8)
        k1 = _causal_products([x + y for x, y in zip(ur, ui)], gr)
        if CFG['conv'] == 'store':
            st(SP_T + 16, k1)
            k2 = _causal_products(ld(SP_U + 16 * f), ld(SP_T))
            im = [x + y for x, y in zip(ld(SP_T + 16), k2)]
            st(SP_T + 24, im)
            k3 = _causal_products(ld(SP_U + 16 * f + 8), ld(SP_T + 8))
            re = [x - y for x, y in zip(ld(SP_T + 16), k3)]
            im = ld(SP_T + 24)
        else:
            k2 = _causal_products(ur, gd)
            k3 = _causal_products(ui, gs)
            re = [x - y for x, y in zip(k1, k3)]
            im = [x + y for x, y in zip(k1, k2)]
        if CFG['yspec']:
            st(SP_Y + 16 * f, re)
            st(SP_Y + 16 * f + 8, im)
        else:
            for a in range(NT):
                yf_s[z[2] + a if CFG['gateh'] else a, 16 * f:16 * f + 16, :] = jnp.concatenate(
                    [re[a], im[a]], axis=0).astype(BF16)

    def inverse(c, z):
        if CFG['yspec']:
            ys = [spec_s[a, pl.ds(z[1] + SP_Y, 2 * T), :].astype(BF16) for a in range(NT)]
        else:
            ys = [yf_s[a] for a in range(NT)]
        y = _dot(inv_v[...], jnp.concatenate(ys, axis=1))
        for a in range(NT):
            ya_s[c, tile(a), :] = (
                q_v[c, tile(a), :].astype(F32) * y[:, tile(a)]).astype(BF16)

    q_scale = (DH ** -0.5) * LOG2E
    PN = CFG['pn']

    def project(c, b):
        frow = slab_cols(c)
        w = jnp.concatenate([wt_s[c, j] for j in range(ND)], axis=1)
        r = _dot_nt(w, x_v[b * PN:(b + 1) * PN, :])
        for n in range(PN // T):
            a = b * (PN // T) + n
            qf, kf, vf = r[0:T, tile(n)], r[T:2 * T, tile(n)], r[2 * T:3 * T, tile(n)]
            qs_s[a, frow, :] = (qf * q_scale).astype(BF16)
            kb = kf.astype(BF16)
            kt_s[a, frow, :] = kb
            vt_s[a, frow, :] = vf.astype(BF16)
            if a * T >= L:
                pq_s[a - L // T, frow, :] = _phi(qf.astype(BF16).astype(F32)).astype(BF16)
            if a * T < S - L:
                pk_s[a, frow, :] = _phi(kb.astype(F32)).astype(BF16)
        return r

    for cp in kvh_copies(0):
        cp.wait()
    cps[3].start()
    q_copy(0).start()
    for cp in kvh_copies(1):
        cp.start()
    z = spec_base(1, 0)
    fwd_h(0, z)
    kv_prep(0)
    fwd_u(z)

    for i in range(3):
        cps[i].wait()
        for c in range(ND):
            for j in range(ND):
                wt_s[c, j, tile(i), :] = w_v[i, tile(j), tile(c)].T
    cps[3].wait()
    cps[-1].start()

    def phase1(c, seq):
        more = 'h' in seq
        if more:
            @pl.when(c + 2 < ND)
            def _():
                for cp in kvh_copies(c + 2):
                    cp.start()
            q_copy(c + 1).start()
            for cp in kvh_copies(c + 1):
                cp.wait()
        q_copy(c).wait()
        z = spec_base(c % 2, (c + 1) % 2)
        nk = CFG['p1seq'].count('k') + CFG['p1seq'].count('K')
        if more and nk == 0:
            kv_prep(c + 1)
        nb = nf = ik = 0
        for ch in seq:
            if ch == 'h':
                fwd_h(c + 1, z)
            elif ch == 'u':
                fwd_u(z)
            elif ch == 'i':
                assert nf == NT
                inverse(c, z)
            elif ch == 'p':
                project(c, nb)
                nb += 1
            elif ch == 'c':
                r = project(c, nb)
                spec_s[0, pl.ds(z[0] + SP_PACE, 8), :] = r[3 * T - 8:, 0:T]
                nb += 1
            elif ch in 'kK':
                last = kv_prep(c + 1, ik * NT // nk, (ik + 1) * NT // nk)
                if ch == 'k':
                    spec_s[0, pl.ds(z[0] + SP_PACE, 8), :] = last
                ik += 1
            elif ch == 'v':
                chunk_conv(c, z, nf)
                nf += 1
        assert nb * PN == S
        outa_copy(c).start()

    if CFG['only'] == 'p2':
        for c in range(ND):
            outa_copy(c).start()
    else:
        def body1(c, carry):
            phase1(c, CFG['p1seq'])
            return carry
        lax.fori_loop(0, ND - 1, body1, 0)
        phase1(ND - 1, CFG['p1last'])

    steps = [(s, int(i), j) for s in range(NSEG) for i in CFG['orders'][s]
             for j in range(int(i) + 1)]
    n = len(steps)
    per_seg = n // NSEG
    first = [t for t in range(n) if steps[t][2] == 0]
    if CFG['hmajor']:
        cells = [(t0 + j, h) for t0 in first for h in range(GH) for j in range(steps[t0][1] + 1)]
    else:
        cells = [(t, h) for t in range(n) for h in range(GH)]
    lag, lag2, nc = CFG['lag'], CFG['lag2'], CFG['nc']
    tpl = L // T
    def cell(m):
        t, h = cells[m]
        return steps[t] + (h,)

    max_keys = sorted({cell(m)[:2] for m in range((n - lag) * GH, n * GH)})
    late = [cell(m) for m in range((n - lag2) * GH, n * GH)]
    early = [cell(m) for m in range((n - lag2) * GH)]
    done_late = {(s, i) for s, i, j, h in late}
    acc_keys = sorted({(s, i, h) for s, i, j, h in early if (s, i) in done_late})
    ret_keys = sorted(k for k in done_late if k[0] > 0)

    class Group:
        def __init__(self, g):
            self.g = g
            self.r0 = g * GR if isinstance(g, int) else pl.multiple_of(g * GR, 16)
            self.rows = pl.ds(self.r0, GR)
            self.kn, self.va, self.w = {}, {}, {}
            self.maxes, self.accs, self.rets, self.mems = {}, {}, {}, {}

    r16 = lambda: lax.broadcasted_iota(jnp.int32, (16, T), 0)
    low4 = lambda: lax.broadcasted_iota(jnp.int32, (8, T), 0) < 4

    def pad_rows(x):
        return jnp.concatenate([x, jnp.zeros((T - GR, x.shape[1]), x.dtype)], axis=0)

    def keys(G, a):
        if a not in G.kn:
            G.kn[a] = pad_rows(kt_s[a, G.rows, :]).T
        return G.kn[a]

    def values(G, a):
        if a not in G.va:
            vt = vt_s[a, G.rows, :]
            b = [vt[16 * m:16 * m + 16] for m in range(5)]
            lo = low4()
            one2 = jnp.full((8, T), 0x3F803F80, jnp.uint32)

            def top(x):
                return pltpu.bitcast(jnp.where(lo, pltpu.bitcast(x, jnp.uint32), one2), BF16)

            def bottom(x):
                return pltpu.bitcast(jnp.where(lo, one2, pltpu.bitcast(x, jnp.uint32)), BF16)

            G.va[a] = [
                jnp.concatenate([b[0], top(b[1])], axis=0),
                jnp.concatenate([b[1], top(b[2])], axis=0),
                jnp.concatenate([bottom(b[2]), b[3]], axis=0),
                jnp.concatenate([bottom(b[3]), b[4]], axis=0),
            ]
        return G.va[a]

    def queries(G, a):
        if a not in G.w:
            r16 = lax.broadcasted_iota(jnp.int32, (16, T), 0)
            ws = []
            for h in range(GH):
                lo = (h * DH - 16 * h) // 2
                keep = (r16 >= lo) & (r16 < lo + DH // 2)
                blk = pltpu.bitcast(qs_s[a, pl.ds(G.r0 + 16 * h, 32), :], jnp.uint32)
                blk = pltpu.bitcast(jnp.where(keep, blk, jnp.zeros_like(blk)), BF16)
                pieces = [blk, jnp.zeros((T - 32 - 16 * h, T), BF16)]
                if h:
                    pieces = [jnp.zeros((16 * h, T), BF16)] + pieces
                ws.append(jnp.concatenate(pieces, axis=0))
            G.w[a] = jnp.concatenate(ws, axis=1)
        return G.w[a]

    def recip(d):
        r = pl.reciprocal(d, approx=True)
        return r * (2.0 - d * r)

    def assemble(parts):
        lo = low4()
        u = [[p[8 * m:8 * m + 8] for m in range(4)] for p in parts]
        vals = [u[0][0], u[0][1], jnp.where(lo, u[0][2], u[1][0]), u[1][1], u[1][2],
                u[2][1], u[2][2], jnp.where(lo, u[2][3], u[3][1]), u[3][2], u[3][3]]
        return jnp.concatenate(vals, axis=0), (u[0][3], u[1][3], u[2][0], u[3][0])

    def spread(d):
        lo = low4()
        return jnp.concatenate(
            [d[0], d[0], jnp.where(lo, d[0], d[1]), d[1], d[1],
             d[2], d[2], jnp.where(lo, d[2], d[3]), d[3], d[3]], axis=0)

    def update(G, s):
        va = jnp.concatenate(
            [jnp.concatenate(values(G, s * tpl + j), axis=0) for j in range(tpl)], axis=1)
        pk = jnp.concatenate(
            [pad_rows(pk_s[s * tpl + j, G.rows, :]) for j in range(tpl)], axis=1)
        upd = _dot_nt(va, pk)
        lane = lax.broadcasted_iota(jnp.int32, (32, T), 1)
        upd = jnp.concatenate([
            jnp.where((lane >= h * DH) & (lane < (h + 1) * DH), upd[32 * h:32 * h + 32], 0.0)
            for h in range(GH)], axis=0)
        G.mems[s + 1] = upd if s == 0 else G.mems[s] + upd

    def retrieve(G, s):
        pq = jnp.concatenate(
            [pad_rows(pq_s[(s - 1) * tpl + i, G.rows, :]) for i in range(tpl)], axis=1)
        ret = _dot(G.mems[s].astype(BF16), pq)
        gate = gate_s[G.rows, :]
        for i in range(tpl):
            vals, dens = assemble([ret[32 * h:32 * h + 32, tile(i)] for h in range(GH)])
            G.rets[(s, i)] = vals * (gate * spread([recip(d + 1e-6) for d in dens]))

    def finish(G, s, i):
        vals, dens = assemble([G.accs[(s, i, h)] for h in range(GH)])
        o = vals * ((1.0 - gate_s[G.rows, :]) * spread([recip(d) for d in dens]))
        if s > 0:
            o = o + G.rets[(s, i)]
        ot_s[s * tpl + i, G.rows, :] = o.astype(BF16)

    def qk_dot(G, t):
        s, i, j = steps[t]
        return _dot(keys(G, s * tpl + j), queries(G, s * tpl + i))

    def qk_store(G, t, raw, c, zs):
        s, i, j = steps[t]
        r0, r1 = c * T // nc, (c + 1) * T // nc
        causal = (r0 + lax.broadcasted_iota(jnp.int32, (r1 - r0, T), 0)
                  <= lax.broadcasted_iota(jnp.int32, (r1 - r0, T), 1))
        ms = []
        for h in range(GH):
            sc = raw[r0:r1, tile(h)]
            if j == i:
                sc = jnp.where(causal, sc, NEG)
            s_ref[pl.ds(zs + ((t % RS) * GH + h) * T + r0, r1 - r0), :] = sc
            m8 = sc[0:8]
            for r in range(1, (r1 - r0) // 8):
                m8 = jnp.maximum(m8, sc[8 * r:8 * r + 8])
            if j > 0 or c > 0:
                m8 = jnp.maximum(G.maxes[(s, i)][h], m8)
            if j == i and c == nc - 1:
                m8 = jnp.broadcast_to(jnp.max(m8, axis=0, keepdims=True), (8, T))
            ms.append(m8)
        G.maxes[(s, i)] = ms

    def exp_part(G, t, c, zl, ps):
        per = GH * T // nc
        slot, r0 = (c * per) // T, (c * per) % T
        tq, h = cells[t * GH + slot]
        s, i, j = steps[tq]
        m = jnp.concatenate([G.maxes[(s, i)][h]] * (per // 8), axis=0)
        sc = s_ref[pl.ds(zl + ((tq % RS) * GH + h) * T + r0, per), :]
        p_refs[t % RP][pl.ds(ps + slot * T + r0, per), :] = jnp.exp2(sc - m).astype(BF16)

    def pv_step(G, t, plo):
        for slot in range(GH):
            s, i, j, h = cell(t * GH + slot)
            r = _dot(values(G, s * tpl + j)[h], p_refs[t % RP][pl.ds(plo + slot * T, T), :])
            G.accs[(s, i, h)] = r if j == 0 else G.accs[(s, i, h)] + r
            if j == i and h == GH - 1:
                finish(G, s, i)

    def attn_base():
        return ([pl.multiple_of(zero_ref[m], 8) for m in range(2)]
                + [pl.multiple_of(zero_ref[m], 16) for m in range(2, 4)])

    def export(G):
        return ([G.maxes[k] for k in max_keys], [G.accs[k] for k in acc_keys],
                [G.rets[k] for k in ret_keys])

    def adopt(g, state):
        G = Group(g)
        G.maxes = dict(zip(max_keys, state[0]))
        G.accs = dict(zip(acc_keys, state[1]))
        G.rets = dict(zip(ret_keys, state[2]))
        return G

    def phase2(g, state):
        zs, zl, ps, plo = attn_base()
        G, P = Group(g), adopt(jnp.maximum(g - 1, 0), state)
        G.kn[0] = kn0_s[...]
        for t in range(n):
            raw = qk_dot(G, t)
            s = t // per_seg
            if t % per_seg == CFG['memat'] and s > 0:
                retrieve(G, s)
            if t % per_seg == CFG['updat'] and s < NSEG - 1:
                update(G, s)
            if t >= lag2:
                pv_step(G, t - lag2, plo)
            else:
                pv_step(P, n + t - lag2, plo)
            for c in range(nc):
                qk_store(G, t, raw, c, zs)
                if t >= lag:
                    exp_part(G, t - lag, c, zl, ps)
                else:
                    exp_part(P, n + t - lag, c, zl, ps)
            if t == n - 4:
                kn0_s[...] = keys(Group(jnp.minimum(g + 1, NGRP - 1)), 0)
        return export(G)

    init = ([[jnp.zeros((8, T), F32)] * GH for _ in max_keys],
            [jnp.ones((32, T), F32) for _ in acc_keys],
            [jnp.zeros((GR, T), F32) for _ in ret_keys])
    kn0_s[...] = keys(Group(0), 0)
    state = init if CFG['only'] == 'p1' else lax.fori_loop(0, NGRP, phase2, init)

    cps[-1].wait()

    def phase3(b):
        o = jnp.concatenate(
            [jnp.concatenate([ot_s[b * (OB // T) + m, tile(j), :].T for j in range(ND)], axis=1)
             for m in range(OB // T)], axis=0)
        yb_s[b] = _dot(o, wo_v[...]).astype(BF16)

    zs, zl, ps, plo = attn_base()
    P = adopt(NGRP - 1, state)
    phase3(0)
    for t in range(lag2):
        pv_step(P, n + t - lag2, plo)
        if t < lag:
            for c in range(nc):
                exp_part(P, n + t - lag, c, zl, ps)
    outb_copy(0).start()

    def body3(b, carry):
        phase3(b)
        outb_copy(b).start()
        return carry

    lax.fori_loop(1, S // OB, body3, 0)

    for c in range(ND):
        outa_copy(c).wait()
    for b in range(S // OB):
        outb_copy(b).wait()


@jax.jit
def pallas_concat_heads__ssm_conv_h3__memory_aug_infini_attn__prompt_kernel(
    A_q: jax.Array,
    A_k: jax.Array,
    A_v: jax.Array,
    A_shift_k: jax.Array,
    A_ssm_k: jax.Array,
    A_ssm_D: jax.Array,
    B_x: jax.Array,
    B_wq: jax.Array,
    B_wk: jax.Array,
    B_wv: jax.Array,
    B_wo: jax.Array,
    B_beta: jax.Array,
):
    hbm = pl.BlockSpec(memory_space=pltpu.MemorySpace.HBM)
    vmem = pltpu.VMEM
    dma = pltpu.SemaphoreType.DMA
    out = pl.pallas_call(
        _kernel,
        out_shape=jax.ShapeDtypeStruct((S, 2 * D), BF16),
        in_specs=[pl.BlockSpec(memory_space=pltpu.SMEM)] + [hbm] * 14,
        out_specs=hbm,
        scratch_shapes=[
            vmem((ND, S, T), BF16),
            vmem((ND, S, T), BF16),
            vmem((ND, S, T), BF16),
            vmem((KS, D), BF16),
            vmem((ND, T, S), BF16),
            vmem((1, D), BF16),
            vmem((S, D), BF16),
            vmem((3, D, D), BF16),
            vmem((D, D), BF16),
            vmem((1, H), BF16),
            vmem((2 * T, T), BF16),
            vmem((T, 2 * T), BF16),
            vmem((ND, ND, 3 * T, T), BF16),
            vmem((8, D), F32),
            vmem((D, T), F32),
            vmem((S + 8, T), F32),
            vmem((S, T), BF16),
            vmem((2 * NT, SP_PACE + 8, T), F32),
            vmem((NT + 1, 2 * T, T), BF16),
            vmem((ND, S, T), BF16),
            vmem((NT, D, T), BF16),
            vmem((NT - L // T, D, T), BF16),
            vmem((NT, D, T), BF16),
            vmem((NT - L // T, D, T), BF16),
            vmem((NT, D, T), BF16),
            vmem((NT, D, T), BF16),
            vmem((S // OB, OB, D), BF16),
            vmem((CFG['rs'] * GH * T, T), F32),
            vmem((T, T), BF16),
            dma((10,)),
            dma((4, ND)),
            dma((ND,)),
            dma((S // OB,)),
        ] + [vmem((GH * T, T), BF16)] * CFG['rp'],
        compiler_params=pltpu.CompilerParams(vmem_limit_bytes=100 * 1024 * 1024),
        name="h3_infini_concat",
    )(
        jnp.asarray(np.zeros((8,), np.int32)),
        A_q.reshape(S, D), A_k.reshape(S, D), A_v.reshape(S, D), A_shift_k.T, A_ssm_k,
        A_ssm_D.reshape(1, D), B_x.reshape(S, D), B_wq, B_wk, B_wv, B_wo,
        B_beta.reshape(1, H),
        jnp.asarray(_FWD, dtype=BF16), jnp.asarray(_INV, dtype=BF16),
    )
    return out.reshape(1, S, 2 * D)
```

```python
import math

import jax
import jax.numpy as jnp
import numpy as np
from jax import lax
from jax.experimental import pallas as pl
from jax.experimental.pallas import tpu as pltpu

CFG = dict(lag=4, lag2=6, nc=4, rs=8, rp=4, orders=['0123'] * 4, pn=512,
           p1seq='hvvvvkkcvvvvkcvvvvkcvvvvpiu', p1last='vvvvvcvvvvvcvvvvvvpip', peel=1, conv='reg', yspec=0, gateh=0, only='', hmajor=1,
           memat=2, flag=3, p3seq='vvvvcvvvvc0vvvvc1vvvvp2i3a', wu32=1, splitk=0, cform=3, nomax=0, nodma=0, lateout=0, updat=6, ob=512, p3tail=1)

S = 2048
D = 640
H = 32
DH = D // H
NSEG = 4
L = S // NSEG
KS = 4
T = 128
NT = S // T
ND = D // T
GH = 4
GR = GH * DH
NGRP = H // GH
OB = CFG['ob']
LOG2E = math.log2(math.e)
NEG = -1e30
SUM_LOG2 = CFG.get('sumlog', 30)

F32 = jnp.float32
BF16 = jnp.bfloat16

SP_H, SP_U, SP_Y, SP_T, SP_PACE = 0, 2 * T, 4 * T, 4 * T, 4 * T + 32


def _dft_matrices():
    k = np.arange(T, dtype=np.float64)[:, None]
    t = np.arange(T, dtype=np.float64)[None, :]
    theta = 2.0 * np.pi * (k + 0.25) * t / T
    re = np.cos(theta).reshape(T // 8, 1, 8, T)
    im = np.sin(theta).reshape(T // 8, 1, 8, T)
    fwd = np.concatenate([re, im], axis=1).reshape(2 * T, T)
    inv = fwd.T / T
    return fwd.astype(np.float32), inv.astype(np.float32)


_FWD, _INV = _dft_matrices()


def _dot(a, b):
    return jnp.dot(a, b, preferred_element_type=F32)


def _dot_nt(a, b):
    return lax.dot_general(a, b, (((1,), (1,)), ((), ())), preferred_element_type=F32)


def _phi(t):
    return jnp.where(t > 0, t + 1.0, jnp.exp(t))


def _causal_products(u, h):
    out = []
    for a in range(len(u)):
        acc = u[0] * h[a]
        for j in range(1, a + 1):
            acc = acc + u[j] * h[a - j]
        out.append(acc)
    return out


import contextlib
_stack = []
def mark(name):
    if not CFG.get('scopes'):
        return
    if _stack:
        _stack.pop().__exit__(None, None, None)
    if name:
        cm = jax.named_scope(name)
        cm.__enter__()
        _stack.append(cm)


def _kernel(
    zero_ref, q_hbm, k_hbm, v_hbm, shift_hbm, h_hbm, d_hbm, x_hbm, wq_hbm, wk_hbm, wv_hbm,
    wo_hbm, beta_hbm, fwd_hbm, inv_hbm,
    out_hbm,
    q_v, k_v, v_v, shift_v, h_v, d_v, x_v, w_v, wo_v, beta_v, fwd_v, inv_v,
    wt_s, taps_s, gate_s, kpad_s, kv_s, spec_s, yf_s, ya_s,
    qs_s, pq_s, kt_s, pk_s, vt_s, ot_s, yb_s, s_ref, kn0_s,
    in_sem, slab_sem, w_sem, x_sem, outa_sem, outb_sem, *p_refs,
):
    RS, RP = CFG['rs'], CFG['rp']

    def tile(i):
        return slice(i * T, (i + 1) * T)

    def slab_cols(c):
        return pl.ds(c * T if isinstance(c, int) else pl.multiple_of(c * T, T), T)

    def kvh_copies(c):
        col = slab_cols(c)
        return (
            pltpu.make_async_copy(k_hbm.at[:, col], k_v.at[c], slab_sem.at[0, c]),
            pltpu.make_async_copy(v_hbm.at[:, col], v_v.at[c], slab_sem.at[1, c]),
            pltpu.make_async_copy(h_hbm.at[col, :], h_v.at[c], slab_sem.at[2, c]),
        )

    def q_copy(c):
        return pltpu.make_async_copy(q_hbm.at[:, slab_cols(c)], q_v.at[c], slab_sem.at[3, c])

    def outa_copy(c):
        return pltpu.make_async_copy(ya_s.at[c], out_hbm.at[:, slab_cols(c)], outa_sem.at[c])

    def outb_copy(b):
        row = pl.ds(b * OB if isinstance(b, int) else pl.multiple_of(b * OB, OB), OB)
        return pltpu.make_async_copy(
            yb_s.at[b], out_hbm.at[row, pl.ds(D, D)], outb_sem.at[b])

    def w_copies(c):
        col = slab_cols(c)
        return tuple(
            pltpu.make_async_copy(w.at[:, col], w_v.at[c, i], w_sem.at[i, c])
            for i, w in enumerate((wq_hbm, wk_hbm, wv_hbm)))

    def x_copy(b):
        return pltpu.make_async_copy(
            x_hbm.at[pl.ds(b * L, L), :], x_v.at[pl.ds(b * L, L), :], x_sem.at[b])

    small = [(shift_hbm, shift_v), (d_hbm, d_v), (beta_hbm, beta_v),
             (fwd_hbm, fwd_v), (inv_hbm, inv_v)]
    small = [pltpu.make_async_copy(a, b, in_sem.at[i]) for i, (a, b) in enumerate(small)]
    wo_copy = pltpu.make_async_copy(wo_hbm, wo_v, in_sem.at[len(small)])

    def start(*groups):
        for grp in groups:
            for cp in grp:
                cp.start()

    def wait(*groups):
        for grp in groups:
            for cp in grp:
                cp.wait()

    start(w_copies(0), [x_copy(0)])

    mark('S0_init')
    kpad_s[0:8, :] = jnp.zeros((8, T), F32)

    def small_tables():
        taps_s[0:KS, :] = shift_v[...].astype(F32)
        taps_s[KS:KS + 1, :] = d_v[...].astype(F32)
        g_row = jax.nn.sigmoid(beta_v[...].astype(F32))
        row = lax.broadcasted_iota(jnp.int32, (D, H), 0)
        head = lax.broadcasted_iota(jnp.int32, (D, H), 1)
        own = (row >= head * DH) & (row < (head + 1) * DH)
        g_col = jnp.sum(jnp.where(own, g_row, 0.0), axis=1, keepdims=True)
        gate_s[...] = jnp.broadcast_to(g_col, (D, T))

    def tap(c, j):
        return taps_s[j:j + 1, slab_cols(c)]

    def kv_prep(c, a0=0, a1=NT):
        kpad_s[8 + a0 * T:8 + a1 * T, :] = k_v[c, a0 * T:a1 * T, :].astype(F32)
        w = [tap(c, j) for j in range(KS)]
        for a in range(a0, a1):
            acc = None
            for j in range(KS):
                term = kpad_s[8 + a * T - j:8 + (a + 1) * T - j, :] * w[j]
                acc = term if acc is None else acc + term
            kv = acc * v_v[c, tile(a), :].astype(F32)
            kv_s[tile(a), :] = kv.astype(BF16)
        return kv[T - 8:]

    def spec_base(rd, wr):
        return [pl.multiple_of(zero_ref[n], 8) for n in range(2)] + [zero_ref[2], zero_ref[3], rd * NT, wr * NT]

    def store_spec(z, off, val):
        for a in range(NT):
            spec_s[z[5] + a, pl.ds(z[0] + off, 2 * T), :] = val[:, tile(a)]

    def fwd_h(c, z):
        h_rows = jnp.concatenate([h_v[c, :, tile(a)] for a in range(NT)], axis=0)
        store_spec(z, SP_H, _dot_nt(fwd_v[...], h_rows))

    def fwd_u(z):
        u = jnp.concatenate([kv_s[tile(a), :] for a in range(NT)], axis=1)
        store_spec(z, SP_U, _dot(fwd_v[...], u))

    def chunk_conv(c, z, f):
        def ld(off):
            return [spec_s[z[4] + a, pl.ds(z[1] + off + f16, 8), :] for a in range(NT)]

        def st(off, vals):
            for a in range(NT):
                spec_s[a, pl.ds(z[0] + off, 8), :] = vals[a]

        f16 = 16 * f if isinstance(f, int) else pl.multiple_of(16 * f, 16)
        hr, hi = ld(SP_H), ld(SP_H + 8)
        hr[0] = hr[0] + tap(c, KS)
        gr = [hr[0]] + [hr[a] + hi[a - 1] for a in range(1, NT)]
        gi = [hi[0]] + [hi[a] - hr[a - 1] for a in range(1, NT)]
        gd = [y - x for x, y in zip(gr, gi)]
        gs = [x + y for x, y in zip(gr, gi)]
        ur, ui = ld(SP_U), ld(SP_U + 8)
        k1 = _causal_products([x + y for x, y in zip(ur, ui)], gr)
        if CFG['cform'] == 0:
            k2 = _causal_products(ur, gd)
            k3 = _causal_products(ui, gs)
            re = [x - y for x, y in zip(k1, k3)]
            im = [x + y for x, y in zip(k1, k2)]
        elif CFG['cform'] == 1:
            re, im = [], []
            for a in range(NT):
                x = y = k1[a]
                for j in range(a + 1):
                    x = x - ui[j] * gs[a - j]
                    y = y + ur[j] * gd[a - j]
                re.append(x)
                im.append(y)
        elif CFG['cform'] == 2:
            def cconv(u_r, u_i, g_r, g_i):
                p1 = _causal_products([x + y for x, y in zip(u_r, u_i)], g_r)
                p2 = _causal_products(u_r, [y - x for x, y in zip(g_r, g_i)])
                p3 = _causal_products(u_i, [x + y for x, y in zip(g_r, g_i)])
                return [x - y for x, y in zip(p1, p3)], [x + y for x, y in zip(p1, p2)]
            add = lambda p, q: [x + y for x, y in zip(p, q)]
            er, ei = cconv(ur[0::2], ui[0::2], gr[0::2], gi[0::2])
            o_r, o_i = cconv(ur[1::2], ui[1::2], gr[1::2], gi[1::2])
            mr, mi = cconv(add(ur[0::2], ur[1::2]), add(ui[0::2], ui[1::2]),
                           add(gr[0::2], gr[1::2]), add(gi[0::2], gi[1::2]))
            re, im = [None] * NT, [None] * NT
            for m in range(NT // 2):
                re[2 * m] = er[m] if m == 0 else er[m] + o_r[m - 1]
                im[2 * m] = ei[m] if m == 0 else ei[m] + o_i[m - 1]
                re[2 * m + 1] = mr[m] - er[m] - o_r[m]
                im[2 * m + 1] = mi[m] - ei[m] - o_i[m]
        elif CFG['cform'] == 3:
            re, im = [], []
            for a in range(NT):
                x = ur[0] * gr[a] - ui[0] * gi[a]
                y = ur[0] * gi[a] + ui[0] * gr[a]
                for j in range(1, a + 1):
                    x = x + (ur[j] * gr[a - j] - ui[j] * gi[a - j])
                    y = y + (ur[j] * gi[a - j] + ui[j] * gr[a - j])
                re.append(x)
                im.append(y)
        for a in range(NT):
            y = jnp.concatenate([re[a], im[a]], axis=0)
            yf_s[z[2] + a if CFG['gateh'] else a, pl.ds(f16, 16), :] = y.astype(BF16)

    def inverse(c, z):
        ys = [yf_s[a] for a in range(NT)]
        y = _dot(inv_v[...], jnp.concatenate(ys, axis=1))
        for a in range(NT):
            ya_s[c, tile(a), :] = (
                q_v[c, tile(a), :].astype(F32) * y[:, tile(a)]).astype(BF16)

    q_scale = (DH ** -0.5) * LOG2E
    PN = CFG['pn']

    def project(c, b):
        frow = slab_cols(c)
        if CFG['wu32']:
            w = jnp.concatenate([pltpu.bitcast(wt_s[c, j], BF16) for j in range(ND)], axis=1)
        else:
            w = jnp.concatenate([wt_s[c, j] for j in range(ND)], axis=1)
        if CFG['splitk']:
            r = None
            for j in range(ND):
                part = _dot_nt(w[:, tile(j)], x_v[b * PN:(b + 1) * PN, tile(j)])
                r = part if r is None else r + part
        else:
            r = _dot_nt(w, x_v[b * PN:(b + 1) * PN, :])
        for n in range(PN // T):
            a = b * (PN // T) + n
            qf, kf, vf = r[0:T, tile(n)], r[T:2 * T, tile(n)], r[2 * T:3 * T, tile(n)]
            qs_s[a, frow, :] = (qf * q_scale).astype(BF16)
            kb = kf.astype(BF16)
            kt_s[a, frow, :] = kb
            vt_s[a, frow, :] = vf.astype(BF16)
            if a * T >= L:
                pq_s[a - L // T, frow, :] = _phi(qf.astype(BF16).astype(F32)).astype(BF16)
            if a * T < S - L:
                pk_s[a, frow, :] = _phi(kb.astype(F32)).astype(BF16)
        return r

    def transpose_w(c):
        for i in range(3):
            for j in range(ND):
                wt = w_v[c, i, tile(j), :].T
                if CFG['wu32']:
                    wt_s[c, j, i * T // 2:(i + 1) * T // 2, :] = pltpu.bitcast(wt, jnp.uint32)
                else:
                    wt_s[c, j, tile(i), :] = wt

    def phase1(c, seq):
        if not CFG['nodma']:
            @pl.when(c + 3 < ND)
            def _():
                start(kvh_copies(c + 3), w_copies(c + 3))

            @pl.when(c + 2 < ND)
            def _():
                start([q_copy(c + 2)])
                wait(w_copies(c + 2))

            @pl.when(c == 1)
            def _():
                wo_copy.start()

            wait(kvh_copies(c + 1), [q_copy(c)])
        z = spec_base(c % 2, (c + 1) % 2)
        transpose_w(jnp.minimum(c + 2, ND - 1))
        nk = seq.count('k') + seq.count('K')
        nb = nf = ik = 0
        for ch in seq:
            if ch == 'h':
                fwd_h(c + 1, z)
            elif ch == 'u':
                fwd_u(z)
            elif ch == 'i':
                assert nf == NT
                inverse(c, z)
            elif ch == 'p':
                project(c + 1, nb)
                nb += 1
            elif ch == 'c':
                r = project(c + 1, nb)
                spec_s[0, pl.ds(z[0] + SP_PACE, 8), :] = r[3 * T - 8:, 0:T]
                nb += 1
            elif ch in 'kK':
                last = kv_prep(c + 1, ik * NT // nk, (ik + 1) * NT // nk)
                if ch == 'k':
                    spec_s[0, pl.ds(z[0] + SP_PACE, 8), :] = last
                ik += 1
            elif ch == 'v':
                chunk_conv(c, z, nf)
                nf += 1
        assert nb * PN == S
        if not CFG['nodma'] and not CFG['lateout']:
            outa_copy(c).start()

    def body1(c, carry):
        phase1(c, CFG['p1seq'])
        return carry

    steps = [(s, int(i), j) for s in range(NSEG) for i in CFG['orders'][s]
             for j in range(int(i) + 1)]
    n = len(steps)
    per_seg = n // NSEG
    first = [t for t in range(n) if steps[t][2] == 0]
    if CFG['hmajor']:
        cells = [(t0 + j, h) for t0 in first for h in range(GH) for j in range(steps[t0][1] + 1)]
    else:
        cells = [(t, h) for t in range(n) for h in range(GH)]
    lag, lag2, nc = CFG['lag'], CFG['lag2'], CFG['nc']
    tpl = L // T
    def cell(m):
        t, h = cells[m]
        return steps[t] + (h,)

    flag = CFG['flag']
    late = [steps[t] for t in range(n - flag, n)]
    done_late = {(s, i) for s, i, j in late}
    acc_keys = sorted({(s, i, h) for s, i, j in steps[:n - flag] if (s, i) in done_late
                       for h in range(GH)})
    ret_keys = sorted(k for k in done_late if k[0] > 0)

    class Group:
        def __init__(self, g):
            self.g = g
            self.r0 = g * GR if isinstance(g, int) else pl.multiple_of(g * GR, 16)
            self.rows = pl.ds(self.r0, GR)
            self.kn, self.va, self.w = {}, {}, {}
            self.maxes, self.accs, self.rets, self.mems = {}, {}, {}, {}
            self.lo = self.hi = None

    r16 = lambda: lax.broadcasted_iota(jnp.int32, (16, T), 0)
    low4 = lambda: lax.broadcasted_iota(jnp.int32, (8, T), 0) < 4

    def pad_rows(x):
        return jnp.concatenate([x, jnp.zeros((T - GR, x.shape[1]), x.dtype)], axis=0)

    def keys(G, a):
        if a not in G.kn:
            G.kn[a] = pad_rows(kt_s[a, G.rows, :]).T
        return G.kn[a]

    def values(G, a):
        if a not in G.va:
            vt = vt_s[a, G.rows, :]
            b = [vt[16 * m:16 * m + 16] for m in range(5)]
            lo = low4()
            one2 = jnp.full((8, T), 0x3F803F80, jnp.uint32)

            def top(x):
                return pltpu.bitcast(jnp.where(lo, pltpu.bitcast(x, jnp.uint32), one2), BF16)

            def bottom(x):
                return pltpu.bitcast(jnp.where(lo, one2, pltpu.bitcast(x, jnp.uint32)), BF16)

            G.va[a] = [
                jnp.concatenate([b[0], top(b[1])], axis=0),
                jnp.concatenate([b[1], top(b[2])], axis=0),
                jnp.concatenate([bottom(b[2]), b[3]], axis=0),
                jnp.concatenate([bottom(b[3]), b[4]], axis=0),
            ]
        return G.va[a]

    def queries(G, a):
        if a not in G.w:
            r16 = lax.broadcasted_iota(jnp.int32, (16, T), 0)
            ws = []
            for h in range(GH):
                lo = (h * DH - 16 * h) // 2
                keep = (r16 >= lo) & (r16 < lo + DH // 2)
                blk = pltpu.bitcast(qs_s[a, pl.ds(G.r0 + 16 * h, 32), :], jnp.uint32)
                blk = pltpu.bitcast(jnp.where(keep, blk, jnp.zeros_like(blk)), BF16)
                pieces = [blk, jnp.zeros((T - 32 - 16 * h, T), BF16)]
                if h:
                    pieces = [jnp.zeros((16 * h, T), BF16)] + pieces
                ws.append(jnp.concatenate(pieces, axis=0))
            G.w[a] = jnp.concatenate(ws, axis=1)
        return G.w[a]

    def recip(d):
        r = pl.reciprocal(d, approx=True)
        return r * (2.0 - d * r)

    def assemble(parts):
        lo = low4()
        u = [[p[8 * m:8 * m + 8] for m in range(4)] for p in parts]
        vals = [u[0][0], u[0][1], jnp.where(lo, u[0][2], u[1][0]), u[1][1], u[1][2],
                u[2][1], u[2][2], jnp.where(lo, u[2][3], u[3][1]), u[3][2], u[3][3]]
        return jnp.concatenate(vals, axis=0), (u[0][3], u[1][3], u[2][0], u[3][0])

    def spread(d):
        lo = low4()
        return jnp.concatenate(
            [d[0], d[0], jnp.where(lo, d[0], d[1]), d[1], d[1],
             d[2], d[2], jnp.where(lo, d[2], d[3]), d[3], d[3]], axis=0)

    def update(G, s):
        va = jnp.concatenate(
            [jnp.concatenate(values(G, s * tpl + j), axis=0) for j in range(tpl)], axis=1)
        pk = jnp.concatenate(
            [pad_rows(pk_s[s * tpl + j, G.rows, :]) for j in range(tpl)], axis=1)
        upd = _dot_nt(va, pk)
        lane = lax.broadcasted_iota(jnp.int32, (32, T), 1)
        upd = jnp.concatenate([
            jnp.where((lane >= h * DH) & (lane < (h + 1) * DH), upd[32 * h:32 * h + 32], 0.0)
            for h in range(GH)], axis=0)
        G.mems[s + 1] = upd if s == 0 else G.mems[s] + upd

    def retrieve(G, s):
        pq = jnp.concatenate(
            [pad_rows(pq_s[(s - 1) * tpl + i, G.rows, :]) for i in range(tpl)], axis=1)
        ret = _dot(G.mems[s].astype(BF16), pq)
        gate = gate_s[G.rows, :]
        for i in range(tpl):
            vals, dens = assemble([ret[32 * h:32 * h + 32, tile(i)] for h in range(GH)])
            G.rets[(s, i)] = vals * (gate * spread([recip(d + 1e-6) for d in dens]))

    def finish(G, s, i):
        vals, dens = assemble([G.accs[(s, i, h)] for h in range(GH)])
        if G.lo is not None:
            for d in dens:
                G.lo, G.hi = jnp.minimum(G.lo, d), jnp.maximum(G.hi, d)
        o = vals * ((1.0 - gate_s[G.rows, :]) * spread([recip(d) for d in dens]))
        if s > 0:
            o = o + G.rets[(s, i)]
        ot_s[s * tpl + i, G.rows, :] = o.astype(BF16)

    def qk_dot(G, t):
        s, i, j = steps[t]
        return _dot(keys(G, s * tpl + j), queries(G, s * tpl + i))

    def qk_store(G, t, raw, c, zs):
        s, i, j = steps[t]
        r0, r1 = c * T // nc, (c + 1) * T // nc
        causal = (r0 + lax.broadcasted_iota(jnp.int32, (r1 - r0, T), 0)
                  <= lax.broadcasted_iota(jnp.int32, (r1 - r0, T), 1))
        ms = []
        for h in range(GH):
            sc = raw[r0:r1, tile(h)]
            if j == i:
                sc = jnp.where(causal, sc, NEG)
            s_ref[pl.ds(zs + ((t % RS) * GH + h) * T + r0, r1 - r0), :] = sc
            m8 = sc[0:8]
            for r in range(1, (r1 - r0) // 8):
                m8 = jnp.maximum(m8, sc[8 * r:8 * r + 8])
            if j > 0 or c > 0:
                m8 = jnp.maximum(G.maxes[(s, i)][h], m8)
            if j == i and c == nc - 1:
                m8 = jnp.broadcast_to(jnp.max(m8, axis=0, keepdims=True), (8, T))
            ms.append(m8)
        G.maxes[(s, i)] = ms

    def exp_part(G, t, c, zl, ps):
        per = GH * T // nc
        slot, r0 = (c * per) // T, (c * per) % T
        tq, h = cells[t * GH + slot]
        s, i, j = steps[tq]
        m = jnp.concatenate([G.maxes[(s, i)][h]] * (per // 8), axis=0)
        sc = s_ref[pl.ds(zl + ((tq % RS) * GH + h) * T + r0, per), :]
        p_refs[t % RP][pl.ds(ps + slot * T + r0, per), :] = jnp.exp2(sc - m).astype(BF16)

    def pv_step(G, t, plo):
        for slot in range(GH):
            s, i, j, h = cell(t * GH + slot)
            r = _dot(values(G, s * tpl + j)[h], p_refs[t % RP][pl.ds(plo + slot * T, T), :])
            G.accs[(s, i, h)] = r if j == 0 else G.accs[(s, i, h)] + r
            if j == i and h == GH - 1:
                finish(G, s, i)

    def exp_direct(t, raw, ps):
        s, i, j = steps[t]
        causal = (lax.broadcasted_iota(jnp.int32, (T, T), 0)
                  <= lax.broadcasted_iota(jnp.int32, (T, T), 1))
        for h in range(GH):
            p = jnp.exp2(raw[:, tile(h)])
            if j == i:
                p = jnp.where(causal, p, 0.0)
            p_refs[t % RP][pl.ds(ps + h * T, T), :] = p.astype(BF16)

    def pv_direct(G, t, plo):
        s, i, j = steps[t]
        for h in range(GH):
            r = _dot(values(G, s * tpl + j)[h], p_refs[t % RP][pl.ds(plo + h * T, T), :])
            G.accs[(s, i, h)] = r if j == 0 else G.accs[(s, i, h)] + r
        if j == i:
            finish(G, s, i)

    def attn_base():
        return ([pl.multiple_of(zero_ref[m], 8) for m in range(2)]
                + [pl.multiple_of(zero_ref[m], 16) for m in range(2, 4)])

    def adopt(g, state):
        P = Group(g)
        P.accs = dict(zip(acc_keys, state[0]))
        P.rets = dict(zip(ret_keys, state[1]))
        P.lo, P.hi = state[2]
        return P

    def memory_steps(G, t):
        s = t // per_seg
        if t % per_seg == CFG['memat'] and s > 0:
            retrieve(G, s)
        if t % per_seg == CFG['updat'] and s < NSEG - 1:
            update(G, s)

    def attention(g, state):
        _, _, ps, plo = attn_base()
        G = Group(g)
        if isinstance(g, int):
            P = None
            G.lo = G.hi = jnp.ones((8, T), F32)
        else:
            P = adopt(g - 1, state)
        G.kn[0] = kn0_s[...]
        for t in range(n):
            raw = qk_dot(G, t)
            memory_steps(G, t)
            if t >= flag:
                pv_direct(G, t - flag, plo)
            elif P is not None:
                pv_direct(P, n + t - flag, plo)
                G.lo, G.hi = P.lo, P.hi
            exp_direct(t, raw, ps)
            if t == n - 4 and P is not None:
                kn0_s[...] = keys(Group(jnp.minimum(g + 1, NGRP - 1)), 0)
        return ([G.accs[k] for k in acc_keys], [G.rets[k] for k in ret_keys], (G.lo, G.hi))

    def attention_true_max(g, carry):
        zs, zl, ps, plo = attn_base()
        G = Group(g)
        for t in range(n + lag2):
            if t < n:
                raw = qk_dot(G, t)
                memory_steps(G, t)
            if t >= lag2:
                pv_step(G, t - lag2, plo)
            for c in range(nc):
                if t < n:
                    qk_store(G, t, raw, c, zs)
                if lag <= t < n + lag:
                    exp_part(G, t - lag, c, zl, ps)
        return carry

    def out_proj(b):
        o = jnp.concatenate(
            [jnp.concatenate([ot_s[b * (OB // T) + m, tile(j), :].T for j in range(ND)], axis=1)
             for m in range(OB // T)], axis=0)
        r = _dot(o, wo_v[...])
        yb_s[b] = r.astype(BF16)
        return r

    init = ([jnp.ones((32, T), F32) for _ in acc_keys],
            [jnp.zeros((GR, T), F32) for _ in ret_keys],
            (jnp.ones((8, T), F32), jnp.ones((8, T), F32)))
    mark('S1_wait0')
    wait(w_copies(0))
    transpose_w(0)
    wait([x_copy(0)])
    mark('S2_proj0')
    start([x_copy(1)], small)
    project(0, 0)
    wait([x_copy(1)], small)
    start([x_copy(2)])
    small_tables()
    project(0, 1)
    wait([x_copy(2)])
    start([x_copy(3)])
    project(0, 2)
    mark('S3_proj0b')
    wait([x_copy(3)])
    start(kvh_copies(0), w_copies(1), kvh_copies(1), [q_copy(0)], w_copies(2), kvh_copies(2), [q_copy(1)])
    kn0_s[...] = keys(Group(0), 0)
    project(0, 3)
    mark('S4_attn0')
    state = attention(0, None) if CFG['only'] != 'p1' else init
    mark('S5_fwd0')
    wait(kvh_copies(0), w_copies(1))
    z = spec_base(1, 0)
    fwd_h(0, z)
    kv_prep(0)
    transpose_w(1)
    fwd_u(z)
    if CFG['nodma']:
        mark('S5b_dma')
        for c in (3, 4):
            start(kvh_copies(c), w_copies(c))
        start([q_copy(2), q_copy(3), q_copy(4), wo_copy])
        for c in (1, 2, 3, 4):
            wait(kvh_copies(c), [q_copy(c - 1)])
        for c in (2, 3, 4):
            wait(w_copies(c))
    mark('S6_p1loop')

    def body1(c, carry):
        phase1(c, CFG['p1seq'])
        return carry

    lax.fori_loop(0, ND - 1, body1, 0)
    mark('S7_p2')
    if CFG['nodma'] or CFG['lateout']:
        start([outa_copy(c) for c in range(ND - 1)])
    kn0_s[...] = keys(Group(1), 0)
    if CFG['only'] != 'p1':
        state = lax.fori_loop(1, NGRP, attention, state)

    mark('S7b_check')
    _, _, ps, plo = attn_base()
    P = adopt(NGRP - 1, state)
    for t in range(n - flag, n):
        pv_direct(P, t, plo)
    safe = (jnp.min(P.lo) >= 2.0 ** -SUM_LOG2) & (jnp.max(P.hi) <= 2.0 ** SUM_LOG2)

    @pl.when(jnp.logical_not(safe))
    def _():
        lax.fori_loop(0, NGRP, attention_true_max, 0)

    mark('S8_p3')
    wait([wo_copy, q_copy(ND - 1)])
    z = spec_base((ND - 1) % 2, 0)
    nb = nf = 0
    for ch in CFG['p3seq']:
        if ch == 'v':
            chunk_conv(ND - 1, z, nf)
            nf += 1
        elif ch == 'i':
            inverse(ND - 1, z)
        elif ch == 'a':
            outa_copy(ND - 1).start()
        elif ch in 'pc':
            r = out_proj(nb)
            if ch == 'c':
                spec_s[0, pl.ds(z[0] + SP_PACE, 8), :] = r[OB - 8:, D - T:]
            nb += 1
        elif ch.isdigit():
            outb_copy(int(ch)).start()
    assert nb == S // OB and nf == NT
    mark('SA_final')

    for c in range(ND):
        outa_copy(c).wait()
    for b in range(S // OB):
        outb_copy(b).wait()
    mark(None)


@jax.jit
def pallas_concat_heads__ssm_conv_h3__memory_aug_infini_attn__prompt_kernel(
    A_q: jax.Array,
    A_k: jax.Array,
    A_v: jax.Array,
    A_shift_k: jax.Array,
    A_ssm_k: jax.Array,
    A_ssm_D: jax.Array,
    B_x: jax.Array,
    B_wq: jax.Array,
    B_wk: jax.Array,
    B_wv: jax.Array,
    B_wo: jax.Array,
    B_beta: jax.Array,
):
    hbm = pl.BlockSpec(memory_space=pltpu.MemorySpace.HBM)
    vmem = pltpu.VMEM
    dma = pltpu.SemaphoreType.DMA
    out = pl.pallas_call(
        _kernel,
        out_shape=jax.ShapeDtypeStruct((S, 2 * D), BF16),
        in_specs=[pl.BlockSpec(memory_space=pltpu.SMEM)] + [hbm] * 14,
        out_specs=hbm,
        scratch_shapes=[
            vmem((ND, S, T), BF16),
            vmem((ND, S, T), BF16),
            vmem((ND, S, T), BF16),
            vmem((KS, D), BF16),
            vmem((ND, T, S), BF16),
            vmem((1, D), BF16),
            vmem((S, D), BF16),
            vmem((ND, 3, D, T), BF16),
            vmem((D, D), BF16),
            vmem((1, H), BF16),
            vmem((2 * T, T), BF16),
            vmem((T, 2 * T), BF16),
            vmem((ND, ND, 3 * T // 2, T), jnp.uint32) if CFG['wu32'] else vmem((ND, ND, 3 * T, T), BF16),
            vmem((8, D), F32),
            vmem((D, T), F32),
            vmem((S + 8, T), F32),
            vmem((S, T), BF16),
            vmem((2 * NT, SP_PACE + 8, T), F32),
            vmem((NT, 2 * T, T), BF16),
            vmem((ND, S, T), BF16),
            vmem((NT, D, T), BF16),
            vmem((NT - L // T, D, T), BF16),
            vmem((NT, D, T), BF16),
            vmem((NT - L // T, D, T), BF16),
            vmem((NT, D, T), BF16),
            vmem((NT, D, T), BF16),
            vmem((S // OB, OB, D), BF16),
            vmem((CFG['rs'] * GH * T, T), F32),
            vmem((T, T), BF16),
            dma((6,)),
            dma((4, ND)),
            dma((3, ND)),
            dma((NSEG,)),
            dma((ND,)),
            dma((S // OB,)),
        ] + [vmem((GH * T, T), BF16)] * CFG['rp'],
        compiler_params=pltpu.CompilerParams(vmem_limit_bytes=100 * 1024 * 1024),
        name="h3_infini_concat",
    )(
        jnp.asarray(np.zeros((8,), np.int32)),
        A_q.reshape(S, D), A_k.reshape(S, D), A_v.reshape(S, D), A_shift_k.T, A_ssm_k,
        A_ssm_D.reshape(1, D), B_x.reshape(S, D), B_wq, B_wk, B_wv, B_wo,
        B_beta.reshape(1, H),
        jnp.asarray(_FWD, dtype=BF16), jnp.asarray(_INV, dtype=BF16),
    )
    return out.reshape(1, S, 2 * D)
```

```python
import math

import jax
import jax.numpy as jnp
import numpy as np
from jax import lax
from jax.experimental import pallas as pl
from jax.experimental.pallas import tpu as pltpu

CFG = dict(lag=4, lag2=6, nc=4, rs=8, rp=4, orders=['0123'] * 4, pn=512,
           p1seq='hvvvkkcvvvvkkcvvvvvcvvvvpiu', p1last='vvvvvcvvvvvcvvvvvvpip', peel=1, conv='reg', yspec=0, gateh=0, only='', hmajor=1,
           memat=2, flag=3, xu32=1, convat=[], p3seq='vvvvcvvvvc0vvvvc1vvvvp2i3a', wu32=1, splitk=0, cform=3, nomax=0, nodma=0, lateout=0, updat=6, ob=512, p3tail=1)

S = 2048
D = 640
H = 32
DH = D // H
NSEG = 4
L = S // NSEG
KS = 4
T = 128
NT = S // T
ND = D // T
GH = 4
GR = GH * DH
NGRP = H // GH
OB = CFG['ob']
LOG2E = math.log2(math.e)
NEG = -1e30
SUM_LOG2 = CFG.get('sumlog', 30)

F32 = jnp.float32
BF16 = jnp.bfloat16

SP_H, SP_U, SP_Y, SP_T, SP_PACE = 0, 2 * T, 4 * T, 4 * T, 4 * T + 32


def _dft_matrices():
    k = np.arange(T, dtype=np.float64)[:, None]
    t = np.arange(T, dtype=np.float64)[None, :]
    theta = 2.0 * np.pi * (k + 0.25) * t / T
    re = np.cos(theta).reshape(T // 8, 1, 8, T)
    im = np.sin(theta).reshape(T // 8, 1, 8, T)
    fwd = np.concatenate([re, im], axis=1).reshape(2 * T, T)
    inv = fwd.T / T
    return fwd.astype(np.float32), inv.astype(np.float32)


_FWD, _INV = _dft_matrices()


def _dot(a, b):
    return jnp.dot(a, b, preferred_element_type=F32)


def _dot_nt(a, b):
    return lax.dot_general(a, b, (((1,), (1,)), ((), ())), preferred_element_type=F32)


def _phi(t):
    return jnp.where(t > 0, t + 1.0, jnp.exp(t))


def _causal_products(u, h):
    out = []
    for a in range(len(u)):
        acc = u[0] * h[a]
        for j in range(1, a + 1):
            acc = acc + u[j] * h[a - j]
        out.append(acc)
    return out


import contextlib
_stack = []
def mark(name):
    if not CFG.get('scopes'):
        return
    if _stack:
        _stack.pop().__exit__(None, None, None)
    if name:
        cm = jax.named_scope(name)
        cm.__enter__()
        _stack.append(cm)


def _kernel(
    zero_ref, q_hbm, k_hbm, v_hbm, shift_hbm, h_hbm, d_hbm, x_hbm, wq_hbm, wk_hbm, wv_hbm,
    wo_hbm, beta_hbm, fwd_hbm, inv_hbm,
    out_hbm,
    q_v, k_v, v_v, shift_v, h_v, d_v, x_v, w_v, wo_v, beta_v, fwd_v, inv_v,
    wt_s, taps_s, gate_s, kpad_s, kv_s, spec_s, yf_s, ya_s,
    qs_s, pq_s, kt_s, pk_s, vt_s, ot_s, yb_s, s_ref, kn0_s, xu_s,
    in_sem, slab_sem, w_sem, x_sem, outa_sem, outb_sem, *p_refs,
):
    RS, RP = CFG['rs'], CFG['rp']

    def tile(i):
        return slice(i * T, (i + 1) * T)

    def slab_cols(c):
        return pl.ds(c * T if isinstance(c, int) else pl.multiple_of(c * T, T), T)

    def kvh_copies(c):
        col = slab_cols(c)
        return (
            pltpu.make_async_copy(k_hbm.at[:, col], k_v.at[c], slab_sem.at[0, c]),
            pltpu.make_async_copy(v_hbm.at[:, col], v_v.at[c], slab_sem.at[1, c]),
            pltpu.make_async_copy(h_hbm.at[col, :], h_v.at[c], slab_sem.at[2, c]),
        )

    def q_copy(c):
        return pltpu.make_async_copy(q_hbm.at[:, slab_cols(c)], q_v.at[c], slab_sem.at[3, c])

    def outa_copy(c):
        return pltpu.make_async_copy(ya_s.at[c], out_hbm.at[:, slab_cols(c)], outa_sem.at[c])

    def outb_copy(b):
        row = pl.ds(b * OB if isinstance(b, int) else pl.multiple_of(b * OB, OB), OB)
        return pltpu.make_async_copy(
            yb_s.at[b], out_hbm.at[row, pl.ds(D, D)], outb_sem.at[b])

    def w_copies(c):
        col = slab_cols(c)
        return tuple(
            pltpu.make_async_copy(w.at[:, col], w_v.at[c, i], w_sem.at[i, c])
            for i, w in enumerate((wq_hbm, wk_hbm, wv_hbm)))

    def x_copy(b):
        return pltpu.make_async_copy(
            x_hbm.at[pl.ds(b * L, L), :], x_v.at[pl.ds(b * L, L), :], x_sem.at[b])

    small = [(shift_hbm, shift_v), (d_hbm, d_v), (beta_hbm, beta_v),
             (fwd_hbm, fwd_v), (inv_hbm, inv_v)]
    small = [pltpu.make_async_copy(a, b, in_sem.at[i]) for i, (a, b) in enumerate(small)]
    wo_copy = pltpu.make_async_copy(wo_hbm, wo_v, in_sem.at[len(small)])

    def start(*groups):
        for grp in groups:
            for cp in grp:
                cp.start()

    def wait(*groups):
        for grp in groups:
            for cp in grp:
                cp.wait()

    start(w_copies(0), [x_copy(0)])

    mark('S0_init')
    kpad_s[0:8, :] = jnp.zeros((8, T), F32)

    def small_tables():
        shift, skip = shift_v[...].astype(F32), d_v[...].astype(F32)
        for c in range(ND):
            taps_s[c, 0:KS, :] = shift[:, tile(c)]
            taps_s[c, KS:KS + 1, :] = skip[c:c + 1, :]
        g_row = jax.nn.sigmoid(beta_v[...].astype(F32))
        row = lax.broadcasted_iota(jnp.int32, (D, H), 0)
        head = lax.broadcasted_iota(jnp.int32, (D, H), 1)
        own = (row >= head * DH) & (row < (head + 1) * DH)
        g_col = jnp.sum(jnp.where(own, g_row, 0.0), axis=1, keepdims=True)
        gate_s[...] = jnp.broadcast_to(g_col, (D, T))

    def tap(c, j):
        return taps_s[c, j:j + 1, :]

    def kv_prep(c, a0=0, a1=NT):
        kpad_s[8 + a0 * T:8 + a1 * T, :] = k_v[c, a0 * T:a1 * T, :].astype(F32)
        w = [tap(c, j) for j in range(KS)]
        for a in range(a0, a1):
            acc = None
            for j in range(KS):
                term = kpad_s[8 + a * T - j:8 + (a + 1) * T - j, :] * w[j]
                acc = term if acc is None else acc + term
            kv = acc * v_v[c, tile(a), :].astype(F32)
            kv_s[tile(a), :] = kv.astype(BF16)
        return kv[T - 8:]

    def spec_base(rd, wr):
        return [pl.multiple_of(zero_ref[n], 8) for n in range(2)] + [zero_ref[2], zero_ref[3], rd * NT, wr * NT]

    def store_spec(z, off, val):
        for a in range(NT):
            spec_s[z[5] + a, pl.ds(z[0] + off, 2 * T), :] = val[:, tile(a)]

    def fwd_h(c, z):
        h_rows = jnp.concatenate([h_v[c, :, tile(a)] for a in range(NT)], axis=0)
        store_spec(z, SP_H, _dot_nt(fwd_v[...], h_rows))

    def fwd_u(z):
        u = jnp.concatenate([kv_s[tile(a), :] for a in range(NT)], axis=1)
        store_spec(z, SP_U, _dot(fwd_v[...], u))

    def chunk_conv(c, z, f):
        def ld(off):
            return [spec_s[z[4] + a, pl.ds(z[1] + off + f16, 8), :] for a in range(NT)]

        def st(off, vals):
            for a in range(NT):
                spec_s[a, pl.ds(z[0] + off, 8), :] = vals[a]

        f16 = 16 * f if isinstance(f, int) else pl.multiple_of(16 * f, 16)
        hr, hi = ld(SP_H), ld(SP_H + 8)
        hr[0] = hr[0] + tap(c, KS)
        gr = [hr[0]] + [hr[a] + hi[a - 1] for a in range(1, NT)]
        gi = [hi[0]] + [hi[a] - hr[a - 1] for a in range(1, NT)]
        gd = [y - x for x, y in zip(gr, gi)]
        gs = [x + y for x, y in zip(gr, gi)]
        ur, ui = ld(SP_U), ld(SP_U + 8)
        k1 = _causal_products([x + y for x, y in zip(ur, ui)], gr)
        if CFG['cform'] == 0:
            k2 = _causal_products(ur, gd)
            k3 = _causal_products(ui, gs)
            re = [x - y for x, y in zip(k1, k3)]
            im = [x + y for x, y in zip(k1, k2)]
        elif CFG['cform'] == 1:
            re, im = [], []
            for a in range(NT):
                x = y = k1[a]
                for j in range(a + 1):
                    x = x - ui[j] * gs[a - j]
                    y = y + ur[j] * gd[a - j]
                re.append(x)
                im.append(y)
        elif CFG['cform'] in (2, 4):
            def cconv(u_r, u_i, g_r, g_i):
                if CFG['cform'] == 4:
                    xs, ys = [], []
                    for a in range(len(u_r)):
                        x = u_r[0] * g_r[a] - u_i[0] * g_i[a]
                        y = u_r[0] * g_i[a] + u_i[0] * g_r[a]
                        for j in range(1, a + 1):
                            x = x + (u_r[j] * g_r[a - j] - u_i[j] * g_i[a - j])
                            y = y + (u_r[j] * g_i[a - j] + u_i[j] * g_r[a - j])
                        xs.append(x)
                        ys.append(y)
                    return xs, ys
                p1 = _causal_products([x + y for x, y in zip(u_r, u_i)], g_r)
                p2 = _causal_products(u_r, [y - x for x, y in zip(g_r, g_i)])
                p3 = _causal_products(u_i, [x + y for x, y in zip(g_r, g_i)])
                return [x - y for x, y in zip(p1, p3)], [x + y for x, y in zip(p1, p2)]
            add = lambda p, q: [x + y for x, y in zip(p, q)]
            er, ei = cconv(ur[0::2], ui[0::2], gr[0::2], gi[0::2])
            o_r, o_i = cconv(ur[1::2], ui[1::2], gr[1::2], gi[1::2])
            mr, mi = cconv(add(ur[0::2], ur[1::2]), add(ui[0::2], ui[1::2]),
                           add(gr[0::2], gr[1::2]), add(gi[0::2], gi[1::2]))
            re, im = [None] * NT, [None] * NT
            for m in range(NT // 2):
                re[2 * m] = er[m] if m == 0 else er[m] + o_r[m - 1]
                im[2 * m] = ei[m] if m == 0 else ei[m] + o_i[m - 1]
                re[2 * m + 1] = mr[m] - er[m] - o_r[m]
                im[2 * m + 1] = mi[m] - ei[m] - o_i[m]
        elif CFG['cform'] == 3:
            re, im = [], []
            for a in range(NT):
                x = ur[0] * gr[a] - ui[0] * gi[a]
                y = ur[0] * gi[a] + ui[0] * gr[a]
                for j in range(1, a + 1):
                    x = x + (ur[j] * gr[a - j] - ui[j] * gi[a - j])
                    y = y + (ur[j] * gi[a - j] + ui[j] * gr[a - j])
                re.append(x)
                im.append(y)
        for a in range(NT):
            y = jnp.concatenate([re[a], im[a]], axis=0)
            yf_s[z[2] + a if CFG['gateh'] else a, pl.ds(f16, 16), :] = y.astype(BF16)

    def inverse(c, z):
        ys = [yf_s[a] for a in range(NT)]
        y = _dot(inv_v[...], jnp.concatenate(ys, axis=1))
        for a in range(NT):
            ya_s[c, tile(a), :] = (
                q_v[c, tile(a), :].astype(F32) * y[:, tile(a)]).astype(BF16)

    q_scale = (DH ** -0.5) * LOG2E
    PN = CFG['pn']

    def project(c, b):
        frow = slab_cols(c)
        if CFG['wu32']:
            w = jnp.concatenate([pltpu.bitcast(wt_s[c, j], BF16) for j in range(ND)], axis=1)
        else:
            w = jnp.concatenate([wt_s[c, j] for j in range(ND)], axis=1)
        half = slice(b * PN // 2, (b + 1) * PN // 2)
        if not CFG['xu32']:
            xb = x_v[b * PN:(b + 1) * PN, :]
        elif isinstance(c, int):
            xb = x_v[b * PN:(b + 1) * PN, :]
            for j in range(ND):
                xu_s[j, half, :] = pltpu.bitcast(xb[:, tile(j)], jnp.uint32)
        else:
            xb = jnp.concatenate(
                [pltpu.bitcast(xu_s[j, half, :], BF16) for j in range(ND)], axis=1)
        if CFG['splitk']:
            r = None
            for j in range(ND):
                part = _dot_nt(w[:, tile(j)], xb[:, tile(j)])
                r = part if r is None else r + part
        else:
            r = _dot_nt(w, xb)
        for n in range(PN // T):
            a = b * (PN // T) + n
            qf, kf, vf = r[0:T, tile(n)], r[T:2 * T, tile(n)], r[2 * T:3 * T, tile(n)]
            qs_s[a, frow, :] = (qf * q_scale).astype(BF16)
            kb = kf.astype(BF16)
            kt_s[a, frow, :] = kb
            vt_s[a, frow, :] = vf.astype(BF16)
            if a * T >= L:
                pq_s[a - L // T, frow, :] = _phi(qf.astype(BF16).astype(F32)).astype(BF16)
            if a * T < S - L:
                pk_s[a, frow, :] = _phi(kb.astype(F32)).astype(BF16)
        return r

    def transpose_w(c):
        for i in range(3):
            for j in range(ND):
                wt = w_v[c, i, tile(j), :].T
                if CFG['wu32']:
                    wt_s[c, j, i * T // 2:(i + 1) * T // 2, :] = pltpu.bitcast(wt, jnp.uint32)
                else:
                    wt_s[c, j, tile(i), :] = wt

    def phase1(c, seq):
        if not CFG['nodma']:
            wait(kvh_copies(c + 1), [q_copy(c)])

            @pl.when(c + 2 < ND)
            def _():
                wait(w_copies(c + 2))
                start(kvh_copies(c + 2))

            @pl.when(c + 3 < ND)
            def _():
                start(w_copies(c + 3))

            @pl.when(c + 3 == ND)
            def _():
                wo_copy.start()

            start([q_copy(c + 1)])
        z = spec_base(c % 2, (c + 1) % 2)
        transpose_w(jnp.minimum(c + 2, ND - 1))
        nk = seq.count('k') + seq.count('K')
        nb = nf = ik = 0
        for ch in seq:
            if ch == 'h':
                fwd_h(c + 1, z)
            elif ch == 'u':
                fwd_u(z)
            elif ch == 'i':
                assert nf == NT
                inverse(c, z)
            elif ch == 'p':
                project(c + 1, nb)
                nb += 1
            elif ch == 'c':
                r = project(c + 1, nb)
                spec_s[0, pl.ds(z[0] + SP_PACE, 8), :] = r[3 * T - 8:, 0:T]
                nb += 1
            elif ch in 'kK':
                last = kv_prep(c + 1, ik * NT // nk, (ik + 1) * NT // nk)
                if ch == 'k':
                    spec_s[0, pl.ds(z[0] + SP_PACE, 8), :] = last
                ik += 1
            elif ch == 'v':
                chunk_conv(c, z, nf)
                nf += 1
        assert nb * PN == S
        if not CFG['nodma'] and not CFG['lateout']:
            outa_copy(c).start()

    def body1(c, carry):
        phase1(c, CFG['p1seq'])
        return carry

    steps = [(s, int(i), j) for s in range(NSEG) for i in CFG['orders'][s]
             for j in range(int(i) + 1)]
    n = len(steps)
    per_seg = n // NSEG
    first = [t for t in range(n) if steps[t][2] == 0]
    if CFG['hmajor']:
        cells = [(t0 + j, h) for t0 in first for h in range(GH) for j in range(steps[t0][1] + 1)]
    else:
        cells = [(t, h) for t in range(n) for h in range(GH)]
    lag, lag2, nc = CFG['lag'], CFG['lag2'], CFG['nc']
    tpl = L // T
    def cell(m):
        t, h = cells[m]
        return steps[t] + (h,)

    flag = CFG['flag']
    late = [steps[t] for t in range(n - flag, n)]
    done_late = {(s, i) for s, i, j in late}
    acc_keys = sorted({(s, i, h) for s, i, j in steps[:n - flag] if (s, i) in done_late
                       for h in range(GH)})
    ret_keys = sorted(k for k in done_late if k[0] > 0)

    class Group:
        def __init__(self, g):
            self.g = g
            self.r0 = g * GR if isinstance(g, int) else pl.multiple_of(g * GR, 16)
            self.rows = pl.ds(self.r0, GR)
            self.kn, self.va, self.w = {}, {}, {}
            self.maxes, self.accs, self.rets, self.mems = {}, {}, {}, {}
            self.lo = self.hi = None

    r16 = lambda: lax.broadcasted_iota(jnp.int32, (16, T), 0)
    low4 = lambda: lax.broadcasted_iota(jnp.int32, (8, T), 0) < 4

    def pad_rows(x):
        return jnp.concatenate([x, jnp.zeros((T - GR, x.shape[1]), x.dtype)], axis=0)

    def keys(G, a):
        if a not in G.kn:
            G.kn[a] = pad_rows(kt_s[a, G.rows, :]).T
        return G.kn[a]

    def values(G, a):
        if a not in G.va:
            vt = vt_s[a, G.rows, :]
            b = [vt[16 * m:16 * m + 16] for m in range(5)]
            lo = low4()
            one2 = jnp.full((8, T), 0x3F803F80, jnp.uint32)

            def top(x):
                return pltpu.bitcast(jnp.where(lo, pltpu.bitcast(x, jnp.uint32), one2), BF16)

            def bottom(x):
                return pltpu.bitcast(jnp.where(lo, one2, pltpu.bitcast(x, jnp.uint32)), BF16)

            G.va[a] = [
                jnp.concatenate([b[0], top(b[1])], axis=0),
                jnp.concatenate([b[1], top(b[2])], axis=0),
                jnp.concatenate([bottom(b[2]), b[3]], axis=0),
                jnp.concatenate([bottom(b[3]), b[4]], axis=0),
            ]
        return G.va[a]

    def queries(G, a):
        if a not in G.w:
            r16 = lax.broadcasted_iota(jnp.int32, (16, T), 0)
            ws = []
            for h in range(GH):
                lo = (h * DH - 16 * h) // 2
                keep = (r16 >= lo) & (r16 < lo + DH // 2)
                blk = pltpu.bitcast(qs_s[a, pl.ds(G.r0 + 16 * h, 32), :], jnp.uint32)
                blk = pltpu.bitcast(jnp.where(keep, blk, jnp.zeros_like(blk)), BF16)
                pieces = [blk, jnp.zeros((T - 32 - 16 * h, T), BF16)]
                if h:
                    pieces = [jnp.zeros((16 * h, T), BF16)] + pieces
                ws.append(jnp.concatenate(pieces, axis=0))
            G.w[a] = jnp.concatenate(ws, axis=1)
        return G.w[a]

    def recip(d):
        r = pl.reciprocal(d, approx=True)
        return r * (2.0 - d * r)

    def assemble(parts):
        lo = low4()
        u = [[p[8 * m:8 * m + 8] for m in range(4)] for p in parts]
        vals = [u[0][0], u[0][1], jnp.where(lo, u[0][2], u[1][0]), u[1][1], u[1][2],
                u[2][1], u[2][2], jnp.where(lo, u[2][3], u[3][1]), u[3][2], u[3][3]]
        return jnp.concatenate(vals, axis=0), (u[0][3], u[1][3], u[2][0], u[3][0])

    def spread(d):
        lo = low4()
        return jnp.concatenate(
            [d[0], d[0], jnp.where(lo, d[0], d[1]), d[1], d[1],
             d[2], d[2], jnp.where(lo, d[2], d[3]), d[3], d[3]], axis=0)

    def update(G, s):
        va = jnp.concatenate(
            [jnp.concatenate(values(G, s * tpl + j), axis=0) for j in range(tpl)], axis=1)
        pk = jnp.concatenate(
            [pad_rows(pk_s[s * tpl + j, G.rows, :]) for j in range(tpl)], axis=1)
        upd = _dot_nt(va, pk)
        lane = lax.broadcasted_iota(jnp.int32, (32, T), 1)
        upd = jnp.concatenate([
            jnp.where((lane >= h * DH) & (lane < (h + 1) * DH), upd[32 * h:32 * h + 32], 0.0)
            for h in range(GH)], axis=0)
        G.mems[s + 1] = upd if s == 0 else G.mems[s] + upd

    def retrieve(G, s):
        pq = jnp.concatenate(
            [pad_rows(pq_s[(s - 1) * tpl + i, G.rows, :]) for i in range(tpl)], axis=1)
        ret = _dot(G.mems[s].astype(BF16), pq)
        gate = gate_s[G.rows, :]
        for i in range(tpl):
            vals, dens = assemble([ret[32 * h:32 * h + 32, tile(i)] for h in range(GH)])
            G.rets[(s, i)] = vals * (gate * spread([recip(d + 1e-6) for d in dens]))

    def finish(G, s, i):
        vals, dens = assemble([G.accs[(s, i, h)] for h in range(GH)])
        if G.lo is not None:
            for d in dens:
                G.lo, G.hi = jnp.minimum(G.lo, d), jnp.maximum(G.hi, d)
        o = vals * ((1.0 - gate_s[G.rows, :]) * spread([recip(d) for d in dens]))
        if s > 0:
            o = o + G.rets[(s, i)]
        ot_s[s * tpl + i, G.rows, :] = o.astype(BF16)

    def qk_dot(G, t):
        s, i, j = steps[t]
        return _dot(keys(G, s * tpl + j), queries(G, s * tpl + i))

    def qk_store(G, t, raw, c, zs):
        s, i, j = steps[t]
        r0, r1 = c * T // nc, (c + 1) * T // nc
        causal = (r0 + lax.broadcasted_iota(jnp.int32, (r1 - r0, T), 0)
                  <= lax.broadcasted_iota(jnp.int32, (r1 - r0, T), 1))
        ms = []
        for h in range(GH):
            sc = raw[r0:r1, tile(h)]
            if j == i:
                sc = jnp.where(causal, sc, NEG)
            s_ref[pl.ds(zs + ((t % RS) * GH + h) * T + r0, r1 - r0), :] = sc
            m8 = sc[0:8]
            for r in range(1, (r1 - r0) // 8):
                m8 = jnp.maximum(m8, sc[8 * r:8 * r + 8])
            if j > 0 or c > 0:
                m8 = jnp.maximum(G.maxes[(s, i)][h], m8)
            if j == i and c == nc - 1:
                m8 = jnp.broadcast_to(jnp.max(m8, axis=0, keepdims=True), (8, T))
            ms.append(m8)
        G.maxes[(s, i)] = ms

    def exp_part(G, t, c, zl, ps):
        per = GH * T // nc
        slot, r0 = (c * per) // T, (c * per) % T
        tq, h = cells[t * GH + slot]
        s, i, j = steps[tq]
        m = jnp.concatenate([G.maxes[(s, i)][h]] * (per // 8), axis=0)
        sc = s_ref[pl.ds(zl + ((tq % RS) * GH + h) * T + r0, per), :]
        p_refs[t % RP][pl.ds(ps + slot * T + r0, per), :] = jnp.exp2(sc - m).astype(BF16)

    def pv_step(G, t, plo):
        for slot in range(GH):
            s, i, j, h = cell(t * GH + slot)
            r = _dot(values(G, s * tpl + j)[h], p_refs[t % RP][pl.ds(plo + slot * T, T), :])
            G.accs[(s, i, h)] = r if j == 0 else G.accs[(s, i, h)] + r
            if j == i and h == GH - 1:
                finish(G, s, i)

    def exp_direct(t, raw, ps):
        s, i, j = steps[t]
        causal = (lax.broadcasted_iota(jnp.int32, (T, T), 0)
                  <= lax.broadcasted_iota(jnp.int32, (T, T), 1))
        for h in range(GH):
            p = jnp.exp2(raw[:, tile(h)])
            if j == i:
                p = jnp.where(causal, p, 0.0)
            p_refs[t % RP][pl.ds(ps + h * T, T), :] = p.astype(BF16)

    def pv_direct(G, t, plo):
        s, i, j = steps[t]
        for h in range(GH):
            r = _dot(values(G, s * tpl + j)[h], p_refs[t % RP][pl.ds(plo + h * T, T), :])
            G.accs[(s, i, h)] = r if j == 0 else G.accs[(s, i, h)] + r
        if j == i:
            finish(G, s, i)

    def attn_base():
        return ([pl.multiple_of(zero_ref[m], 8) for m in range(2)]
                + [pl.multiple_of(zero_ref[m], 16) for m in range(2, 4)])

    def adopt(g, state):
        P = Group(g)
        P.accs = dict(zip(acc_keys, state[0]))
        P.rets = dict(zip(ret_keys, state[1]))
        P.lo, P.hi = state[2]
        return P

    def memory_steps(G, t):
        s = t // per_seg
        if t % per_seg == CFG['memat'] and s > 0:
            retrieve(G, s)
        if t % per_seg == CFG['updat'] and s < NSEG - 1:
            update(G, s)

    def attention(g, state):
        _, _, ps, plo = attn_base()
        G = Group(g)
        if isinstance(g, int):
            P = None
            G.lo = G.hi = jnp.ones((8, T), F32)
        else:
            P = adopt(g - 1, state)
        G.kn[0] = kn0_s[...]
        for t in range(n):
            raw = qk_dot(G, t)
            memory_steps(G, t)
            if t >= flag:
                pv_direct(G, t - flag, plo)
            elif P is not None:
                pv_direct(P, n + t - flag, plo)
                G.lo, G.hi = P.lo, P.hi
            exp_direct(t, raw, ps)
            if t in CFG['convat'] and P is not None:
                z = spec_base((ND - 1) % 2, 0)
                spec_s[0, pl.ds(z[0] + SP_PACE, 8), :] = raw[T - 8:, 0:T]
                chunk_conv(ND - 1, z, ((g - 1) * len(CFG['convat']) + CFG['convat'].index(t)) % NT)
            if t == n - 4 and P is not None:
                kn0_s[...] = keys(Group(jnp.minimum(g + 1, NGRP - 1)), 0)
        return ([G.accs[k] for k in acc_keys], [G.rets[k] for k in ret_keys], (G.lo, G.hi))

    def attention_true_max(g, carry):
        zs, zl, ps, plo = attn_base()
        G = Group(g)
        for t in range(n + lag2):
            if t < n:
                raw = qk_dot(G, t)
                memory_steps(G, t)
            if t >= lag2:
                pv_step(G, t - lag2, plo)
            for c in range(nc):
                if t < n:
                    qk_store(G, t, raw, c, zs)
                if lag <= t < n + lag:
                    exp_part(G, t - lag, c, zl, ps)
        return carry

    def out_proj(b):
        o = jnp.concatenate(
            [jnp.concatenate([ot_s[b * (OB // T) + m, tile(j), :].T for j in range(ND)], axis=1)
             for m in range(OB // T)], axis=0)
        r = _dot(o, wo_v[...])
        yb_s[b] = r.astype(BF16)
        return r

    init = ([jnp.ones((32, T), F32) for _ in acc_keys],
            [jnp.zeros((GR, T), F32) for _ in ret_keys],
            (jnp.ones((8, T), F32), jnp.ones((8, T), F32)))
    mark('S1_wait0')
    wait(w_copies(0))
    transpose_w(0)
    wait([x_copy(0)])
    mark('S2_proj0')
    start([x_copy(1)], small)
    project(0, 0)
    wait([x_copy(1)], small)
    start([x_copy(2)])
    small_tables()
    project(0, 1)
    wait([x_copy(2)])
    start([x_copy(3)])
    project(0, 2)
    mark('S3_proj0b')
    wait([x_copy(3)])
    start(kvh_copies(0), w_copies(1), kvh_copies(1), [q_copy(0)], w_copies(2))
    kn0_s[...] = keys(Group(0), 0)
    project(0, 3)
    mark('S4_attn0')
    state = attention(0, None) if CFG['only'] != 'p1' else init
    mark('S5_fwd0')
    wait(kvh_copies(0), w_copies(1))
    z = spec_base(1, 0)
    fwd_h(0, z)
    kv_prep(0)
    transpose_w(1)
    fwd_u(z)
    if CFG['nodma']:
        mark('S5b_dma')
        for c in (3, 4):
            start(kvh_copies(c), w_copies(c))
        start([q_copy(2), q_copy(3), q_copy(4), wo_copy])
        for c in (1, 2, 3, 4):
            wait(kvh_copies(c), [q_copy(c - 1)])
        for c in (2, 3, 4):
            wait(w_copies(c))
    mark('S6_p1loop')

    def body1(c, carry):
        phase1(c, CFG['p1seq'])
        return carry

    lax.fori_loop(0, ND - 1, body1, 0)
    mark('S7_p2')
    if CFG['nodma'] or CFG['lateout']:
        start([outa_copy(c) for c in range(ND - 1)])
    kn0_s[...] = keys(Group(1), 0)
    if CFG['only'] != 'p1':
        state = lax.fori_loop(1, NGRP, attention, state)

    mark('S7b_check')
    _, _, ps, plo = attn_base()
    P = adopt(NGRP - 1, state)
    for t in range(n - flag, n):
        pv_direct(P, t, plo)
    safe = (jnp.min(P.lo) >= 2.0 ** -SUM_LOG2) & (jnp.max(P.hi) <= 2.0 ** SUM_LOG2)

    @pl.when(jnp.logical_not(safe))
    def _():
        lax.fori_loop(0, NGRP, attention_true_max, 0)

    mark('S8_p3')
    wait([wo_copy, q_copy(ND - 1)])
    z = spec_base((ND - 1) % 2, 0)
    nb = nf = 0
    for ch in CFG['p3seq']:
        if ch == 'v':
            chunk_conv(ND - 1, z, nf)
            nf += 1
        elif ch == 'i':
            inverse(ND - 1, z)
        elif ch == 'a':
            outa_copy(ND - 1).start()
        elif ch in 'pc':
            r = out_proj(nb)
            if ch == 'c':
                spec_s[0, pl.ds(z[0] + SP_PACE, 8), :] = r[OB - 8:, D - T:]
            nb += 1
        elif ch.isdigit():
            outb_copy(int(ch)).start()
    assert nb == S // OB and nf == NT
    mark('SA_final')

    for c in range(ND):
        outa_copy(c).wait()
    for b in range(S // OB):
        outb_copy(b).wait()
    mark(None)


@jax.jit
def pallas_concat_heads__ssm_conv_h3__memory_aug_infini_attn__prompt_kernel(
    A_q: jax.Array,
    A_k: jax.Array,
    A_v: jax.Array,
    A_shift_k: jax.Array,
    A_ssm_k: jax.Array,
    A_ssm_D: jax.Array,
    B_x: jax.Array,
    B_wq: jax.Array,
    B_wk: jax.Array,
    B_wv: jax.Array,
    B_wo: jax.Array,
    B_beta: jax.Array,
):
    hbm = pl.BlockSpec(memory_space=pltpu.MemorySpace.HBM)
    vmem = pltpu.VMEM
    dma = pltpu.SemaphoreType.DMA
    out = pl.pallas_call(
        _kernel,
        out_shape=jax.ShapeDtypeStruct((S, 2 * D), BF16),
        in_specs=[pl.BlockSpec(memory_space=pltpu.SMEM)] + [hbm] * 14,
        out_specs=hbm,
        scratch_shapes=[
            vmem((ND, S, T), BF16),
            vmem((ND, S, T), BF16),
            vmem((ND, S, T), BF16),
            vmem((KS, D), BF16),
            vmem((ND, T, S), BF16),
            vmem((ND, T), BF16),
            vmem((S, D), BF16),
            vmem((ND, 3, D, T), BF16),
            vmem((D, D), BF16),
            vmem((1, H), BF16),
            vmem((2 * T, T), BF16),
            vmem((T, 2 * T), BF16),
            vmem((ND, ND, 3 * T // 2, T), jnp.uint32) if CFG['wu32'] else vmem((ND, ND, 3 * T, T), BF16),
            vmem((ND, 8, T), F32),
            vmem((D, T), F32),
            vmem((S + 8, T), F32),
            vmem((S, T), BF16),
            vmem((2 * NT, SP_PACE + 8, T), F32),
            vmem((NT, 2 * T, T), BF16),
            vmem((ND, S, T), BF16),
            vmem((NT, D, T), BF16),
            vmem((NT - L // T, D, T), BF16),
            vmem((NT, D, T), BF16),
            vmem((NT - L // T, D, T), BF16),
            vmem((NT, D, T), BF16),
            vmem((NT, D, T), BF16),
            vmem((S // OB, OB, D), BF16),
            vmem((CFG['rs'] * GH * T, T), F32),
            vmem((T, T), BF16),
            vmem((ND, S // 2, T), jnp.uint32),
            dma((6,)),
            dma((4, ND)),
            dma((3, ND)),
            dma((NSEG,)),
            dma((ND,)),
            dma((S // OB,)),
        ] + [vmem((GH * T, T), BF16)] * CFG['rp'],
        compiler_params=pltpu.CompilerParams(vmem_limit_bytes=100 * 1024 * 1024),
        name="h3_infini_concat",
    )(
        jnp.asarray(np.zeros((8,), np.int32)),
        A_q.reshape(S, D), A_k.reshape(S, D), A_v.reshape(S, D), A_shift_k.T, A_ssm_k,
        A_ssm_D.reshape(ND, T), B_x.reshape(S, D), B_wq, B_wk, B_wv, B_wo,
        B_beta.reshape(1, H),
        jnp.asarray(_FWD, dtype=BF16), jnp.asarray(_INV, dtype=BF16),
    )
    return out.reshape(1, S, 2 * D)
```

```python
import math

import jax
import jax.numpy as jnp
import numpy as np
from jax import lax
from jax.experimental import pallas as pl
from jax.experimental.pallas import tpu as pltpu

S = 2048
D = 640
H = 32
DH = D // H
NSEG = 4
L = S // NSEG
KS = 4
T = 128
NT = S // T
TPL = L // T
ND = D // T
GH = 4
GR = GH * DH
NGRP = H // GH
OB = 256
RS, RP = 8, 4
Q_SCALE = DH ** -0.5 * math.log2(math.e)
NEG = -1e30
SUM_LOG2 = 30

F32 = jnp.float32
BF16 = jnp.bfloat16
U32 = jnp.uint32

SP_H, SP_U, SP_PACE = 0, 2 * T, 4 * T

PHASE1_ORDER = "vhvvvkkcvvvvkkcvvvvcvvvvpiu"
PHASE3_ORDER = "txvvcvvc0vvc1vvvc2vvvc3vvvvp4i5ap6p7"

STEPS = [(s, i, j) for s in range(NSEG) for i in range(TPL) for j in range(i + 1)]
NSTEP = len(STEPS)
PV_LAG = 3
PV_CARRY = 2
_LATE = {st[:2] for st in STEPS[NSTEP - PV_CARRY:]}
_ACC_KEYS = sorted({(s, i, h) for s, i, _ in STEPS[:NSTEP - PV_CARRY]
                    if (s, i) in _LATE for h in range(GH)})
_RET_KEYS = sorted(k for k in _LATE if k[0] > 0)
_CELLS = [(t + j, h) for t, (_, i, j0) in enumerate(STEPS) if j0 == 0
          for h in range(GH) for j in range(i + 1)]
EXP_LAG, MAX_PV_LAG = 4, 6


def _dft_matrices():
    k = np.arange(T, dtype=np.float64)[:, None]
    t = np.arange(T, dtype=np.float64)[None, :]
    theta = 2.0 * np.pi * (k + 0.25) * t / T
    re = np.cos(theta).reshape(T // 8, 1, 8, T)
    im = np.sin(theta).reshape(T // 8, 1, 8, T)
    fwd = np.concatenate([re, im], axis=1).reshape(2 * T, T)
    return (fwd.astype(np.float32).astype(BF16),
            (fwd.T / T).astype(np.float32).astype(BF16))


_FWD, _INV = _dft_matrices()
_ZEROS = np.zeros((8,), np.int32)


def _dot(a, b):
    return jnp.dot(a, b, preferred_element_type=F32)


def _dot_nt(a, b):
    return lax.dot_general(a, b, (((1,), (1,)), ((), ())), preferred_element_type=F32)


def _phi(t):
    return jnp.where(t > 0, t + 1.0, jnp.exp(t))


def _tile(i):
    return slice(i * T, (i + 1) * T)


def _iota(shape, axis):
    return lax.broadcasted_iota(jnp.int32, shape, axis)


def _add(xs, ys):
    return [x + y for x, y in zip(xs, ys)]


def _causal_complex(ur, ui, gr, gi):
    re, im = [], []
    for a in range(len(ur)):
        x = ur[0] * gr[a] - ui[0] * gi[a]
        y = ur[0] * gi[a] + ui[0] * gr[a]
        for j in range(1, a + 1):
            x = x + (ur[j] * gr[a - j] - ui[j] * gi[a - j])
            y = y + (ur[j] * gi[a - j] + ui[j] * gr[a - j])
        re.append(x)
        im.append(y)
    return re, im


class _Group:
    def __init__(self, g, paired):
        self.r0 = g * GR if isinstance(g, int) else pl.multiple_of(g * GR, 16)
        self.rows = pl.ds(self.r0, GR)
        self.paired = paired
        self.kn, self.va, self.w, self.w2 = {}, {}, {}, {}
        self.maxes, self.accs, self.rets, self.mems = {}, {}, {}, {}
        self.lo = self.hi = None


def _kernel(
    zero_ref, q_hbm, k_hbm, v_hbm, shift_hbm, h_hbm, d_hbm, x_hbm,
    wq_hbm, wk_hbm, wv_hbm, wo_hbm, beta_hbm, fwd_hbm, inv_hbm,
    out_hbm,
    q_v, k_v, v_v, shift_v, h_v, d_v, x_v, w_v, wo_v, beta_v, fwd_v, inv_v,
    wt_s, xu_s, taps_s, gate_s, kpad_s, kv_s, spec_s, yf_s, ya_s,
    qs_s, pq_s, kt_s, pk_s, vt_s, ot_s, yb_s, s_ring, kn0_s,
    in_sem, slab_sem, w_sem, x_sem, outa_sem, outb_sem, *p_ring,
):
    def slab(c):
        return pl.ds(c * T if isinstance(c, int) else pl.multiple_of(c * T, T), T)

    def kvh_copies(c):
        return (
            pltpu.make_async_copy(k_hbm.at[:, slab(c)], k_v.at[c], slab_sem.at[0, c]),
            pltpu.make_async_copy(v_hbm.at[:, slab(c)], v_v.at[c], slab_sem.at[1, c]),
            pltpu.make_async_copy(h_hbm.at[slab(c), :], h_v.at[c], slab_sem.at[2, c]),
        )

    def q_copy(c):
        return [pltpu.make_async_copy(q_hbm.at[:, slab(c)], q_v.at[c], slab_sem.at[3, c])]

    def w_copies(c):
        return [pltpu.make_async_copy(w.at[:, slab(c)], w_v.at[c, i], w_sem.at[i, c])
                for i, w in enumerate((wq_hbm, wk_hbm, wv_hbm))]

    def x_copy(b):
        rows = pl.ds(b * L, L)
        return [pltpu.make_async_copy(x_hbm.at[rows, :], x_v.at[rows, :], x_sem.at[b])]

    def outa_copy(c):
        return [pltpu.make_async_copy(ya_s.at[c], out_hbm.at[:, slab(c)], outa_sem.at[c])]

    def outb_copy(b):
        dst = out_hbm.at[pl.ds(b * OB, OB), pl.ds(D, D)]
        return [pltpu.make_async_copy(yb_s.at[b], dst, outb_sem.at[b])]

    small = [pltpu.make_async_copy(src, dst, in_sem.at[i]) for i, (src, dst) in enumerate(
        [(shift_hbm, shift_v), (d_hbm, d_v), (beta_hbm, beta_v),
         (fwd_hbm, fwd_v), (inv_hbm, inv_v)])]
    wo_copy = [pltpu.make_async_copy(wo_hbm, wo_v, in_sem.at[len(small)])]

    def start(*groups):
        for group in groups:
            for copy in group:
                copy.start()

    def wait(*groups):
        for group in groups:
            for copy in group:
                copy.wait()

    def zeros(n0, n1, align):
        return [pl.multiple_of(zero_ref[n], align) for n in range(n0, n1)]

    def small_tables():
        shift, skip = shift_v[...].astype(F32), d_v[...].astype(F32)
        for c in range(ND):
            taps_s[c, 0:KS, :] = shift[:, _tile(c)]
            taps_s[c, KS:KS + 1, :] = skip[c:c + 1, :]
        g_row = jax.nn.sigmoid(beta_v[...].astype(F32))
        row, head = _iota((D, H), 0), _iota((D, H), 1)
        own = (row >= head * DH) & (row < (head + 1) * DH)
        g_col = jnp.sum(jnp.where(own, g_row, 0.0), axis=1, keepdims=True)
        gate_s[...] = jnp.broadcast_to(g_col, (D, T))

    def tap(c, j):
        return taps_s[c, j:j + 1, :]

    def kv_prep(c, a0=0, a1=NT):
        w = [tap(c, j) for j in range(KS)]
        kpad_s[8 + a0 * T:8 + a1 * T, :] = k_v[c, a0 * T:a1 * T, :].astype(F32)
        for a in range(a0, a1):
            acc = None
            for j in range(KS):
                term = kpad_s[8 + a * T - j:8 + (a + 1) * T - j, :] * w[j]
                acc = term if acc is None else acc + term
            kv = acc * v_v[c, _tile(a), :].astype(F32)
            kv_s[_tile(a), :] = kv.astype(BF16)
        return kv[T - 8:]

    def store_spectrum(c, z, off, a, re, im):
        for f in range(T // 8):
            for m, part in enumerate((re, im)):
                rows = pl.ds(z[0] + off + 16 * f + 8 * m, 8)
                spec_s[(c % 2) * NT + a, rows, :] = part[f]

    def split(val, a):
        return ([val[16 * f:16 * f + 8, _tile(a)] for f in range(T // 8)],
                [val[16 * f + 8:16 * f + 16, _tile(a)] for f in range(T // 8)])

    def fwd_h(c, z):
        h_rows = jnp.concatenate([h_v[c, :, _tile(a)] for a in range(NT)], axis=0)
        val = _dot_nt(fwd_v[...], h_rows)
        skip = tap(c, KS)
        prev = None
        for a in range(NT):
            hr, hi = split(val, a)
            if prev is None:
                hr = [x + skip for x in hr]
                gr, gi = hr, hi
            else:
                gr = _add(hr, prev[1])
                gi = [x - y for x, y in zip(hi, prev[0])]
            prev = (hr, hi)
            store_spectrum(c, z, SP_H, a, gr, gi)

    def fwd_u(c, z):
        u = jnp.concatenate([kv_s[_tile(a), :] for a in range(NT)], axis=1)
        val = _dot(fwd_v[...], u)
        for a in range(NT):
            store_spectrum(c, z, SP_U, a, *split(val, a))

    def pace(z, val):
        spec_s[0, pl.ds(z[0] + SP_PACE, 8), :] = val

    def chunk_conv(c, z, f):
        def load(off):
            return [spec_s[(c % 2) * NT + a, pl.ds(z[1] + off + 16 * f, 8), :]
                    for a in range(NT)]

        gr, gi, ur, ui = load(SP_H), load(SP_H + 8), load(SP_U), load(SP_U + 8)
        er, ei = _causal_complex(ur[0::2], ui[0::2], gr[0::2], gi[0::2])
        o_r, o_i = _causal_complex(ur[1::2], ui[1::2], gr[1::2], gi[1::2])
        mr, mi = _causal_complex(_add(ur[0::2], ur[1::2]), _add(ui[0::2], ui[1::2]),
                                 _add(gr[0::2], gr[1::2]), _add(gi[0::2], gi[1::2]))
        re, im = [None] * NT, [None] * NT
        for m in range(NT // 2):
            re[2 * m] = er[m] if m == 0 else er[m] + o_r[m - 1]
            im[2 * m] = ei[m] if m == 0 else ei[m] + o_i[m - 1]
            re[2 * m + 1] = mr[m] - er[m] - o_r[m]
            im[2 * m + 1] = mi[m] - ei[m] - o_i[m]
        for a in range(NT):
            yf_s[a, 16 * f:16 * f + 16, :] = jnp.concatenate(
                [re[a], im[a]], axis=0).astype(BF16)

    def inverse(c):
        y = _dot(inv_v[...], jnp.concatenate([yf_s[a] for a in range(NT)], axis=1))
        for a in range(NT):
            ya_s[c, _tile(a), :] = (
                q_v[c, _tile(a), :].astype(F32) * y[:, _tile(a)]).astype(BF16)

    def transpose_w(c):
        for i in range(3):
            for j in range(ND):
                wt_s[c, j, i * T // 2:(i + 1) * T // 2, :] = pltpu.bitcast(
                    w_v[c, i, _tile(j), :].T, U32)

    def project(c, b):
        w = jnp.concatenate([pltpu.bitcast(wt_s[c, j], BF16) for j in range(ND)], axis=1)
        half = slice(b * L // 2, (b + 1) * L // 2)
        if isinstance(c, int):
            xb = x_v[b * L:(b + 1) * L, :]
            for j in range(ND):
                xu_s[j, half, :] = pltpu.bitcast(xb[:, _tile(j)], U32)
        else:
            xb = jnp.concatenate(
                [pltpu.bitcast(xu_s[j, half, :], BF16) for j in range(ND)], axis=1)
        r = _dot_nt(w, xb)
        rows = slab(c)
        for m in range(TPL):
            a = b * TPL + m
            qf, kf, vf = (r[_tile(i), _tile(m)] for i in range(3))
            qs_s[a, rows, :] = (qf * Q_SCALE).astype(BF16)
            kb = kf.astype(BF16)
            kt_s[a, rows, :] = kb
            vt_s[a, rows, :] = vf.astype(BF16)
            if b > 0:
                pq_s[a - TPL, rows, :] = _phi(qf.astype(BF16).astype(F32)).astype(BF16)
            if b < NSEG - 1:
                pk_s[a, rows, :] = _phi(kb.astype(F32)).astype(BF16)
        return r[3 * T - 8:, 0:T]

    def phase1(c, carry):
        wait(kvh_copies(c + 1), q_copy(c))

        @pl.when(c + 2 < ND)
        def _():
            wait(w_copies(c + 2))
            start(kvh_copies(c + 2))

        @pl.when(c + 3 < ND)
        def _():
            start(w_copies(c + 3))

        @pl.when(c + 3 == ND)
        def _():
            start(wo_copy)

        start(q_copy(c + 1))
        z = zeros(0, 2, 8)
        transpose_w(jnp.minimum(c + 2, ND - 1))
        halves = PHASE1_ORDER.count("k")
        nb = nf = nk = 0
        for ch in PHASE1_ORDER:
            if ch == "h":
                fwd_h(c + 1, z)
            elif ch == "u":
                fwd_u(c + 1, z)
            elif ch == "i":
                inverse(c)
            elif ch in "pc":
                last = project(c + 1, nb)
                nb += 1
                if ch == "c":
                    pace(z, last)
            elif ch == "k":
                pace(z, kv_prep(c + 1, nk * NT // halves, (nk + 1) * NT // halves))
                nk += 1
            else:
                chunk_conv(c, z, nf)
                nf += 1
        assert nb == NSEG and nf == NT
        start(outa_copy(c))
        return carry

    def low4():
        return _iota((8, T), 0) < 4

    def pad_rows(x):
        return jnp.concatenate([x, jnp.zeros((T - GR, x.shape[1]), x.dtype)], axis=0)

    def keys(G, a):
        if a not in G.kn:
            G.kn[a] = pad_rows(kt_s[a, G.rows, :]).T
        return G.kn[a]

    def values(G, a):
        if a not in G.va:
            vt = vt_s[a, G.rows, :]
            b = [vt[16 * m:16 * m + 16] for m in range(5)]
            lo = low4()
            one2 = jnp.full((8, T), 0x3F803F80, U32)

            def top(x):
                return pltpu.bitcast(jnp.where(lo, pltpu.bitcast(x, U32), one2), BF16)

            def bottom(x):
                return pltpu.bitcast(jnp.where(lo, one2, pltpu.bitcast(x, U32)), BF16)

            G.va[a] = [jnp.concatenate(p, axis=0) for p in (
                [b[0], top(b[1])], [b[1], top(b[2])],
                [bottom(b[2]), b[3]], [bottom(b[3]), b[4]])]
        return G.va[a]

    def queries(G, a):
        if a not in G.w:
            pair = _iota((16, T), 0)
            blks = []
            for h in range(GH):
                lo = (h * DH - 16 * h) // 2
                blk = pltpu.bitcast(qs_s[a, pl.ds(G.r0 + 16 * h, 32), :], U32)
                blk = jnp.where((pair >= lo) & (pair < lo + DH // 2), blk,
                                jnp.zeros_like(blk))
                if G.paired and h % 2:
                    blk = pltpu.roll(blk, T // 2, 1)
                blks.append(blk)

            def place(blk, h):
                rest = T - 16 * h - 2 * blk.shape[0]
                pieces = [pltpu.bitcast(blk, BF16), jnp.zeros((rest, T), BF16)]
                if h:
                    pieces = [jnp.zeros((16 * h, T), BF16)] + pieces
                return jnp.concatenate(pieces, axis=0)

            G.w[a] = jnp.concatenate([place(blks[h], h) for h in range(GH)], axis=1)
            if G.paired:
                left = _iota((24, T), 1) < T // 2
                zero = jnp.zeros((8, T), U32)
                G.w2[a] = jnp.concatenate([
                    place(jnp.where(left, jnp.concatenate([zero, blks[h + 1]], axis=0),
                                    jnp.concatenate([blks[h], zero], axis=0)), h)
                    for h in range(0, GH, 2)], axis=1)
        return G.w[a]

    def update(G, s):
        ones = jnp.ones((16, T), BF16)
        va = jnp.concatenate(
            [jnp.concatenate([vt_s[s * TPL + j, G.rows, :], ones], axis=0)
             for j in range(TPL)], axis=1)
        pk = jnp.concatenate(
            [pad_rows(pk_s[s * TPL + j, G.rows, :]) for j in range(TPL)], axis=1)
        row, lane = _iota((GR + 16, T), 0), _iota((GR + 16, T), 1)
        keep = None
        for h in range(GH):
            mine = (((row >= h * DH) & (row < (h + 1) * DH))
                    | ((row >= GR + 4 * h) & (row < GR + 4 * h + 4)))
            mine = mine & (lane >= h * DH) & (lane < (h + 1) * DH)
            keep = mine if keep is None else keep | mine
        upd = jnp.where(keep, _dot_nt(va, pk), 0.0)
        G.mems[s + 1] = upd if s == 0 else G.mems[s] + upd

    def retrieve(G, s):
        pq = jnp.concatenate(
            [pad_rows(pq_s[(s - 1) * TPL + i, G.rows, :]) for i in range(TPL)], axis=1)
        ret = _dot(G.mems[s].astype(BF16), pq)
        gate = gate_s[G.rows, :]
        lo = low4()
        for i in range(TPL):
            inv = []
            for m in range(2):
                r = 1.0 / (ret[GR + 8 * m:GR + 8 * m + 8, _tile(i)] + 1e-6)
                other = pltpu.roll(r, 4, 0)
                first, second = jnp.where(lo, r, other), jnp.where(lo, other, r)
                inv += [first, first, r, second, second]
            G.rets[(s, i)] = ret[:GR, _tile(i)] * (gate * jnp.concatenate(inv, axis=0))

    def memory_steps(G, t):
        s, k = divmod(t, NSTEP // NSEG)
        if k == 2 and s > 0:
            retrieve(G, s)
        if k == 6 and s < NSEG - 1:
            update(G, s)

    def finish(G, s, i):
        accs = [G.accs[(s, i, h)] for h in range(GH)]
        if G.paired:
            accs = [pltpu.roll(x, T // 2, 1) if h % 2 else x for h, x in enumerate(accs)]
        u = [[x[8 * m:8 * m + 8] for m in range(4)] for x in accs]
        lo = low4()
        vals = jnp.concatenate(
            [u[0][0], u[0][1], jnp.where(lo, u[0][2], u[1][0]), u[1][1], u[1][2],
             u[2][1], u[2][2], jnp.where(lo, u[2][3], u[3][1]), u[3][2], u[3][3]], axis=0)
        sums = (u[0][3], u[1][3], u[2][0], u[3][0])
        if G.lo is not None:
            for d in sums:
                G.lo, G.hi = jnp.minimum(G.lo, d), jnp.maximum(G.hi, d)
        r = [1.0 / d for d in sums]
        inv = jnp.concatenate(
            [r[0], r[0], jnp.where(lo, r[0], r[1]), r[1], r[1],
             r[2], r[2], jnp.where(lo, r[2], r[3]), r[3], r[3]], axis=0)
        o = vals * ((1.0 - gate_s[G.rows, :]) * inv)
        if s > 0:
            o = o + G.rets[(s, i)]
        ot_s[s * TPL + i, G.rows, :] = o.astype(BF16)

    def accumulate(G, s, i, j, h, p):
        r = _dot(values(G, s * TPL + j)[h], p)
        G.accs[(s, i, h)] = r if j == 0 else G.accs[(s, i, h)] + r

    def qk_direct(G, t):
        s, i, j = STEPS[t]
        kn, w = keys(G, s * TPL + j), queries(G, s * TPL + i)
        if j < i:
            return _dot(kn, w)
        late_keys = _dot(kn[T // 2:], G.w2[s * TPL + i])
        return _dot(kn[:T // 2], w), late_keys

    def exp_direct(t, raw, ps):
        _, i, j = STEPS[t]
        if j < i:
            for h in range(GH):
                p_ring[t % RP][pl.ds(ps + h * T, T), :] = jnp.exp2(
                    raw[:, _tile(h)]).astype(BF16)
            return
        key, lane = _iota((T // 2, T), 0), _iota((T // 2, T), 1)
        qry = (lane, (lane + T // 2) & (T - 1))
        shared = [jnp.exp2(raw[1][:, _tile(m)]) for m in range(GH // 2)]
        for h in range(GH):
            top = jnp.where(key <= qry[h % 2], jnp.exp2(raw[0][:, _tile(h)]), 0.0)
            bot = jnp.where(key + T // 2 <= qry[h % 2], shared[h // 2], 0.0)
            p_ring[t % RP][pl.ds(ps + h * T, T), :] = jnp.concatenate(
                [top, bot], axis=0).astype(BF16)

    def pv_direct(G, t, po):
        s, i, j = STEPS[t]
        for h in range(GH):
            accumulate(G, s, i, j, h, p_ring[t % RP][pl.ds(po + h * T, T), :])
        if j == i:
            finish(G, s, i)

    def adopt(g, state):
        P = _Group(g, True)
        P.accs = dict(zip(_ACC_KEYS, state[0]))
        P.rets = dict(zip(_RET_KEYS, state[1]))
        P.lo, P.hi = state[2]
        return P

    def attention(g, state):
        ps, po = zeros(2, 4, 16)
        G = _Group(g, True)
        if state is None:
            P = None
            G.lo = G.hi = jnp.ones((8, T), F32)
        else:
            P = adopt(g - 1, state)
        G.kn[0] = kn0_s[...]
        done = 0
        for t in range(NSTEP):
            raw = qk_direct(G, t)
            memory_steps(G, t)
            if t < PV_CARRY and P is not None:
                pv_direct(P, NSTEP - PV_CARRY + t, po)
                G.lo, G.hi = P.lo, P.hi
            while done <= (t - PV_LAG if t < NSTEP - 1 else t - PV_CARRY):
                pv_direct(G, done, po)
                done += 1
            exp_direct(t, raw, ps)
            if t == NSTEP - 4 and P is not None:
                kn0_s[...] = keys(_Group(jnp.minimum(g + 1, NGRP - 1), True), 0)
        return ([G.accs[k] for k in _ACC_KEYS], [G.rets[k] for k in _RET_KEYS],
                (G.lo, G.hi))

    def attention_true_max(g, carry):
        zs, zl = zeros(0, 2, 8)
        ps, po = zeros(2, 4, 16)
        G = _Group(g, False)
        part = T // GH
        for t in range(NSTEP + MAX_PV_LAG):
            if t < NSTEP:
                s, i, j = STEPS[t]
                raw = _dot(keys(G, s * TPL + j), queries(G, s * TPL + i))
                memory_steps(G, t)
            if t >= MAX_PV_LAG:
                tp = t - MAX_PV_LAG
                for m in range(GH):
                    tq, h = _CELLS[tp * GH + m]
                    sp, ip, jp = STEPS[tq]
                    accumulate(G, sp, ip, jp, h, p_ring[tp % RP][pl.ds(po + m * T, T), :])
                    if jp == ip and h == GH - 1:
                        finish(G, sp, ip)
            for m in range(GH):
                if t < NSTEP:
                    r0 = m * part
                    causal = r0 + _iota((part, T), 0) <= _iota((part, T), 1)
                    ms = []
                    for h in range(GH):
                        sc = raw[r0:r0 + part, _tile(h)]
                        if j == i:
                            sc = jnp.where(causal, sc, NEG)
                        s_ring[pl.ds(zs + ((t % RS) * GH + h) * T + r0, part), :] = sc
                        m8 = sc[0:8]
                        for r in range(1, part // 8):
                            m8 = jnp.maximum(m8, sc[8 * r:8 * r + 8])
                        if j > 0 or m > 0:
                            m8 = jnp.maximum(G.maxes[(s, i)][h], m8)
                        if j == i and m == GH - 1:
                            m8 = jnp.broadcast_to(
                                jnp.max(m8, axis=0, keepdims=True), (8, T))
                        ms.append(m8)
                    G.maxes[(s, i)] = ms
                if EXP_LAG <= t < NSTEP + EXP_LAG:
                    te = t - EXP_LAG
                    tq, h = _CELLS[te * GH + m]
                    top = jnp.concatenate([G.maxes[STEPS[tq][:2]][h]] * (T // 8), axis=0)
                    sc = s_ring[pl.ds(zl + ((tq % RS) * GH + h) * T, T), :]
                    p_ring[te % RP][pl.ds(ps + m * T, T), :] = jnp.exp2(
                        sc - top).astype(BF16)
        return carry

    def out_proj(b):
        o = jnp.concatenate(
            [jnp.concatenate([ot_s[b * (OB // T) + m, _tile(j), :].T for j in range(ND)],
                             axis=1) for m in range(OB // T)], axis=0)
        r = _dot(o, wo_v[...])
        yb_s[b] = r.astype(BF16)
        return r[OB - 8:, D - T:]

    start(w_copies(0), x_copy(0))
    kpad_s[0:8, :] = jnp.zeros((8, T), F32)
    wait(w_copies(0))
    transpose_w(0)
    wait(x_copy(0))
    start(x_copy(1), small)
    project(0, 0)
    wait(x_copy(1), small)
    start(x_copy(2))
    small_tables()
    project(0, 1)
    wait(x_copy(2))
    start(x_copy(3))
    project(0, 2)
    wait(x_copy(3))
    start(kvh_copies(0), w_copies(1), kvh_copies(1), q_copy(0), w_copies(2))
    kn0_s[...] = keys(_Group(0, True), 0)
    project(0, 3)
    state = attention(0, None)
    wait(kvh_copies(0), w_copies(1))
    z = zeros(0, 2, 8)
    fwd_h(0, z)
    kv_prep(0)
    transpose_w(1)
    fwd_u(0, z)

    lax.fori_loop(0, ND - 1, phase1, 0)

    kn0_s[...] = keys(_Group(1, True), 0)
    state = lax.fori_loop(1, NGRP, attention, state)

    wait(wo_copy, q_copy(ND - 1))
    last_group = adopt(NGRP - 1, state)
    z = zeros(0, 2, 8)
    nb = nf = 0
    for ch in PHASE3_ORDER:
        if ch == "t":
            (po,) = zeros(3, 4, 16)
            for t in range(NSTEP - PV_CARRY, NSTEP):
                pv_direct(last_group, t, po)
        elif ch == "x":
            safe = ((jnp.min(last_group.lo) >= 2.0 ** -SUM_LOG2)
                    & (jnp.max(last_group.hi) <= 2.0 ** SUM_LOG2))

            @pl.when(jnp.logical_not(safe))
            def _():
                lax.fori_loop(0, NGRP, attention_true_max, 0)
        elif ch == "v":
            chunk_conv(ND - 1, z, nf)
            nf += 1
        elif ch == "i":
            inverse(ND - 1)
        elif ch == "a":
            start(outa_copy(ND - 1))
        elif ch in "pc":
            last = out_proj(nb)
            nb += 1
            if ch == "c":
                pace(z, last)
        else:
            start(outb_copy(int(ch)))
    assert nb == S // OB and nf == NT

    for c in range(ND):
        wait(outa_copy(c))
    for b in range(S // OB):
        wait(outb_copy(b))


@jax.jit
def pallas_concat_heads__ssm_conv_h3__memory_aug_infini_attn__prompt_kernel(
    A_q: jax.Array,
    A_k: jax.Array,
    A_v: jax.Array,
    A_shift_k: jax.Array,
    A_ssm_k: jax.Array,
    A_ssm_D: jax.Array,
    B_x: jax.Array,
    B_wq: jax.Array,
    B_wk: jax.Array,
    B_wv: jax.Array,
    B_wo: jax.Array,
    B_beta: jax.Array,
):
    hbm = pl.BlockSpec(memory_space=pltpu.MemorySpace.HBM)
    vmem = pltpu.VMEM
    dma = pltpu.SemaphoreType.DMA
    out = pl.pallas_call(
        _kernel,
        out_shape=jax.ShapeDtypeStruct((S, 2 * D), BF16),
        in_specs=[pl.BlockSpec(memory_space=pltpu.SMEM)] + [hbm] * 14,
        out_specs=hbm,
        scratch_shapes=[
            vmem((ND, S, T), BF16),
            vmem((ND, S, T), BF16),
            vmem((ND, S, T), BF16),
            vmem((KS, D), BF16),
            vmem((ND, T, S), BF16),
            vmem((ND, T), BF16),
            vmem((S, D), BF16),
            vmem((ND, 3, D, T), BF16),
            vmem((D, D), BF16),
            vmem((1, H), BF16),
            vmem((2 * T, T), BF16),
            vmem((T, 2 * T), BF16),
            vmem((ND, ND, 3 * T // 2, T), U32),
            vmem((ND, S // 2, T), U32),
            vmem((ND, 8, T), F32),
            vmem((D, T), F32),
            vmem((S + 8, T), F32),
            vmem((S, T), BF16),
            vmem((2 * NT, SP_PACE + 8, T), F32),
            vmem((NT, 2 * T, T), BF16),
            vmem((ND, S, T), BF16),
            vmem((NT, D, T), BF16),
            vmem((NT - TPL, D, T), BF16),
            vmem((NT, D, T), BF16),
            vmem((NT - TPL, D, T), BF16),
            vmem((NT, D, T), BF16),
            vmem((NT, D, T), BF16),
            vmem((S // OB, OB, D), BF16),
            vmem((RS * GH * T, T), F32),
            vmem((T, T), BF16),
            dma((6,)),
            dma((4, ND)),
            dma((3, ND)),
            dma((NSEG,)),
            dma((ND,)),
            dma((S // OB,)),
        ] + [vmem((GH * T, T), BF16)] * RP,
        compiler_params=pltpu.CompilerParams(vmem_limit_bytes=100 * 1024 * 1024),
        name="h3_infini_concat",
    )(
        jnp.asarray(_ZEROS),
        A_q.reshape(S, D), A_k.reshape(S, D), A_v.reshape(S, D), A_shift_k.T, A_ssm_k,
        A_ssm_D.reshape(ND, T), B_x.reshape(S, D), B_wq, B_wk, B_wv, B_wo,
        B_beta.reshape(1, H), jnp.asarray(_FWD), jnp.asarray(_INV),
    )
    return out.reshape(1, S, 2 * D)
```

```python
import math

import jax
import jax.numpy as jnp
import numpy as np
from jax import lax
from jax.experimental import pallas as pl
from jax.experimental.pallas import tpu as pltpu

S = 2048
D = 640
H = 32
DH = D // H
NSEG = 4
L = S // NSEG
KS = 4
T = 128
NT = S // T
TPL = L // T
ND = D // T
GH = 4
GR = GH * DH
NGRP = H // GH
OB = 256
RS, RP = 8, 4
Q_SCALE = DH ** -0.5 * math.log2(math.e)
NEG = -1e30
SUM_LOG2 = 30

F32 = jnp.float32
BF16 = jnp.bfloat16
U32 = jnp.uint32

SP_H, SP_U, SP_PACE = 0, 2 * T, 4 * T

PHASE1_ORDER = "vhvvvkkcvvvvkkcvvvvcvvvvpiu"
PHASE3_ORDER = "txvvcvvc0vvc1vvvc2vvvc3vvvvp4i5ap6p7"

STEPS = [(s, i, j) for s in range(NSEG) for i in range(TPL) for j in range(i + 1)]
NSTEP = len(STEPS)
PV_LAG = 3
PV_CARRY = 2
_LATE = {st[:2] for st in STEPS[NSTEP - PV_CARRY:]}
_ACC_KEYS = sorted({(s, i, h) for s, i, _ in STEPS[:NSTEP - PV_CARRY]
                    if (s, i) in _LATE for h in range(GH)})
_RET_KEYS = sorted(k for k in _LATE if k[0] > 0)
_CELLS = [(t + j, h) for t, (_, i, j0) in enumerate(STEPS) if j0 == 0
          for h in range(GH) for j in range(i + 1)]
EXP_LAG, MAX_PV_LAG = 4, 6


def _dft_matrices():
    k = np.arange(T, dtype=np.float64)[:, None]
    t = np.arange(T, dtype=np.float64)[None, :]
    theta = 2.0 * np.pi * (k + 0.25) * t / T
    re = np.cos(theta).reshape(T // 8, 1, 8, T)
    im = np.sin(theta).reshape(T // 8, 1, 8, T)
    fwd = np.concatenate([re, im], axis=1).reshape(2 * T, T)
    return (fwd.astype(np.float32).astype(BF16),
            (fwd.T / T).astype(np.float32).astype(BF16))


_FWD, _INV = _dft_matrices()
_ZEROS = np.zeros((8,), np.int32)


def _dot(a, b):
    return jnp.dot(a, b, preferred_element_type=F32)


def _dot_nt(a, b):
    return lax.dot_general(a, b, (((1,), (1,)), ((), ())), preferred_element_type=F32)


def _phi(t):
    return jnp.where(t > 0, t + 1.0, jnp.exp(t))


def _tile(i):
    return slice(i * T, (i + 1) * T)


def _iota(shape, axis):
    return lax.broadcasted_iota(jnp.int32, shape, axis)


def _add(xs, ys):
    return [x + y for x, y in zip(xs, ys)]


def _causal_complex(ur, ui, gr, gi):
    re, im = [], []
    for a in range(len(ur)):
        x = ur[0] * gr[a] - ui[0] * gi[a]
        y = ur[0] * gi[a] + ui[0] * gr[a]
        for j in range(1, a + 1):
            x = x + (ur[j] * gr[a - j] - ui[j] * gi[a - j])
            y = y + (ur[j] * gi[a - j] + ui[j] * gr[a - j])
        re.append(x)
        im.append(y)
    return re, im


class _Group:
    def __init__(self, g, paired):
        self.r0 = g * GR if isinstance(g, int) else pl.multiple_of(g * GR, 16)
        self.rows = pl.ds(self.r0, GR)
        self.paired = paired
        self.kn, self.va, self.w, self.w2 = {}, {}, {}, {}
        self.maxes, self.accs, self.rets, self.mems = {}, {}, {}, {}
        self.lo = self.hi = None


def _kernel(
    zero_ref, q_hbm, k_hbm, v_hbm, shift_hbm, h_hbm, d_hbm, x_hbm,
    wq_hbm, wk_hbm, wv_hbm, wo_hbm, beta_hbm, fwd_hbm, inv_hbm,
    out_hbm,
    q_v, k_v, v_v, shift_v, h_v, d_v, x_v, w_v, wo_v, beta_v, fwd_v, inv_v,
    wt_s, xu_s, taps_s, gate_s, kpad_s, kv_s, spec_s, yf_s, ya_s,
    qs_s, pq_s, kt_s, pk_s, vt_s, ot_s, yb_s, s_ring, kn0_s,
    in_sem, slab_sem, w_sem, x_sem, outa_sem, outb_sem, *p_ring,
):
    def slab(c):
        return pl.ds(c * T if isinstance(c, int) else pl.multiple_of(c * T, T), T)

    def kvh_copies(c):
        return (
            pltpu.make_async_copy(k_hbm.at[:, slab(c)], k_v.at[c], slab_sem.at[0, c]),
            pltpu.make_async_copy(v_hbm.at[:, slab(c)], v_v.at[c], slab_sem.at[1, c]),
            pltpu.make_async_copy(h_hbm.at[slab(c), :], h_v.at[c], slab_sem.at[2, c]),
        )

    def q_copy(c):
        return [pltpu.make_async_copy(q_hbm.at[:, slab(c)], q_v.at[c], slab_sem.at[3, c])]

    def w_copies(c):
        return [pltpu.make_async_copy(w.at[:, slab(c)], w_v.at[c, i], w_sem.at[i, c])
                for i, w in enumerate((wq_hbm, wk_hbm, wv_hbm))]

    def x_copy(b):
        rows = pl.ds(b * L, L)
        return [pltpu.make_async_copy(x_hbm.at[rows, :], x_v.at[rows, :], x_sem.at[b])]

    def outa_copy(c):
        return [pltpu.make_async_copy(ya_s.at[c], out_hbm.at[:, slab(c)], outa_sem.at[c])]

    def outb_copy(b):
        dst = out_hbm.at[pl.ds(b * OB, OB), pl.ds(D, D)]
        return [pltpu.make_async_copy(yb_s.at[b], dst, outb_sem.at[b])]

    small = [pltpu.make_async_copy(src, dst, in_sem.at[i]) for i, (src, dst) in enumerate(
        [(shift_hbm, shift_v), (d_hbm, d_v), (beta_hbm, beta_v),
         (fwd_hbm, fwd_v), (inv_hbm, inv_v)])]
    wo_copy = [pltpu.make_async_copy(wo_hbm, wo_v, in_sem.at[len(small)])]

    def start(*groups):
        for group in groups:
            for copy in group:
                copy.start()

    def wait(*groups):
        for group in groups:
            for copy in group:
                copy.wait()

    def start_now(*groups):
        def body(_, carry):
            start(*groups)
            return carry

        lax.fori_loop(0, zero_ref[7] + 1, body, 0)

    def zeros(n0, n1, align):
        return [pl.multiple_of(zero_ref[n], align) for n in range(n0, n1)]

    def small_tables():
        shift, skip = shift_v[...].astype(F32), d_v[...].astype(F32)
        for c in range(ND):
            taps_s[c, 0:KS, :] = shift[:, _tile(c)]
            taps_s[c, KS:KS + 1, :] = skip[c:c + 1, :]
        g_row = jax.nn.sigmoid(beta_v[...].astype(F32))
        row, head = _iota((D, H), 0), _iota((D, H), 1)
        own = (row >= head * DH) & (row < (head + 1) * DH)
        g_col = jnp.sum(jnp.where(own, g_row, 0.0), axis=1, keepdims=True)
        gate_s[...] = jnp.broadcast_to(g_col, (D, T))

    def tap(c, j):
        return taps_s[c, j:j + 1, :]

    def kv_prep(c, a0=0, a1=NT):
        w = [tap(c, j) for j in range(KS)]
        kpad_s[8 + a0 * T:8 + a1 * T, :] = k_v[c, a0 * T:a1 * T, :].astype(F32)
        for a in range(a0, a1):
            acc = None
            for j in range(KS):
                term = kpad_s[8 + a * T - j:8 + (a + 1) * T - j, :] * w[j]
                acc = term if acc is None else acc + term
            kv = acc * v_v[c, _tile(a), :].astype(F32)
            kv_s[_tile(a), :] = kv.astype(BF16)
        return kv[T - 8:]

    def store_spectrum(c, z, off, a, re, im):
        for f in range(T // 8):
            for m, part in enumerate((re, im)):
                rows = pl.ds(z[0] + off + 16 * f + 8 * m, 8)
                spec_s[(c % 2) * NT + a, rows, :] = part[f]

    def split(val, a):
        return ([val[16 * f:16 * f + 8, _tile(a)] for f in range(T // 8)],
                [val[16 * f + 8:16 * f + 16, _tile(a)] for f in range(T // 8)])

    def fwd_h(c, z):
        h_rows = jnp.concatenate([h_v[c, :, _tile(a)] for a in range(NT)], axis=0)
        val = _dot_nt(fwd_v[...], h_rows)
        skip = tap(c, KS)
        prev = None
        for a in range(NT):
            hr, hi = split(val, a)
            if prev is None:
                hr = [x + skip for x in hr]
                gr, gi = hr, hi
            else:
                gr = _add(hr, prev[1])
                gi = [x - y for x, y in zip(hi, prev[0])]
            prev = (hr, hi)
            store_spectrum(c, z, SP_H, a, gr, gi)

    def fwd_u(c, z):
        u = jnp.concatenate([kv_s[_tile(a), :] for a in range(NT)], axis=1)
        val = _dot(fwd_v[...], u)
        for a in range(NT):
            store_spectrum(c, z, SP_U, a, *split(val, a))

    def pace(z, val):
        spec_s[0, pl.ds(z[0] + SP_PACE, 8), :] = val

    def chunk_conv(c, z, f):
        def load(off):
            return [spec_s[(c % 2) * NT + a, pl.ds(z[1] + off + 16 * f, 8), :]
                    for a in range(NT)]

        gr, gi, ur, ui = load(SP_H), load(SP_H + 8), load(SP_U), load(SP_U + 8)
        er, ei = _causal_complex(ur[0::2], ui[0::2], gr[0::2], gi[0::2])
        o_r, o_i = _causal_complex(ur[1::2], ui[1::2], gr[1::2], gi[1::2])
        mr, mi = _causal_complex(_add(ur[0::2], ur[1::2]), _add(ui[0::2], ui[1::2]),
                                 _add(gr[0::2], gr[1::2]), _add(gi[0::2], gi[1::2]))
        re, im = [None] * NT, [None] * NT
        for m in range(NT // 2):
            re[2 * m] = er[m] if m == 0 else er[m] + o_r[m - 1]
            im[2 * m] = ei[m] if m == 0 else ei[m] + o_i[m - 1]
            re[2 * m + 1] = mr[m] - er[m] - o_r[m]
            im[2 * m + 1] = mi[m] - ei[m] - o_i[m]
        for a in range(NT):
            yf_s[a, 16 * f:16 * f + 16, :] = jnp.concatenate(
                [re[a], im[a]], axis=0).astype(BF16)

    def inverse(c):
        y = _dot(inv_v[...], jnp.concatenate([yf_s[a] for a in range(NT)], axis=1))
        for a in range(NT):
            ya_s[c, _tile(a), :] = (
                q_v[c, _tile(a), :].astype(F32) * y[:, _tile(a)]).astype(BF16)

    def transpose_w(c):
        for i in range(3):
            for j in range(ND):
                wt_s[c, j, i * T // 2:(i + 1) * T // 2, :] = pltpu.bitcast(
                    w_v[c, i, _tile(j), :].T, U32)

    def project(c, b):
        w = jnp.concatenate([pltpu.bitcast(wt_s[c, j], BF16) for j in range(ND)], axis=1)
        half = slice(b * L // 2, (b + 1) * L // 2)
        if isinstance(c, int):
            xb = x_v[b * L:(b + 1) * L, :]
            for j in range(ND):
                xu_s[j, half, :] = pltpu.bitcast(xb[:, _tile(j)], U32)
        else:
            xb = jnp.concatenate(
                [pltpu.bitcast(xu_s[j, half, :], BF16) for j in range(ND)], axis=1)
        r = _dot_nt(w, xb)
        rows = slab(c)
        for m in range(TPL):
            a = b * TPL + m
            qf, kf, vf = (r[_tile(i), _tile(m)] for i in range(3))
            qs_s[a, rows, :] = (qf * Q_SCALE).astype(BF16)
            kb = kf.astype(BF16)
            kt_s[a, rows, :] = kb
            vt_s[a, rows, :] = vf.astype(BF16)
            if b > 0:
                pq_s[a - TPL, rows, :] = _phi(qf.astype(BF16).astype(F32)).astype(BF16)
            if b < NSEG - 1:
                pk_s[a, rows, :] = _phi(kb.astype(F32)).astype(BF16)
        return r[3 * T - 8:, 0:T]

    def phase1(c, carry):
        wait(kvh_copies(c + 1), q_copy(c))

        @pl.when(c + 2 < ND)
        def _():
            wait(w_copies(c + 2))
            start(kvh_copies(c + 2))

        @pl.when(c + 3 < ND)
        def _():
            start(w_copies(c + 3))

        @pl.when(c + 3 == ND)
        def _():
            start(wo_copy)

        @pl.when(zero_ref[7] == 0)
        def _():
            start(q_copy(c + 1))

        z = zeros(0, 2, 8)
        transpose_w(jnp.minimum(c + 2, ND - 1))
        halves = PHASE1_ORDER.count("k")
        nb = nf = nk = 0
        for ch in PHASE1_ORDER:
            if ch == "h":
                fwd_h(c + 1, z)
            elif ch == "u":
                fwd_u(c + 1, z)
            elif ch == "i":
                inverse(c)
            elif ch in "pc":
                last = project(c + 1, nb)
                nb += 1
                if ch == "c":
                    pace(z, last)
            elif ch == "k":
                pace(z, kv_prep(c + 1, nk * NT // halves, (nk + 1) * NT // halves))
                nk += 1
            else:
                chunk_conv(c, z, nf)
                nf += 1
        assert nb == NSEG and nf == NT
        start(outa_copy(c))
        return carry

    def low4():
        return _iota((8, T), 0) < 4

    def pad_rows(x):
        return jnp.concatenate([x, jnp.zeros((T - GR, x.shape[1]), x.dtype)], axis=0)

    def keys(G, a):
        if a not in G.kn:
            G.kn[a] = pad_rows(kt_s[a, G.rows, :]).T
        return G.kn[a]

    def values(G, a):
        if a not in G.va:
            vt = vt_s[a, G.rows, :]
            b = [vt[16 * m:16 * m + 16] for m in range(5)]
            lo = low4()
            one2 = jnp.full((8, T), 0x3F803F80, U32)

            def top(x):
                return pltpu.bitcast(jnp.where(lo, pltpu.bitcast(x, U32), one2), BF16)

            def bottom(x):
                return pltpu.bitcast(jnp.where(lo, one2, pltpu.bitcast(x, U32)), BF16)

            G.va[a] = [jnp.concatenate(p, axis=0) for p in (
                [b[0], top(b[1])], [b[1], top(b[2])],
                [bottom(b[2]), b[3]], [bottom(b[3]), b[4]])]
        return G.va[a]

    def queries(G, a):
        if a not in G.w:
            pair = _iota((16, T), 0)
            blks = []
            for h in range(GH):
                lo = (h * DH - 16 * h) // 2
                blk = pltpu.bitcast(qs_s[a, pl.ds(G.r0 + 16 * h, 32), :], U32)
                blk = jnp.where((pair >= lo) & (pair < lo + DH // 2), blk,
                                jnp.zeros_like(blk))
                if G.paired and h % 2:
                    blk = pltpu.roll(blk, T // 2, 1)
                blks.append(blk)

            def place(blk, h):
                rest = T - 16 * h - 2 * blk.shape[0]
                pieces = [pltpu.bitcast(blk, BF16), jnp.zeros((rest, T), BF16)]
                if h:
                    pieces = [jnp.zeros((16 * h, T), BF16)] + pieces
                return jnp.concatenate(pieces, axis=0)

            G.w[a] = jnp.concatenate([place(blks[h], h) for h in range(GH)], axis=1)
            if G.paired:
                left = _iota((24, T), 1) < T // 2
                zero = jnp.zeros((8, T), U32)
                G.w2[a] = jnp.concatenate([
                    place(jnp.where(left, jnp.concatenate([zero, blks[h + 1]], axis=0),
                                    jnp.concatenate([blks[h], zero], axis=0)), h)
                    for h in range(0, GH, 2)], axis=1)
        return G.w[a]

    def update(G, s):
        ones = jnp.ones((16, T), BF16)
        va = jnp.concatenate(
            [jnp.concatenate([vt_s[s * TPL + j, G.rows, :], ones], axis=0)
             for j in range(TPL)], axis=1)
        pk = jnp.concatenate(
            [pad_rows(pk_s[s * TPL + j, G.rows, :]) for j in range(TPL)], axis=1)
        row, lane = _iota((GR + 16, T), 0), _iota((GR + 16, T), 1)
        keep = None
        for h in range(GH):
            mine = (((row >= h * DH) & (row < (h + 1) * DH))
                    | ((row >= GR + 4 * h) & (row < GR + 4 * h + 4)))
            mine = mine & (lane >= h * DH) & (lane < (h + 1) * DH)
            keep = mine if keep is None else keep | mine
        upd = jnp.where(keep, _dot_nt(va, pk), 0.0)
        G.mems[s + 1] = upd if s == 0 else G.mems[s] + upd

    def retrieve(G, s):
        pq = jnp.concatenate(
            [pad_rows(pq_s[(s - 1) * TPL + i, G.rows, :]) for i in range(TPL)], axis=1)
        ret = _dot(G.mems[s].astype(BF16), pq)
        gate = gate_s[G.rows, :]
        lo = low4()
        for i in range(TPL):
            inv = []
            for m in range(2):
                r = 1.0 / (ret[GR + 8 * m:GR + 8 * m + 8, _tile(i)] + 1e-6)
                other = pltpu.roll(r, 4, 0)
                first, second = jnp.where(lo, r, other), jnp.where(lo, other, r)
                inv += [first, first, r, second, second]
            G.rets[(s, i)] = ret[:GR, _tile(i)] * (gate * jnp.concatenate(inv, axis=0))

    def memory_steps(G, t):
        s, k = divmod(t, NSTEP // NSEG)
        if k == 2 and s > 0:
            retrieve(G, s)
        if k == 6 and s < NSEG - 1:
            update(G, s)

    def finish(G, s, i):
        accs = [G.accs[(s, i, h)] for h in range(GH)]
        if G.paired:
            accs = [pltpu.roll(x, T // 2, 1) if h % 2 else x for h, x in enumerate(accs)]
        u = [[x[8 * m:8 * m + 8] for m in range(4)] for x in accs]
        lo = low4()
        vals = jnp.concatenate(
            [u[0][0], u[0][1], jnp.where(lo, u[0][2], u[1][0]), u[1][1], u[1][2],
             u[2][1], u[2][2], jnp.where(lo, u[2][3], u[3][1]), u[3][2], u[3][3]], axis=0)
        sums = (u[0][3], u[1][3], u[2][0], u[3][0])
        if G.lo is not None:
            for d in sums:
                G.lo, G.hi = jnp.minimum(G.lo, d), jnp.maximum(G.hi, d)
        r = [1.0 / d for d in sums]
        inv = jnp.concatenate(
            [r[0], r[0], jnp.where(lo, r[0], r[1]), r[1], r[1],
             r[2], r[2], jnp.where(lo, r[2], r[3]), r[3], r[3]], axis=0)
        o = vals * ((1.0 - gate_s[G.rows, :]) * inv)
        if s > 0:
            o = o + G.rets[(s, i)]
        ot_s[s * TPL + i, G.rows, :] = o.astype(BF16)

    def accumulate(G, s, i, j, h, p):
        r = _dot(values(G, s * TPL + j)[h], p)
        G.accs[(s, i, h)] = r if j == 0 else G.accs[(s, i, h)] + r

    def qk_direct(G, t):
        s, i, j = STEPS[t]
        kn, w = keys(G, s * TPL + j), queries(G, s * TPL + i)
        if j < i:
            return _dot(kn, w)
        late_keys = _dot(kn[T // 2:], G.w2[s * TPL + i])
        return _dot(kn[:T // 2], w), late_keys

    def exp_direct(t, raw, ps):
        _, i, j = STEPS[t]
        if j < i:
            for h in range(GH):
                p_ring[t % RP][pl.ds(ps + h * T, T), :] = jnp.exp2(
                    raw[:, _tile(h)]).astype(BF16)
            return
        key, lane = _iota((T // 2, T), 0), _iota((T // 2, T), 1)
        qry = (lane, (lane + T // 2) & (T - 1))
        shared = [jnp.exp2(raw[1][:, _tile(m)]) for m in range(GH // 2)]
        for h in range(GH):
            top = jnp.where(key <= qry[h % 2], jnp.exp2(raw[0][:, _tile(h)]), 0.0)
            bot = jnp.where(key + T // 2 <= qry[h % 2], shared[h // 2], 0.0)
            p_ring[t % RP][pl.ds(ps + h * T, T), :] = jnp.concatenate(
                [top, bot], axis=0).astype(BF16)

    def pv_direct(G, t, po):
        s, i, j = STEPS[t]
        for h in range(GH):
            accumulate(G, s, i, j, h, p_ring[t % RP][pl.ds(po + h * T, T), :])
        if j == i:
            finish(G, s, i)

    def adopt(g, state):
        P = _Group(g, True)
        P.accs = dict(zip(_ACC_KEYS, state[0]))
        P.rets = dict(zip(_RET_KEYS, state[1]))
        P.lo, P.hi = state[2]
        return P

    def attention(g, state):
        ps, po = zeros(2, 4, 16)
        G = _Group(g, True)
        if state is None:
            P = None
            G.lo = G.hi = jnp.ones((8, T), F32)
        else:
            P = adopt(g - 1, state)
        G.kn[0] = kn0_s[...]
        done = 0
        for t in range(NSTEP):
            raw = qk_direct(G, t)
            memory_steps(G, t)
            if t < PV_CARRY and P is not None:
                pv_direct(P, NSTEP - PV_CARRY + t, po)
                G.lo, G.hi = P.lo, P.hi
            while done <= (t - PV_LAG if t < NSTEP - 1 else t - PV_CARRY):
                pv_direct(G, done, po)
                done += 1
            exp_direct(t, raw, ps)
            if t == NSTEP - 4 and P is not None:
                kn0_s[...] = keys(_Group(jnp.minimum(g + 1, NGRP - 1), True), 0)
        return ([G.accs[k] for k in _ACC_KEYS], [G.rets[k] for k in _RET_KEYS],
                (G.lo, G.hi))

    def attention_true_max(g, carry):
        zs, zl = zeros(0, 2, 8)
        ps, po = zeros(2, 4, 16)
        G = _Group(g, False)
        part = T // GH
        for t in range(NSTEP + MAX_PV_LAG):
            if t < NSTEP:
                s, i, j = STEPS[t]
                raw = _dot(keys(G, s * TPL + j), queries(G, s * TPL + i))
                memory_steps(G, t)
            if t >= MAX_PV_LAG:
                tp = t - MAX_PV_LAG
                for m in range(GH):
                    tq, h = _CELLS[tp * GH + m]
                    sp, ip, jp = STEPS[tq]
                    accumulate(G, sp, ip, jp, h, p_ring[tp % RP][pl.ds(po + m * T, T), :])
                    if jp == ip and h == GH - 1:
                        finish(G, sp, ip)
            for m in range(GH):
                if t < NSTEP:
                    r0 = m * part
                    causal = r0 + _iota((part, T), 0) <= _iota((part, T), 1)
                    ms = []
                    for h in range(GH):
                        sc = raw[r0:r0 + part, _tile(h)]
                        if j == i:
                            sc = jnp.where(causal, sc, NEG)
                        s_ring[pl.ds(zs + ((t % RS) * GH + h) * T + r0, part), :] = sc
                        m8 = sc[0:8]
                        for r in range(1, part // 8):
                            m8 = jnp.maximum(m8, sc[8 * r:8 * r + 8])
                        if j > 0 or m > 0:
                            m8 = jnp.maximum(G.maxes[(s, i)][h], m8)
                        if j == i and m == GH - 1:
                            m8 = jnp.broadcast_to(
                                jnp.max(m8, axis=0, keepdims=True), (8, T))
                        ms.append(m8)
                    G.maxes[(s, i)] = ms
                if EXP_LAG <= t < NSTEP + EXP_LAG:
                    te = t - EXP_LAG
                    tq, h = _CELLS[te * GH + m]
                    top = jnp.concatenate([G.maxes[STEPS[tq][:2]][h]] * (T // 8), axis=0)
                    sc = s_ring[pl.ds(zl + ((tq % RS) * GH + h) * T, T), :]
                    p_ring[te % RP][pl.ds(ps + m * T, T), :] = jnp.exp2(
                        sc - top).astype(BF16)
        return carry

    def out_proj(b):
        o = jnp.concatenate(
            [jnp.concatenate([ot_s[b * (OB // T) + m, _tile(j), :].T for j in range(ND)],
                             axis=1) for m in range(OB // T)], axis=0)
        r = _dot(o, wo_v[...])
        yb_s[b] = r.astype(BF16)
        return r[OB - 8:, D - T:]

    start(w_copies(0), x_copy(0))
    kpad_s[0:8, :] = jnp.zeros((8, T), F32)
    wait(w_copies(0))
    transpose_w(0)
    wait(x_copy(0))
    start(x_copy(1), small)
    project(0, 0)
    wait(x_copy(1), small)
    start(x_copy(2))
    small_tables()
    project(0, 1)
    wait(x_copy(2))
    start(x_copy(3))
    project(0, 2)
    wait(x_copy(3))
    start_now(kvh_copies(0), w_copies(1), kvh_copies(1), q_copy(0), w_copies(2))
    kn0_s[...] = keys(_Group(0, True), 0)
    project(0, 3)
    state = attention(0, None)
    wait(kvh_copies(0), w_copies(1))
    z = zeros(0, 2, 8)
    fwd_h(0, z)
    kv_prep(0)
    transpose_w(1)
    fwd_u(0, z)

    lax.fori_loop(0, ND - 1, phase1, 0)

    kn0_s[...] = keys(_Group(1, True), 0)
    state = lax.fori_loop(1, NGRP, attention, state)

    wait(wo_copy, q_copy(ND - 1))
    last_group = adopt(NGRP - 1, state)
    z = zeros(0, 2, 8)
    nb = nf = 0
    for ch in PHASE3_ORDER:
        if ch == "t":
            (po,) = zeros(3, 4, 16)
            for t in range(NSTEP - PV_CARRY, NSTEP):
                pv_direct(last_group, t, po)
        elif ch == "x":
            safe = ((jnp.min(last_group.lo) >= 2.0 ** -SUM_LOG2)
                    & (jnp.max(last_group.hi) <= 2.0 ** SUM_LOG2))

            @pl.when(jnp.logical_not(safe))
            def _():
                lax.fori_loop(0, NGRP, attention_true_max, 0)
        elif ch == "v":
            chunk_conv(ND - 1, z, nf)
            nf += 1
        elif ch == "i":
            inverse(ND - 1)
        elif ch == "a":
            start(outa_copy(ND - 1))
        elif ch in "pc":
            last = out_proj(nb)
            nb += 1
            if ch == "c":
                pace(z, last)
        else:
            start(outb_copy(int(ch)))
    assert nb == S // OB and nf == NT

    for c in range(ND):
        wait(outa_copy(c))
    for b in range(S // OB):
        wait(outb_copy(b))


@jax.jit
def pallas_concat_heads__ssm_conv_h3__memory_aug_infini_attn__prompt_kernel(
    A_q: jax.Array,
    A_k: jax.Array,
    A_v: jax.Array,
    A_shift_k: jax.Array,
    A_ssm_k: jax.Array,
    A_ssm_D: jax.Array,
    B_x: jax.Array,
    B_wq: jax.Array,
    B_wk: jax.Array,
    B_wv: jax.Array,
    B_wo: jax.Array,
    B_beta: jax.Array,
):
    hbm = pl.BlockSpec(memory_space=pltpu.MemorySpace.HBM)
    vmem = pltpu.VMEM
    dma = pltpu.SemaphoreType.DMA
    out = pl.pallas_call(
        _kernel,
        out_shape=jax.ShapeDtypeStruct((S, 2 * D), BF16),
        in_specs=[pl.BlockSpec(memory_space=pltpu.SMEM)] + [hbm] * 14,
        out_specs=hbm,
        scratch_shapes=[
            vmem((ND, S, T), BF16),
            vmem((ND, S, T), BF16),
            vmem((ND, S, T), BF16),
            vmem((KS, D), BF16),
            vmem((ND, T, S), BF16),
            vmem((ND, T), BF16),
            vmem((S, D), BF16),
            vmem((ND, 3, D, T), BF16),
            vmem((D, D), BF16),
            vmem((1, H), BF16),
            vmem((2 * T, T), BF16),
            vmem((T, 2 * T), BF16),
            vmem((ND, ND, 3 * T // 2, T), U32),
            vmem((ND, S // 2, T), U32),
            vmem((ND, 8, T), F32),
            vmem((D, T), F32),
            vmem((S + 8, T), F32),
            vmem((S, T), BF16),
            vmem((2 * NT, SP_PACE + 8, T), F32),
            vmem((NT, 2 * T, T), BF16),
            vmem((ND, S, T), BF16),
            vmem((NT, D, T), BF16),
            vmem((NT - TPL, D, T), BF16),
            vmem((NT, D, T), BF16),
            vmem((NT - TPL, D, T), BF16),
            vmem((NT, D, T), BF16),
            vmem((NT, D, T), BF16),
            vmem((S // OB, OB, D), BF16),
            vmem((RS * GH * T, T), F32),
            vmem((T, T), BF16),
            dma((6,)),
            dma((4, ND)),
            dma((3, ND)),
            dma((NSEG,)),
            dma((ND,)),
            dma((S // OB,)),
        ] + [vmem((GH * T, T), BF16)] * RP,
        compiler_params=pltpu.CompilerParams(vmem_limit_bytes=100 * 1024 * 1024),
        name="h3_infini_concat",
    )(
        jnp.asarray(_ZEROS),
        A_q.reshape(S, D), A_k.reshape(S, D), A_v.reshape(S, D), A_shift_k.T, A_ssm_k,
        A_ssm_D.reshape(ND, T), B_x.reshape(S, D), B_wq, B_wk, B_wv, B_wo,
        B_beta.reshape(1, H), jnp.asarray(_FWD), jnp.asarray(_INV),
    )
    return out.reshape(1, S, 2 * D)
```

```python
import math

import jax
import jax.numpy as jnp
import numpy as np
from jax import lax
from jax.experimental import pallas as pl
from jax.experimental.pallas import tpu as pltpu

S = 2048
D = 640
H = 32
DH = D // H
NSEG = 4
L = S // NSEG
KS = 4
T = 128
NT = S // T
TPL = L // T
ND = D // T
GH = 4
GR = GH * DH
NGRP = H // GH
OB = 256
RS, RP = 8, 4
Q_SCALE = DH ** -0.5 * math.log2(math.e)
NEG = -1e30
SUM_LOG2 = 30

F32 = jnp.float32
BF16 = jnp.bfloat16
U32 = jnp.uint32

SP_H, SP_U, SP_PACE = 0, 2 * T, 4 * T

PHASE1_ORDER = "vhvvvkkcvvvvkkcvvvvcvvvvpiu"
PHASE3_ORDER = "tvvcvvc0vvvc1vvvc2vvvc3vvvp4i5ap6p7"

STEPS = [(s, i, j) for s in range(NSEG) for i in range(TPL) for j in range(i + 1)]
NSTEP = len(STEPS)
PV_LAG = 3
PV_CARRY = 2
_LATE = {st[:2] for st in STEPS[NSTEP - PV_CARRY:]}
_ACC_KEYS = sorted({(s, i, h) for s, i, _ in STEPS[:NSTEP - PV_CARRY]
                    if (s, i) in _LATE for h in range(GH)})
_RET_KEYS = sorted(k for k in _LATE if k[0] > 0)
_CELLS = [(t + j, h) for t, (_, i, j0) in enumerate(STEPS) if j0 == 0
          for h in range(GH) for j in range(i + 1)]
EXP_LAG, MAX_PV_LAG = 4, 6


def _dft_matrices():
    k = np.arange(T, dtype=np.float64)[:, None]
    t = np.arange(T, dtype=np.float64)[None, :]
    theta = 2.0 * np.pi * (k + 0.25) * t / T
    re = np.cos(theta).reshape(T // 8, 1, 8, T)
    im = np.sin(theta).reshape(T // 8, 1, 8, T)
    fwd = np.concatenate([re, im], axis=1).reshape(2 * T, T)
    return (fwd.astype(np.float32).astype(BF16),
            (fwd.T / T).astype(np.float32).astype(BF16))


_FWD, _INV = _dft_matrices()
_ZEROS = np.zeros((8,), np.int32)


def _dot(a, b):
    return jnp.dot(a, b, preferred_element_type=F32)


def _dot_nt(a, b):
    return lax.dot_general(a, b, (((1,), (1,)), ((), ())), preferred_element_type=F32)


def _phi(t):
    return jnp.where(t > 0, t + 1.0, jnp.exp(t))


def _tile(i):
    return slice(i * T, (i + 1) * T)


def _iota(shape, axis):
    return lax.broadcasted_iota(jnp.int32, shape, axis)


def _add(xs, ys):
    return [x + y for x, y in zip(xs, ys)]


def _causal_complex(ur, ui, gr, gi):
    re, im = [], []
    for a in range(len(ur)):
        x = ur[0] * gr[a] - ui[0] * gi[a]
        y = ur[0] * gi[a] + ui[0] * gr[a]
        for j in range(1, a + 1):
            x = x + (ur[j] * gr[a - j] - ui[j] * gi[a - j])
            y = y + (ur[j] * gi[a - j] + ui[j] * gr[a - j])
        re.append(x)
        im.append(y)
    return re, im


class _Group:
    def __init__(self, g, paired):
        self.r0 = g * GR if isinstance(g, int) else pl.multiple_of(g * GR, 16)
        self.rows = pl.ds(self.r0, GR)
        self.paired = paired
        self.kn, self.va, self.w, self.w2 = {}, {}, {}, {}
        self.maxes, self.accs, self.rets, self.mems = {}, {}, {}, {}
        self.lo = self.hi = None


def _kernel(
    zero_ref, q_hbm, k_hbm, v_hbm, shift_hbm, h_hbm, d_hbm, x_hbm,
    wq_hbm, wk_hbm, wv_hbm, wo_hbm, beta_hbm, fwd_hbm, inv_hbm,
    out_hbm,
    q_v, k_v, v_v, shift_v, h_v, d_v, x_v, w_v, wo_v, beta_v, fwd_v, inv_v,
    wt_s, xu_s, taps_s, gate_s, kpad_s, kv_s, spec_s, yf_s, ya_s,
    qs_s, pq_s, kt_s, pk_s, vt_s, ot_s, yb_s, s_ring, kn0_s,
    in_sem, slab_sem, w_sem, x_sem, outa_sem, outb_sem, *p_ring,
):
    def slab(c):
        return pl.ds(c * T if isinstance(c, int) else pl.multiple_of(c * T, T), T)

    def kvh_copies(c):
        return (
            pltpu.make_async_copy(k_hbm.at[:, slab(c)], k_v.at[c], slab_sem.at[0, c]),
            pltpu.make_async_copy(v_hbm.at[:, slab(c)], v_v.at[c], slab_sem.at[1, c]),
            pltpu.make_async_copy(h_hbm.at[slab(c), :], h_v.at[c], slab_sem.at[2, c]),
        )

    def q_copy(c):
        return [pltpu.make_async_copy(q_hbm.at[:, slab(c)], q_v.at[c], slab_sem.at[3, c])]

    def w_copies(c):
        return [pltpu.make_async_copy(w.at[:, slab(c)], w_v.at[c, i], w_sem.at[i, c])
                for i, w in enumerate((wq_hbm, wk_hbm, wv_hbm))]

    def x_copy(b):
        rows = pl.ds(b * L, L)
        return [pltpu.make_async_copy(x_hbm.at[rows, :], x_v.at[rows, :], x_sem.at[b])]

    def outa_copy(c):
        return [pltpu.make_async_copy(ya_s.at[c], out_hbm.at[:, slab(c)], outa_sem.at[c])]

    def outb_copy(b):
        r0 = b * OB if isinstance(b, int) else pl.multiple_of(b * OB, OB)
        dst = out_hbm.at[pl.ds(r0, OB), pl.ds(D, D)]
        return [pltpu.make_async_copy(yb_s.at[b], dst, outb_sem.at[b])]

    small = [pltpu.make_async_copy(src, dst, in_sem.at[i]) for i, (src, dst) in enumerate(
        [(shift_hbm, shift_v), (d_hbm, d_v), (beta_hbm, beta_v),
         (fwd_hbm, fwd_v), (inv_hbm, inv_v)])]
    wo_copy = [pltpu.make_async_copy(wo_hbm, wo_v, in_sem.at[len(small)])]

    def start(*groups):
        for group in groups:
            for copy in group:
                copy.start()

    def wait(*groups):
        for group in groups:
            for copy in group:
                copy.wait()

    def start_now(*groups):
        def body(_, carry):
            start(*groups)
            return carry

        lax.fori_loop(0, zero_ref[7] + 1, body, 0)

    def zeros(n0, n1, align):
        return [pl.multiple_of(zero_ref[n], align) for n in range(n0, n1)]

    def small_tables():
        shift, skip = shift_v[...].astype(F32), d_v[...].astype(F32)
        for c in range(ND):
            taps_s[c, 0:KS, :] = shift[:, _tile(c)]
            taps_s[c, KS:KS + 1, :] = skip[c:c + 1, :]
        g_row = jax.nn.sigmoid(beta_v[...].astype(F32))
        row, head = _iota((D, H), 0), _iota((D, H), 1)
        own = (row >= head * DH) & (row < (head + 1) * DH)
        g_col = jnp.sum(jnp.where(own, g_row, 0.0), axis=1, keepdims=True)
        gate_s[...] = jnp.broadcast_to(g_col, (D, T))

    def tap(c, j):
        return taps_s[c, j:j + 1, :]

    def kv_prep(c, a0=0, a1=NT):
        w = [tap(c, j) for j in range(KS)]
        kpad_s[8 + a0 * T:8 + a1 * T, :] = k_v[c, a0 * T:a1 * T, :].astype(F32)
        for a in range(a0, a1):
            acc = None
            for j in range(KS):
                term = kpad_s[8 + a * T - j:8 + (a + 1) * T - j, :] * w[j]
                acc = term if acc is None else acc + term
            kv = acc * v_v[c, _tile(a), :].astype(F32)
            kv_s[_tile(a), :] = kv.astype(BF16)
        return kv[T - 8:]

    def store_spectrum(c, z, off, a, re, im):
        for f in range(T // 8):
            for m, part in enumerate((re, im)):
                rows = pl.ds(z[0] + off + 16 * f + 8 * m, 8)
                spec_s[(c % 2) * NT + a, rows, :] = part[f]

    def split(val, a):
        return ([val[16 * f:16 * f + 8, _tile(a)] for f in range(T // 8)],
                [val[16 * f + 8:16 * f + 16, _tile(a)] for f in range(T // 8)])

    def fwd_h(c, z):
        h_rows = jnp.concatenate([h_v[c, :, _tile(a)] for a in range(NT)], axis=0)
        val = _dot_nt(fwd_v[...], h_rows)
        skip = tap(c, KS)
        prev = None
        for a in range(NT):
            hr, hi = split(val, a)
            if prev is None:
                hr = [x + skip for x in hr]
                gr, gi = hr, hi
            else:
                gr = _add(hr, prev[1])
                gi = [x - y for x, y in zip(hi, prev[0])]
            prev = (hr, hi)
            store_spectrum(c, z, SP_H, a, gr, gi)

    def fwd_u(c, z):
        u = jnp.concatenate([kv_s[_tile(a), :] for a in range(NT)], axis=1)
        val = _dot(fwd_v[...], u)
        for a in range(NT):
            store_spectrum(c, z, SP_U, a, *split(val, a))

    def pace(z, val):
        spec_s[0, pl.ds(z[0] + SP_PACE, 8), :] = val

    def chunk_conv(c, z, f):
        def load(off):
            return [spec_s[(c % 2) * NT + a, pl.ds(z[1] + off + 16 * f, 8), :]
                    for a in range(NT)]

        gr, gi, ur, ui = load(SP_H), load(SP_H + 8), load(SP_U), load(SP_U + 8)
        er, ei = _causal_complex(ur[0::2], ui[0::2], gr[0::2], gi[0::2])
        o_r, o_i = _causal_complex(ur[1::2], ui[1::2], gr[1::2], gi[1::2])
        mr, mi = _causal_complex(_add(ur[0::2], ur[1::2]), _add(ui[0::2], ui[1::2]),
                                 _add(gr[0::2], gr[1::2]), _add(gi[0::2], gi[1::2]))
        re, im = [None] * NT, [None] * NT
        for m in range(NT // 2):
            re[2 * m] = er[m] if m == 0 else er[m] + o_r[m - 1]
            im[2 * m] = ei[m] if m == 0 else ei[m] + o_i[m - 1]
            re[2 * m + 1] = mr[m] - er[m] - o_r[m]
            im[2 * m + 1] = mi[m] - ei[m] - o_i[m]
        for a in range(NT):
            yf_s[a, 16 * f:16 * f + 16, :] = jnp.concatenate(
                [re[a], im[a]], axis=0).astype(BF16)

    def inverse(c):
        y = _dot(inv_v[...], jnp.concatenate([yf_s[a] for a in range(NT)], axis=1))
        for a in range(NT):
            ya_s[c, _tile(a), :] = (
                q_v[c, _tile(a), :].astype(F32) * y[:, _tile(a)]).astype(BF16)

    def transpose_w(c):
        for i in range(3):
            for j in range(ND):
                wt_s[c, j, i * T // 2:(i + 1) * T // 2, :] = pltpu.bitcast(
                    w_v[c, i, _tile(j), :].T, U32)

    def project(c, b):
        w = jnp.concatenate([pltpu.bitcast(wt_s[c, j], BF16) for j in range(ND)], axis=1)
        half = slice(b * L // 2, (b + 1) * L // 2)
        if isinstance(c, int):
            xb = x_v[b * L:(b + 1) * L, :]
            for j in range(ND):
                xu_s[j, half, :] = pltpu.bitcast(xb[:, _tile(j)], U32)
        else:
            xb = jnp.concatenate(
                [pltpu.bitcast(xu_s[j, half, :], BF16) for j in range(ND)], axis=1)
        r = _dot_nt(w, xb)
        rows = slab(c)
        for m in range(TPL):
            a = b * TPL + m
            qf, kf, vf = (r[_tile(i), _tile(m)] for i in range(3))
            qs_s[a, rows, :] = (qf * Q_SCALE).astype(BF16)
            kb = kf.astype(BF16)
            kt_s[a, rows, :] = kb
            vt_s[a, rows, :] = vf.astype(BF16)
            if b > 0:
                pq_s[a - TPL, rows, :] = _phi(qf.astype(BF16).astype(F32)).astype(BF16)
            if b < NSEG - 1:
                pk_s[a, rows, :] = _phi(kb.astype(F32)).astype(BF16)
        return r[3 * T - 8:, 0:T]

    def phase1(c, carry):
        wait(kvh_copies(c + 1), q_copy(c))

        @pl.when(c + 2 < ND)
        def _():
            wait(w_copies(c + 2))
            start(kvh_copies(c + 2))

        @pl.when(c + 3 < ND)
        def _():
            start(w_copies(c + 3))

        @pl.when(c + 3 == ND)
        def _():
            start(wo_copy)

        @pl.when(zero_ref[7] == 0)
        def _():
            start(q_copy(c + 1))

        z = zeros(0, 2, 8)
        transpose_w(jnp.minimum(c + 2, ND - 1))
        halves = PHASE1_ORDER.count("k")
        nb = nf = nk = 0
        for ch in PHASE1_ORDER:
            if ch == "h":
                fwd_h(c + 1, z)
            elif ch == "u":
                fwd_u(c + 1, z)
            elif ch == "i":
                inverse(c)
            elif ch in "pc":
                last = project(c + 1, nb)
                nb += 1
                if ch == "c":
                    pace(z, last)
            elif ch == "k":
                pace(z, kv_prep(c + 1, nk * NT // halves, (nk + 1) * NT // halves))
                nk += 1
            else:
                chunk_conv(c, z, nf)
                nf += 1
        assert nb == NSEG and nf == NT
        start(outa_copy(c))
        return carry

    def low4():
        return _iota((8, T), 0) < 4

    def pad_rows(x):
        return jnp.concatenate([x, jnp.zeros((T - GR, x.shape[1]), x.dtype)], axis=0)

    def keys(G, a):
        if a not in G.kn:
            G.kn[a] = pad_rows(kt_s[a, G.rows, :]).T
        return G.kn[a]

    def values(G, a):
        if a not in G.va:
            vt = vt_s[a, G.rows, :]
            b = [vt[16 * m:16 * m + 16] for m in range(5)]
            lo = low4()
            one2 = jnp.full((8, T), 0x3F803F80, U32)

            def top(x):
                return pltpu.bitcast(jnp.where(lo, pltpu.bitcast(x, U32), one2), BF16)

            def bottom(x):
                return pltpu.bitcast(jnp.where(lo, one2, pltpu.bitcast(x, U32)), BF16)

            G.va[a] = [jnp.concatenate(p, axis=0) for p in (
                [b[0], top(b[1])], [b[1], top(b[2])],
                [bottom(b[2]), b[3]], [bottom(b[3]), b[4]])]
        return G.va[a]

    def queries(G, a):
        if a not in G.w:
            pair = _iota((16, T), 0)
            blks = []
            for h in range(GH):
                lo = (h * DH - 16 * h) // 2
                blk = pltpu.bitcast(qs_s[a, pl.ds(G.r0 + 16 * h, 32), :], U32)
                blk = jnp.where((pair >= lo) & (pair < lo + DH // 2), blk,
                                jnp.zeros_like(blk))
                if G.paired and h % 2:
                    blk = pltpu.roll(blk, T // 2, 1)
                blks.append(blk)

            def place(blk, h):
                rest = T - 16 * h - 2 * blk.shape[0]
                pieces = [pltpu.bitcast(blk, BF16), jnp.zeros((rest, T), BF16)]
                if h:
                    pieces = [jnp.zeros((16 * h, T), BF16)] + pieces
                return jnp.concatenate(pieces, axis=0)

            G.w[a] = jnp.concatenate([place(blks[h], h) for h in range(GH)], axis=1)
            if G.paired:
                left = _iota((24, T), 1) < T // 2
                zero = jnp.zeros((8, T), U32)
                G.w2[a] = jnp.concatenate([
                    place(jnp.where(left, jnp.concatenate([zero, blks[h + 1]], axis=0),
                                    jnp.concatenate([blks[h], zero], axis=0)), h)
                    for h in range(0, GH, 2)], axis=1)
        return G.w[a]

    def update(G, s):
        ones = jnp.ones((16, T), BF16)
        va = jnp.concatenate(
            [jnp.concatenate([vt_s[s * TPL + j, G.rows, :], ones], axis=0)
             for j in range(TPL)], axis=1)
        pk = jnp.concatenate(
            [pad_rows(pk_s[s * TPL + j, G.rows, :]) for j in range(TPL)], axis=1)
        row, lane = _iota((GR + 16, T), 0), _iota((GR + 16, T), 1)
        keep = None
        for h in range(GH):
            mine = (((row >= h * DH) & (row < (h + 1) * DH))
                    | ((row >= GR + 4 * h) & (row < GR + 4 * h + 4)))
            mine = mine & (lane >= h * DH) & (lane < (h + 1) * DH)
            keep = mine if keep is None else keep | mine
        upd = jnp.where(keep, _dot_nt(va, pk), 0.0)
        G.mems[s + 1] = upd if s == 0 else G.mems[s] + upd

    def retrieve(G, s):
        pq = jnp.concatenate(
            [pad_rows(pq_s[(s - 1) * TPL + i, G.rows, :]) for i in range(TPL)], axis=1)
        ret = _dot(G.mems[s].astype(BF16), pq)
        gate = gate_s[G.rows, :]
        lo = low4()
        for i in range(TPL):
            inv = []
            for m in range(2):
                r = 1.0 / (ret[GR + 8 * m:GR + 8 * m + 8, _tile(i)] + 1e-6)
                other = pltpu.roll(r, 4, 0)
                first, second = jnp.where(lo, r, other), jnp.where(lo, other, r)
                inv += [first, first, r, second, second]
            G.rets[(s, i)] = ret[:GR, _tile(i)] * (gate * jnp.concatenate(inv, axis=0))

    def memory_steps(G, t):
        s, k = divmod(t, NSTEP // NSEG)
        if k == 2 and s > 0:
            retrieve(G, s)
        if k == 6 and s < NSEG - 1:
            update(G, s)

    def finish(G, s, i):
        accs = [G.accs[(s, i, h)] for h in range(GH)]
        if G.paired:
            accs = [pltpu.roll(x, T // 2, 1) if h % 2 else x for h, x in enumerate(accs)]
        u = [[x[8 * m:8 * m + 8] for m in range(4)] for x in accs]
        lo = low4()
        vals = jnp.concatenate(
            [u[0][0], u[0][1], jnp.where(lo, u[0][2], u[1][0]), u[1][1], u[1][2],
             u[2][1], u[2][2], jnp.where(lo, u[2][3], u[3][1]), u[3][2], u[3][3]], axis=0)
        sums = (u[0][3], u[1][3], u[2][0], u[3][0])
        if G.lo is not None:
            for d in sums:
                G.lo, G.hi = jnp.minimum(G.lo, d), jnp.maximum(G.hi, d)
        r = [1.0 / d for d in sums]
        inv = jnp.concatenate(
            [r[0], r[0], jnp.where(lo, r[0], r[1]), r[1], r[1],
             r[2], r[2], jnp.where(lo, r[2], r[3]), r[3], r[3]], axis=0)
        o = vals * ((1.0 - gate_s[G.rows, :]) * inv)
        if s > 0:
            o = o + G.rets[(s, i)]
        ot_s[s * TPL + i, G.rows, :] = o.astype(BF16)

    def accumulate(G, s, i, j, h, p):
        r = _dot(values(G, s * TPL + j)[h], p)
        G.accs[(s, i, h)] = r if j == 0 else G.accs[(s, i, h)] + r

    def qk_direct(G, t):
        s, i, j = STEPS[t]
        kn, w = keys(G, s * TPL + j), queries(G, s * TPL + i)
        if j < i:
            return _dot(kn, w)
        late_keys = _dot(kn[T // 2:], G.w2[s * TPL + i])
        return _dot(kn[:T // 2], w), late_keys

    def exp_direct(t, raw, ps):
        _, i, j = STEPS[t]
        if j < i:
            for h in range(GH):
                p_ring[t % RP][pl.ds(ps + h * T, T), :] = jnp.exp2(
                    raw[:, _tile(h)]).astype(BF16)
            return
        key, lane = _iota((T // 2, T), 0), _iota((T // 2, T), 1)
        qry = (lane, (lane + T // 2) & (T - 1))
        shared = [jnp.exp2(raw[1][:, _tile(m)]) for m in range(GH // 2)]
        for h in range(GH):
            top = jnp.where(key <= qry[h % 2], jnp.exp2(raw[0][:, _tile(h)]), 0.0)
            bot = jnp.where(key + T // 2 <= qry[h % 2], shared[h // 2], 0.0)
            p_ring[t % RP][pl.ds(ps + h * T, T), :] = jnp.concatenate(
                [top, bot], axis=0).astype(BF16)

    def pv_direct(G, t, po):
        s, i, j = STEPS[t]
        for h in range(GH):
            accumulate(G, s, i, j, h, p_ring[t % RP][pl.ds(po + h * T, T), :])
        if j == i:
            finish(G, s, i)

    def adopt(g, state):
        P = _Group(g, True)
        P.accs = dict(zip(_ACC_KEYS, state[0]))
        P.rets = dict(zip(_RET_KEYS, state[1]))
        P.lo, P.hi = state[2]
        return P

    def attention(g, state):
        ps, po = zeros(2, 4, 16)
        G = _Group(g, True)
        if state is None:
            P = None
            G.lo = G.hi = jnp.ones((8, T), F32)
        else:
            P = adopt(g - 1, state)
        G.kn[0] = kn0_s[...]
        done = 0
        for t in range(NSTEP):
            raw = qk_direct(G, t)
            memory_steps(G, t)
            if t < PV_CARRY and P is not None:
                pv_direct(P, NSTEP - PV_CARRY + t, po)
                G.lo, G.hi = P.lo, P.hi
            while done <= (t - PV_LAG if t < NSTEP - 1 else t - PV_CARRY):
                pv_direct(G, done, po)
                done += 1
            exp_direct(t, raw, ps)
            if t == NSTEP - 4 and P is not None:
                kn0_s[...] = keys(_Group(jnp.minimum(g + 1, NGRP - 1), True), 0)
        return ([G.accs[k] for k in _ACC_KEYS], [G.rets[k] for k in _RET_KEYS],
                (G.lo, G.hi))

    def attention_true_max(g, carry):
        zs, zl = zeros(0, 2, 8)
        ps, po = zeros(2, 4, 16)
        G = _Group(g, False)
        part = T // GH
        for t in range(NSTEP + MAX_PV_LAG):
            if t < NSTEP:
                s, i, j = STEPS[t]
                raw = _dot(keys(G, s * TPL + j), queries(G, s * TPL + i))
                memory_steps(G, t)
            if t >= MAX_PV_LAG:
                tp = t - MAX_PV_LAG
                for m in range(GH):
                    tq, h = _CELLS[tp * GH + m]
                    sp, ip, jp = STEPS[tq]
                    accumulate(G, sp, ip, jp, h, p_ring[tp % RP][pl.ds(po + m * T, T), :])
                    if jp == ip and h == GH - 1:
                        finish(G, sp, ip)
            for m in range(GH):
                if t < NSTEP:
                    r0 = m * part
                    causal = r0 + _iota((part, T), 0) <= _iota((part, T), 1)
                    ms = []
                    for h in range(GH):
                        sc = raw[r0:r0 + part, _tile(h)]
                        if j == i:
                            sc = jnp.where(causal, sc, NEG)
                        s_ring[pl.ds(zs + ((t % RS) * GH + h) * T + r0, part), :] = sc
                        m8 = sc[0:8]
                        for r in range(1, part // 8):
                            m8 = jnp.maximum(m8, sc[8 * r:8 * r + 8])
                        if j > 0 or m > 0:
                            m8 = jnp.maximum(G.maxes[(s, i)][h], m8)
                        if j == i and m == GH - 1:
                            m8 = jnp.broadcast_to(
                                jnp.max(m8, axis=0, keepdims=True), (8, T))
                        ms.append(m8)
                    G.maxes[(s, i)] = ms
                if EXP_LAG <= t < NSTEP + EXP_LAG:
                    te = t - EXP_LAG
                    tq, h = _CELLS[te * GH + m]
                    top = jnp.concatenate([G.maxes[STEPS[tq][:2]][h]] * (T // 8), axis=0)
                    sc = s_ring[pl.ds(zl + ((tq % RS) * GH + h) * T, T), :]
                    p_ring[te % RP][pl.ds(ps + m * T, T), :] = jnp.exp2(
                        sc - top).astype(BF16)
        return carry

    def out_proj(b):
        o = jnp.concatenate(
            [jnp.concatenate([ot_s[b * (OB // T) + m, _tile(j), :].T for j in range(ND)],
                             axis=1) for m in range(OB // T)], axis=0)
        r = _dot(o, wo_v[...])
        yb_s[b] = r.astype(BF16)
        return r[OB - 8:, D - T:]

    start(w_copies(0), x_copy(0))
    kpad_s[0:8, :] = jnp.zeros((8, T), F32)
    wait(w_copies(0))
    transpose_w(0)
    wait(x_copy(0))
    start(x_copy(1), small)
    project(0, 0)
    wait(x_copy(1), small)
    start(x_copy(2))
    small_tables()
    project(0, 1)
    wait(x_copy(2))
    start(x_copy(3))
    project(0, 2)
    wait(x_copy(3))
    start_now(kvh_copies(0), w_copies(1), kvh_copies(1), q_copy(0), w_copies(2))
    kn0_s[...] = keys(_Group(0, True), 0)
    project(0, 3)
    state = attention(0, None)
    wait(kvh_copies(0), w_copies(1))
    z = zeros(0, 2, 8)
    fwd_h(0, z)
    kv_prep(0)
    transpose_w(1)
    fwd_u(0, z)

    lax.fori_loop(0, ND - 1, phase1, 0)

    kn0_s[...] = keys(_Group(1, True), 0)
    state = lax.fori_loop(1, NGRP, attention, state)

    wait(wo_copy, q_copy(ND - 1))
    last_group = adopt(NGRP - 1, state)
    z = zeros(0, 2, 8)
    nb = nf = 0
    for ch in PHASE3_ORDER:
        if ch == "t":
            (po,) = zeros(3, 4, 16)
            for t in range(NSTEP - PV_CARRY, NSTEP):
                pv_direct(last_group, t, po)
        elif ch == "v":
            chunk_conv(ND - 1, z, nf)
            nf += 1
        elif ch == "i":
            inverse(ND - 1)
        elif ch == "a":
            start(outa_copy(ND - 1))
        elif ch in "pc":
            last = out_proj(nb)
            nb += 1
            if ch == "c":
                pace(z, last)
        else:
            start(outb_copy(int(ch)))
    assert nb == S // OB and nf == NT
    safe = ((jnp.min(last_group.lo) >= 2.0 ** -SUM_LOG2)
            & (jnp.max(last_group.hi) <= 2.0 ** SUM_LOG2))

    for c in range(ND):
        wait(outa_copy(c))
    for b in range(S // OB):
        wait(outb_copy(b))

    @pl.when(jnp.logical_not(safe))
    def _():
        lax.fori_loop(0, NGRP, attention_true_max, 0)

        def redo_block(b, carry):
            out_proj(b)
            start(outb_copy(b))
            wait(outb_copy(b))
            return carry

        lax.fori_loop(0, S // OB, redo_block, 0)


@jax.jit
def pallas_concat_heads__ssm_conv_h3__memory_aug_infini_attn__prompt_kernel(
    A_q: jax.Array,
    A_k: jax.Array,
    A_v: jax.Array,
    A_shift_k: jax.Array,
    A_ssm_k: jax.Array,
    A_ssm_D: jax.Array,
    B_x: jax.Array,
    B_wq: jax.Array,
    B_wk: jax.Array,
    B_wv: jax.Array,
    B_wo: jax.Array,
    B_beta: jax.Array,
):
    hbm = pl.BlockSpec(memory_space=pltpu.MemorySpace.HBM)
    vmem = pltpu.VMEM
    dma = pltpu.SemaphoreType.DMA
    out = pl.pallas_call(
        _kernel,
        out_shape=jax.ShapeDtypeStruct((S, 2 * D), BF16),
        in_specs=[pl.BlockSpec(memory_space=pltpu.SMEM)] + [hbm] * 14,
        out_specs=hbm,
        scratch_shapes=[
            vmem((ND, S, T), BF16),
            vmem((ND, S, T), BF16),
            vmem((ND, S, T), BF16),
            vmem((KS, D), BF16),
            vmem((ND, T, S), BF16),
            vmem((ND, T), BF16),
            vmem((S, D), BF16),
            vmem((ND, 3, D, T), BF16),
            vmem((D, D), BF16),
            vmem((1, H), BF16),
            vmem((2 * T, T), BF16),
            vmem((T, 2 * T), BF16),
            vmem((ND, ND, 3 * T // 2, T), U32),
            vmem((ND, S // 2, T), U32),
            vmem((ND, 8, T), F32),
            vmem((D, T), F32),
            vmem((S + 8, T), F32),
            vmem((S, T), BF16),
            vmem((2 * NT, SP_PACE + 8, T), F32),
            vmem((NT, 2 * T, T), BF16),
            vmem((ND, S, T), BF16),
            vmem((NT, D, T), BF16),
            vmem((NT - TPL, D, T), BF16),
            vmem((NT, D, T), BF16),
            vmem((NT - TPL, D, T), BF16),
            vmem((NT, D, T), BF16),
            vmem((NT, D, T), BF16),
            vmem((S // OB, OB, D), BF16),
            vmem((RS * GH * T, T), F32),
            vmem((T, T), BF16),
            dma((6,)),
            dma((4, ND)),
            dma((3, ND)),
            dma((NSEG,)),
            dma((ND,)),
            dma((S // OB,)),
        ] + [vmem((GH * T, T), BF16)] * RP,
        compiler_params=pltpu.CompilerParams(vmem_limit_bytes=100 * 1024 * 1024),
        name="h3_infini_concat",
    )(
        jnp.asarray(_ZEROS),
        A_q.reshape(S, D), A_k.reshape(S, D), A_v.reshape(S, D), A_shift_k.T, A_ssm_k,
        A_ssm_D.reshape(ND, T), B_x.reshape(S, D), B_wq, B_wk, B_wv, B_wo,
        B_beta.reshape(1, H), jnp.asarray(_FWD), jnp.asarray(_INV),
    )
    return out.reshape(1, S, 2 * D)
```

```python
import math

import jax
import jax.numpy as jnp
import numpy as np
from jax import lax
from jax.experimental import pallas as pl
from jax.experimental.pallas import tpu as pltpu

S = 2048
D = 640
H = 32
DH = D // H
NSEG = 4
L = S // NSEG
KS = 4
T = 128
NT = S // T
TPL = L // T
ND = D // T
GH = 4
GR = GH * DH
NGRP = H // GH
OB = 256
RS, RP = 8, 4
Q_SCALE = DH ** -0.5 * math.log2(math.e)
NEG = -1e30
SUM_LOG2 = 30

F32 = jnp.float32
BF16 = jnp.bfloat16
U32 = jnp.uint32

SP_H, SP_U, SP_PACE = 0, 2 * T, 4 * T

PHASE1_ORDER = "vhvvvkkcvvvvkkcvvvvvcvvvpiu"
PHASE3_ORDER = "tvvcvvc0vvvc1vvvc2vvvc3vvvp4i5ap6p7"

STEPS = [(s, i, j) for s in range(NSEG) for i in range(TPL) for j in range(i + 1)]
NSTEP = len(STEPS)
PV_LAG = 3
PV_CARRY = 2
_LATE = {st[:2] for st in STEPS[NSTEP - PV_CARRY:]}
_ACC_KEYS = sorted({(s, i, h) for s, i, _ in STEPS[:NSTEP - PV_CARRY]
                    if (s, i) in _LATE for h in range(GH)})
_RET_KEYS = sorted(k for k in _LATE if k[0] > 0)
_CELLS = [(t + j, h) for t, (_, i, j0) in enumerate(STEPS) if j0 == 0
          for h in range(GH) for j in range(i + 1)]
EXP_LAG, MAX_PV_LAG = 4, 6


def _dft_matrices():
    k = np.arange(T, dtype=np.float64)[:, None]
    t = np.arange(T, dtype=np.float64)[None, :]
    theta = 2.0 * np.pi * (k + 0.25) * t / T
    re = np.cos(theta).reshape(T // 8, 1, 8, T)
    im = np.sin(theta).reshape(T // 8, 1, 8, T)
    fwd = np.concatenate([re, im], axis=1).reshape(2 * T, T)
    return (fwd.astype(np.float32).astype(BF16),
            (fwd.T / T).astype(np.float32).astype(BF16))


_FWD, _INV = _dft_matrices()


def _dot(a, b):
    return jnp.dot(a, b, preferred_element_type=F32)


def _dot_nt(a, b):
    return lax.dot_general(a, b, (((1,), (1,)), ((), ())), preferred_element_type=F32)


def _phi(t):
    return jnp.where(t > 0, t + 1.0, jnp.exp(t))


def _tile(i):
    return slice(i * T, (i + 1) * T)


def _iota(shape, axis):
    return lax.broadcasted_iota(jnp.int32, shape, axis)


def _add(xs, ys):
    return [x + y for x, y in zip(xs, ys)]


def _causal_complex(ur, ui, gr, gi):
    re, im = [], []
    for a in range(len(ur)):
        x = ur[0] * gr[a] - ui[0] * gi[a]
        y = ur[0] * gi[a] + ui[0] * gr[a]
        for j in range(1, a + 1):
            x = x + (ur[j] * gr[a - j] - ui[j] * gi[a - j])
            y = y + (ur[j] * gi[a - j] + ui[j] * gr[a - j])
        re.append(x)
        im.append(y)
    return re, im


class _Group:
    def __init__(self, g, paired):
        self.r0 = g * GR if isinstance(g, int) else pl.multiple_of(g * GR, 16)
        self.rows = pl.ds(self.r0, GR)
        self.paired = paired
        self.kn, self.va, self.w, self.w2 = {}, {}, {}, {}
        self.maxes, self.accs, self.rets, self.mems = {}, {}, {}, {}
        self.bad = None


def _kernel(
    q_hbm, k_hbm, v_hbm, shift_hbm, h_hbm, d_hbm, x_hbm,
    wq_hbm, wk_hbm, wv_hbm, wo_hbm, beta_hbm, fwd_hbm, inv_hbm,
    out_hbm,
    q_v, k_v, v_v, shift_v, h_v, d_v, x_v, w_v, wo_v, beta_v, fwd_v, inv_v,
    wt_s, xu_s, taps_s, gate_s, kpad_s, kv_s, spec_s, yf_s, ya_s,
    qs_s, pq_s, kt_s, pk_s, vt_s, ot_s, yb_s, s_ring, kn0_s, zero_ref,
    in_sem, slab_sem, w_sem, x_sem, outa_sem, outb_sem, *p_ring,
):
    def slab(c):
        return pl.ds(c * T if isinstance(c, int) else pl.multiple_of(c * T, T), T)

    def kvh_copies(c):
        return (
            pltpu.make_async_copy(k_hbm.at[:, slab(c)], k_v.at[c], slab_sem.at[0, c]),
            pltpu.make_async_copy(v_hbm.at[:, slab(c)], v_v.at[c], slab_sem.at[1, c]),
            pltpu.make_async_copy(h_hbm.at[slab(c), :], h_v.at[c], slab_sem.at[2, c]),
        )

    def q_copy(c):
        return [pltpu.make_async_copy(q_hbm.at[:, slab(c)], q_v.at[c], slab_sem.at[3, c])]

    def w_copies(c):
        return [pltpu.make_async_copy(w.at[:, slab(c)], w_v.at[c, i], w_sem.at[i, c])
                for i, w in enumerate((wq_hbm, wk_hbm, wv_hbm))]

    def x_copy(b):
        rows = pl.ds(b * L, L)
        return [pltpu.make_async_copy(x_hbm.at[rows, :], x_v.at[rows, :], x_sem.at[b])]

    def outa_copy(c):
        return [pltpu.make_async_copy(ya_s.at[c], out_hbm.at[:, slab(c)], outa_sem.at[c])]

    def outb_copy(b):
        r0 = b * OB if isinstance(b, int) else pl.multiple_of(b * OB, OB)
        dst = out_hbm.at[pl.ds(r0, OB), pl.ds(D, D)]
        return [pltpu.make_async_copy(yb_s.at[b], dst, outb_sem.at[b])]

    small = [pltpu.make_async_copy(src, dst, in_sem.at[i]) for i, (src, dst) in enumerate(
        [(shift_hbm, shift_v), (d_hbm, d_v), (beta_hbm, beta_v),
         (fwd_hbm, fwd_v), (inv_hbm, inv_v)])]
    wo_copy = [pltpu.make_async_copy(wo_hbm, wo_v, in_sem.at[len(small)])]

    def start(*groups):
        for group in groups:
            for copy in group:
                copy.start()

    def wait(*groups):
        for group in groups:
            for copy in group:
                copy.wait()

    def start_now(*groups):
        def body(_, carry):
            start(*groups)
            return carry

        lax.fori_loop(0, zero_ref[7] + 1, body, 0)

    def zeros(n0, n1, align):
        return [pl.multiple_of(zero_ref[n], align) for n in range(n0, n1)]

    def small_tables():
        shift, skip = shift_v[...].astype(F32), d_v[...].astype(F32)
        for c in range(ND):
            taps_s[c, 0:KS, :] = shift[:, _tile(c)]
            taps_s[c, KS:KS + 1, :] = skip[c:c + 1, :]
        g_row = jax.nn.sigmoid(beta_v[...].astype(F32))
        row, head = _iota((D, H), 0), _iota((D, H), 1)
        own = (row >= head * DH) & (row < (head + 1) * DH)
        g_col = jnp.sum(jnp.where(own, g_row, 0.0), axis=1, keepdims=True)
        gate_s[...] = jnp.broadcast_to(g_col, (D, T))

    def tap(c, j):
        return taps_s[c, j:j + 1, :]

    def kv_prep(c, a0=0, a1=NT):
        w = [tap(c, j) for j in range(KS)]
        kpad_s[8 + a0 * T:8 + a1 * T, :] = k_v[c, a0 * T:a1 * T, :].astype(F32)
        for a in range(a0, a1):
            acc = None
            for j in range(KS):
                term = kpad_s[8 + a * T - j:8 + (a + 1) * T - j, :] * w[j]
                acc = term if acc is None else acc + term
            kv = acc * v_v[c, _tile(a), :].astype(F32)
            kv_s[_tile(a), :] = kv.astype(BF16)
        return kv[T - 8:]

    def store_spectrum(c, z, off, a, re, im):
        for f in range(T // 8):
            for m, part in enumerate((re, im)):
                rows = pl.ds(z[0] + off + 16 * f + 8 * m, 8)
                spec_s[(c % 2) * NT + a, rows, :] = part[f]

    def split(val, a):
        return ([val[16 * f:16 * f + 8, _tile(a)] for f in range(T // 8)],
                [val[16 * f + 8:16 * f + 16, _tile(a)] for f in range(T // 8)])

    def fwd_h(c, z):
        h_rows = jnp.concatenate([h_v[c, :, _tile(a)] for a in range(NT)], axis=0)
        val = _dot_nt(fwd_v[...], h_rows)
        skip = tap(c, KS)
        prev = None
        for a in range(NT):
            hr, hi = split(val, a)
            if prev is None:
                hr = [x + skip for x in hr]
                gr, gi = hr, hi
            else:
                gr = _add(hr, prev[1])
                gi = [x - y for x, y in zip(hi, prev[0])]
            prev = (hr, hi)
            store_spectrum(c, z, SP_H, a, gr, gi)

    def fwd_u(c, z):
        u = jnp.concatenate([kv_s[_tile(a), :] for a in range(NT)], axis=1)
        val = _dot(fwd_v[...], u)
        for a in range(NT):
            store_spectrum(c, z, SP_U, a, *split(val, a))

    def pace(z, val):
        spec_s[0, pl.ds(z[0] + SP_PACE, 8), :] = val

    def chunk_conv(c, z, f):
        def load(off):
            return [spec_s[(c % 2) * NT + a, pl.ds(z[1] + off + 16 * f, 8), :]
                    for a in range(NT)]

        gr, gi, ur, ui = load(SP_H), load(SP_H + 8), load(SP_U), load(SP_U + 8)
        er, ei = _causal_complex(ur[0::2], ui[0::2], gr[0::2], gi[0::2])
        o_r, o_i = _causal_complex(ur[1::2], ui[1::2], gr[1::2], gi[1::2])
        mr, mi = _causal_complex(_add(ur[0::2], ur[1::2]), _add(ui[0::2], ui[1::2]),
                                 _add(gr[0::2], gr[1::2]), _add(gi[0::2], gi[1::2]))
        re, im = [None] * NT, [None] * NT
        for m in range(NT // 2):
            re[2 * m] = er[m] if m == 0 else er[m] + o_r[m - 1]
            im[2 * m] = ei[m] if m == 0 else ei[m] + o_i[m - 1]
            re[2 * m + 1] = mr[m] - er[m] - o_r[m]
            im[2 * m + 1] = mi[m] - ei[m] - o_i[m]
        for a in range(NT):
            yf_s[a, 16 * f:16 * f + 16, :] = jnp.concatenate(
                [re[a], im[a]], axis=0).astype(BF16)

    def inverse(c):
        y = _dot(inv_v[...], jnp.concatenate([yf_s[a] for a in range(NT)], axis=1))
        for a in range(NT):
            ya_s[c, _tile(a), :] = (
                q_v[c, _tile(a), :].astype(F32) * y[:, _tile(a)]).astype(BF16)

    def transpose_w(c):
        for i in range(3):
            for j in range(ND):
                wt_s[c, j, i * T // 2:(i + 1) * T // 2, :] = pltpu.bitcast(
                    w_v[c, i, _tile(j), :].T, U32)

    def project(c, b):
        w = jnp.concatenate([pltpu.bitcast(wt_s[c, j], BF16) for j in range(ND)], axis=1)
        half = slice(b * L // 2, (b + 1) * L // 2)
        if isinstance(c, int):
            xb = x_v[b * L:(b + 1) * L, :]
            for j in range(ND):
                xu_s[j, half, :] = pltpu.bitcast(xb[:, _tile(j)], U32)
        else:
            xb = jnp.concatenate(
                [pltpu.bitcast(xu_s[j, half, :], BF16) for j in range(ND)], axis=1)
        r = _dot_nt(w, xb)
        rows = slab(c)
        for m in range(TPL):
            a = b * TPL + m
            qf, kf, vf = (r[_tile(i), _tile(m)] for i in range(3))
            qs_s[a, rows, :] = (qf * Q_SCALE).astype(BF16)
            kb = kf.astype(BF16)
            kt_s[a, rows, :] = kb
            vt_s[a, rows, :] = vf.astype(BF16)
            if b > 0:
                pq_s[a - TPL, rows, :] = _phi(qf.astype(BF16).astype(F32)).astype(BF16)
            if b < NSEG - 1:
                pk_s[a, rows, :] = _phi(kb.astype(F32)).astype(BF16)
        return r[3 * T - 8:, 0:T]

    def phase1(c, carry):
        wait(kvh_copies(c + 1), q_copy(c))

        @pl.when(c + 2 < ND)
        def _():
            wait(w_copies(c + 2))
            start(kvh_copies(c + 2))

        @pl.when(c + 3 < ND)
        def _():
            start(w_copies(c + 3))

        @pl.when(c + 3 == ND)
        def _():
            start(wo_copy)

        @pl.when(zero_ref[7] == 0)
        def _():
            start(q_copy(c + 1))

        z = zeros(0, 2, 8)
        transpose_w(jnp.minimum(c + 2, ND - 1))
        halves = PHASE1_ORDER.count("k")
        nb = nf = nk = 0
        for ch in PHASE1_ORDER:
            if ch == "h":
                fwd_h(c + 1, z)
            elif ch == "u":
                fwd_u(c + 1, z)
            elif ch == "i":
                inverse(c)
            elif ch in "pc":
                last = project(c + 1, nb)
                nb += 1
                if ch == "c":
                    pace(z, last)
            elif ch == "k":
                pace(z, kv_prep(c + 1, nk * NT // halves, (nk + 1) * NT // halves))
                nk += 1
            else:
                chunk_conv(c, z, nf)
                nf += 1
        assert nb == NSEG and nf == NT
        start(outa_copy(c))
        return carry

    def low4():
        return _iota((8, T), 0) < 4

    def pad_rows(x):
        return jnp.concatenate([x, jnp.zeros((T - GR, x.shape[1]), x.dtype)], axis=0)

    def keys(G, a):
        if a not in G.kn:
            G.kn[a] = pad_rows(kt_s[a, G.rows, :]).T
        return G.kn[a]

    def values(G, a):
        if a not in G.va:
            vt = vt_s[a, G.rows, :]
            b = [vt[16 * m:16 * m + 16] for m in range(5)]
            lo = low4()
            one2 = jnp.full((8, T), 0x3F803F80, U32)

            def top(x):
                return pltpu.bitcast(jnp.where(lo, pltpu.bitcast(x, U32), one2), BF16)

            def bottom(x):
                return pltpu.bitcast(jnp.where(lo, one2, pltpu.bitcast(x, U32)), BF16)

            G.va[a] = [jnp.concatenate(p, axis=0) for p in (
                [b[0], top(b[1])], [b[1], top(b[2])],
                [bottom(b[2]), b[3]], [bottom(b[3]), b[4]])]
        return G.va[a]

    def queries(G, a):
        if a not in G.w:
            pair = _iota((16, T), 0)
            blks = []
            for h in range(GH):
                lo = (h * DH - 16 * h) // 2
                blk = pltpu.bitcast(qs_s[a, pl.ds(G.r0 + 16 * h, 32), :], U32)
                blk = jnp.where((pair >= lo) & (pair < lo + DH // 2), blk,
                                jnp.zeros_like(blk))
                if G.paired and h % 2:
                    blk = pltpu.roll(blk, T // 2, 1)
                blks.append(blk)

            def place(blk, h):
                rest = T - 16 * h - 2 * blk.shape[0]
                pieces = [pltpu.bitcast(blk, BF16), jnp.zeros((rest, T), BF16)]
                if h:
                    pieces = [jnp.zeros((16 * h, T), BF16)] + pieces
                return jnp.concatenate(pieces, axis=0)

            G.w[a] = jnp.concatenate([place(blks[h], h) for h in range(GH)], axis=1)
            if G.paired:
                left = _iota((24, T), 1) < T // 2
                zero = jnp.zeros((8, T), U32)
                G.w2[a] = jnp.concatenate([
                    place(jnp.where(left, jnp.concatenate([zero, blks[h + 1]], axis=0),
                                    jnp.concatenate([blks[h], zero], axis=0)), h)
                    for h in range(0, GH, 2)], axis=1)
        return G.w[a]

    def update(G, s):
        ones = jnp.ones((16, T), BF16)
        va = jnp.concatenate(
            [jnp.concatenate([vt_s[s * TPL + j, G.rows, :], ones], axis=0)
             for j in range(TPL)], axis=1)
        pk = jnp.concatenate(
            [pad_rows(pk_s[s * TPL + j, G.rows, :]) for j in range(TPL)], axis=1)
        row, lane = _iota((GR + 16, T), 0), _iota((GR + 16, T), 1)
        keep = None
        for h in range(GH):
            mine = (((row >= h * DH) & (row < (h + 1) * DH))
                    | ((row >= GR + 4 * h) & (row < GR + 4 * h + 4)))
            mine = mine & (lane >= h * DH) & (lane < (h + 1) * DH)
            keep = mine if keep is None else keep | mine
        upd = jnp.where(keep, _dot_nt(va, pk), 0.0)
        G.mems[s + 1] = upd if s == 0 else G.mems[s] + upd

    def retrieve(G, s):
        pq = jnp.concatenate(
            [pad_rows(pq_s[(s - 1) * TPL + i, G.rows, :]) for i in range(TPL)], axis=1)
        ret = _dot(G.mems[s].astype(BF16), pq)
        gate = gate_s[G.rows, :]
        lo = low4()
        for i in range(TPL):
            inv = []
            for m in range(2):
                r = 1.0 / (ret[GR + 8 * m:GR + 8 * m + 8, _tile(i)] + 1e-6)
                other = pltpu.roll(r, 4, 0)
                first, second = jnp.where(lo, r, other), jnp.where(lo, other, r)
                inv += [first, first, r, second, second]
            G.rets[(s, i)] = ret[:GR, _tile(i)] * (gate * jnp.concatenate(inv, axis=0))

    def memory_steps(G, t):
        s, k = divmod(t, NSTEP // NSEG)
        if k == 2 and s > 0:
            retrieve(G, s)
        if k == 6 and s < NSEG - 1:
            update(G, s)

    def finish(G, s, i):
        accs = [G.accs[(s, i, h)] for h in range(GH)]
        if G.paired:
            accs = [pltpu.roll(x, T // 2, 1) if h % 2 else x for h, x in enumerate(accs)]
        u = [[x[8 * m:8 * m + 8] for m in range(4)] for x in accs]
        lo = low4()
        vals = jnp.concatenate(
            [u[0][0], u[0][1], jnp.where(lo, u[0][2], u[1][0]), u[1][1], u[1][2],
             u[2][1], u[2][2], jnp.where(lo, u[2][3], u[3][1]), u[3][2], u[3][3]], axis=0)
        sums = (u[0][3], u[1][3], u[2][0], u[3][0])
        if G.bad is not None:
            for d in sums:
                ok = (d >= 2.0 ** -SUM_LOG2) & (d <= 2.0 ** SUM_LOG2)
                G.bad = jnp.where(ok, G.bad, 1.0)
        r = [1.0 / d for d in sums]
        inv = jnp.concatenate(
            [r[0], r[0], jnp.where(lo, r[0], r[1]), r[1], r[1],
             r[2], r[2], jnp.where(lo, r[2], r[3]), r[3], r[3]], axis=0)
        o = vals * ((1.0 - gate_s[G.rows, :]) * inv)
        if s > 0:
            o = o + G.rets[(s, i)]
        ot_s[s * TPL + i, G.rows, :] = o.astype(BF16)

    def accumulate(G, s, i, j, h, p):
        r = _dot(values(G, s * TPL + j)[h], p)
        G.accs[(s, i, h)] = r if j == 0 else G.accs[(s, i, h)] + r

    def qk_direct(G, t):
        s, i, j = STEPS[t]
        kn, w = keys(G, s * TPL + j), queries(G, s * TPL + i)
        if j < i:
            return _dot(kn, w)
        late_keys = _dot(kn[T // 2:], G.w2[s * TPL + i])
        return _dot(kn[:T // 2], w), late_keys

    def exp_direct(t, raw, ps):
        _, i, j = STEPS[t]
        if j < i:
            for h in range(GH):
                p_ring[t % RP][pl.ds(ps + h * T, T), :] = jnp.exp2(
                    raw[:, _tile(h)]).astype(BF16)
            return
        key, lane = _iota((T // 2, T), 0), _iota((T // 2, T), 1)
        qry = (lane, (lane + T // 2) & (T - 1))
        shared = [jnp.exp2(raw[1][:, _tile(m)]) for m in range(GH // 2)]
        for h in range(GH):
            top = jnp.where(key <= qry[h % 2], jnp.exp2(raw[0][:, _tile(h)]), 0.0)
            bot = jnp.where(key + T // 2 <= qry[h % 2], shared[h // 2], 0.0)
            p_ring[t % RP][pl.ds(ps + h * T, T), :] = jnp.concatenate(
                [top, bot], axis=0).astype(BF16)

    def pv_direct(G, t, po):
        s, i, j = STEPS[t]
        for h in range(GH):
            accumulate(G, s, i, j, h, p_ring[t % RP][pl.ds(po + h * T, T), :])
        if j == i:
            finish(G, s, i)

    def adopt(g, state):
        P = _Group(g, True)
        P.accs = dict(zip(_ACC_KEYS, state[0]))
        P.rets = dict(zip(_RET_KEYS, state[1]))
        P.bad = state[2]
        return P

    def attention(g, state):
        ps, po = zeros(2, 4, 16)
        G = _Group(g, True)
        if state is None:
            P = None
            G.bad = jnp.zeros((8, T), F32)
        else:
            P = adopt(g - 1, state)
        G.kn[0] = kn0_s[...]
        done = 0
        for t in range(NSTEP):
            raw = qk_direct(G, t)
            memory_steps(G, t)
            if t < PV_CARRY and P is not None:
                pv_direct(P, NSTEP - PV_CARRY + t, po)
                G.bad = P.bad
            while done <= (t - PV_LAG if t < NSTEP - 1 else t - PV_CARRY):
                pv_direct(G, done, po)
                done += 1
            exp_direct(t, raw, ps)
            if t == NSTEP - 4 and P is not None:
                kn0_s[...] = keys(_Group(jnp.minimum(g + 1, NGRP - 1), True), 0)
        return [G.accs[k] for k in _ACC_KEYS], [G.rets[k] for k in _RET_KEYS], G.bad

    def attention_true_max(g, carry):
        zs, zl = zeros(0, 2, 8)
        ps, po = zeros(2, 4, 16)
        G = _Group(g, False)
        part = T // GH
        for t in range(NSTEP + MAX_PV_LAG):
            if t < NSTEP:
                s, i, j = STEPS[t]
                raw = _dot(keys(G, s * TPL + j), queries(G, s * TPL + i))
                memory_steps(G, t)
            if t >= MAX_PV_LAG:
                tp = t - MAX_PV_LAG
                for m in range(GH):
                    tq, h = _CELLS[tp * GH + m]
                    sp, ip, jp = STEPS[tq]
                    accumulate(G, sp, ip, jp, h, p_ring[tp % RP][pl.ds(po + m * T, T), :])
                    if jp == ip and h == GH - 1:
                        finish(G, sp, ip)
            for m in range(GH):
                if t < NSTEP:
                    r0 = m * part
                    causal = r0 + _iota((part, T), 0) <= _iota((part, T), 1)
                    ms = []
                    for h in range(GH):
                        sc = raw[r0:r0 + part, _tile(h)]
                        if j == i:
                            sc = jnp.where(causal, sc, NEG)
                        s_ring[pl.ds(zs + ((t % RS) * GH + h) * T + r0, part), :] = sc
                        m8 = sc[0:8]
                        for r in range(1, part // 8):
                            m8 = jnp.maximum(m8, sc[8 * r:8 * r + 8])
                        if j > 0 or m > 0:
                            m8 = jnp.maximum(G.maxes[(s, i)][h], m8)
                        if j == i and m == GH - 1:
                            m8 = jnp.broadcast_to(
                                jnp.max(m8, axis=0, keepdims=True), (8, T))
                        ms.append(m8)
                    G.maxes[(s, i)] = ms
                if EXP_LAG <= t < NSTEP + EXP_LAG:
                    te = t - EXP_LAG
                    tq, h = _CELLS[te * GH + m]
                    top = jnp.concatenate([G.maxes[STEPS[tq][:2]][h]] * (T // 8), axis=0)
                    sc = s_ring[pl.ds(zl + ((tq % RS) * GH + h) * T, T), :]
                    p_ring[te % RP][pl.ds(ps + m * T, T), :] = jnp.exp2(
                        sc - top).astype(BF16)
        return carry

    def out_proj(b):
        o = jnp.concatenate(
            [jnp.concatenate([ot_s[b * (OB // T) + m, _tile(j), :].T for j in range(ND)],
                             axis=1) for m in range(OB // T)], axis=0)
        r = _dot(o, wo_v[...])
        yb_s[b] = r.astype(BF16)
        return r[OB - 8:, D - T:]

    start(w_copies(0), x_copy(0))

    def clear(i, carry):
        zero_ref[i] = jnp.int32(0)
        return carry

    lax.fori_loop(0, 8, clear, 0)
    kpad_s[0:8, :] = jnp.zeros((8, T), F32)
    wait(w_copies(0))
    transpose_w(0)
    wait(x_copy(0))
    start(x_copy(1), small)
    project(0, 0)
    wait(x_copy(1), small)
    start(x_copy(2))
    small_tables()
    project(0, 1)
    wait(x_copy(2))
    start(x_copy(3))
    project(0, 2)
    wait(x_copy(3))
    start_now(kvh_copies(0), w_copies(1), kvh_copies(1), q_copy(0), w_copies(2))
    kn0_s[...] = keys(_Group(0, True), 0)
    project(0, 3)
    state = attention(0, None)
    wait(kvh_copies(0), w_copies(1))
    z = zeros(0, 2, 8)
    fwd_h(0, z)
    kv_prep(0)
    transpose_w(1)
    fwd_u(0, z)

    lax.fori_loop(0, ND - 1, phase1, 0)

    kn0_s[...] = keys(_Group(1, True), 0)
    state = lax.fori_loop(1, NGRP, attention, state)

    wait(wo_copy, q_copy(ND - 1))
    last_group = adopt(NGRP - 1, state)
    z = zeros(0, 2, 8)
    nb = nf = 0
    for ch in PHASE3_ORDER:
        if ch == "t":
            (po,) = zeros(3, 4, 16)
            for t in range(NSTEP - PV_CARRY, NSTEP):
                pv_direct(last_group, t, po)
        elif ch == "v":
            chunk_conv(ND - 1, z, nf)
            nf += 1
        elif ch == "i":
            inverse(ND - 1)
        elif ch == "a":
            start(outa_copy(ND - 1))
        elif ch in "pc":
            last = out_proj(nb)
            nb += 1
            if ch == "c":
                pace(z, last)
        else:
            start(outb_copy(int(ch)))
    assert nb == S // OB and nf == NT
    unsafe = jnp.max(last_group.bad) > 0.0

    for c in range(ND):
        wait(outa_copy(c))
    for b in range(S // OB):
        wait(outb_copy(b))

    @pl.when(unsafe)
    def _():
        lax.fori_loop(0, NGRP, attention_true_max, 0)

        def redo_block(b, carry):
            out_proj(b)
            start(outb_copy(b))
            wait(outb_copy(b))
            return carry

        lax.fori_loop(0, S // OB, redo_block, 0)


@jax.jit
def pallas_concat_heads__ssm_conv_h3__memory_aug_infini_attn__prompt_kernel(
    A_q: jax.Array,
    A_k: jax.Array,
    A_v: jax.Array,
    A_shift_k: jax.Array,
    A_ssm_k: jax.Array,
    A_ssm_D: jax.Array,
    B_x: jax.Array,
    B_wq: jax.Array,
    B_wk: jax.Array,
    B_wv: jax.Array,
    B_wo: jax.Array,
    B_beta: jax.Array,
):
    hbm = pl.BlockSpec(memory_space=pltpu.MemorySpace.HBM)
    vmem = pltpu.VMEM
    dma = pltpu.SemaphoreType.DMA
    out = pl.pallas_call(
        _kernel,
        out_shape=jax.ShapeDtypeStruct((S, 2 * D), BF16),
        in_specs=[hbm] * 14,
        out_specs=hbm,
        scratch_shapes=[
            vmem((ND, S, T), BF16),
            vmem((ND, S, T), BF16),
            vmem((ND, S, T), BF16),
            vmem((KS, D), BF16),
            vmem((ND, T, S), BF16),
            vmem((ND, T), BF16),
            vmem((S, D), BF16),
            vmem((ND, 3, D, T), BF16),
            vmem((D, D), BF16),
            vmem((1, H), BF16),
            vmem((2 * T, T), BF16),
            vmem((T, 2 * T), BF16),
            vmem((ND, ND, 3 * T // 2, T), U32),
            vmem((ND, S // 2, T), U32),
            vmem((ND, 8, T), F32),
            vmem((D, T), F32),
            vmem((S + 8, T), F32),
            vmem((S, T), BF16),
            vmem((2 * NT, SP_PACE + 8, T), F32),
            vmem((NT, 2 * T, T), BF16),
            vmem((ND, S, T), BF16),
            vmem((NT, D, T), BF16),
            vmem((NT - TPL, D, T), BF16),
            vmem((NT, D, T), BF16),
            vmem((NT - TPL, D, T), BF16),
            vmem((NT, D, T), BF16),
            vmem((NT, D, T), BF16),
            vmem((S // OB, OB, D), BF16),
            vmem((RS * GH * T, T), F32),
            vmem((T, T), BF16),
            pltpu.SMEM((8,), jnp.int32),
            dma((6,)),
            dma((4, ND)),
            dma((3, ND)),
            dma((NSEG,)),
            dma((ND,)),
            dma((S // OB,)),
        ] + [vmem((GH * T, T), BF16)] * RP,
        compiler_params=pltpu.CompilerParams(vmem_limit_bytes=100 * 1024 * 1024),
        name="h3_infini_concat",
    )(
        A_q.reshape(S, D), A_k.reshape(S, D), A_v.reshape(S, D), A_shift_k.T, A_ssm_k,
        A_ssm_D.reshape(ND, T), B_x.reshape(S, D), B_wq, B_wk, B_wv, B_wo,
        B_beta.reshape(1, H), jnp.asarray(_FWD), jnp.asarray(_INV),
    )
    return out.reshape(1, S, 2 * D)
```
